```python
import jax
import jax.numpy as jnp

def _softmax(x, axis=-1):
    return jax.nn.softmax(x, axis=axis)
def _gelu(x):
    return jax.nn.gelu(x, approximate=True)
def _silu(x):
    return jax.nn.silu(x)
def _sigmoid(x):
    return jax.nn.sigmoid(x)
def _layernorm(x, axis=-1, eps=1e-5):
    m = jnp.mean(x, axis=axis, keepdims=True)
    v = jnp.var(x, axis=axis, keepdims=True)
    return (x - m) / jnp.sqrt(v + eps)
def _scatter_add(tgt, idx, src, axis=0):
    return tgt.at[idx].add(src)
def _segment_sum(src, seg, n):
    return jax.ops.segment_sum(src, seg, n)
class _Rng:
    def __init__(self, key):
        self._k = key
    def _next(self):
        self._k, sub = jax.random.split(self._k)
        return sub
    def normal(self, shape):
        return jax.random.normal(self._next(), shape, dtype=jnp.bfloat16)
    def randint(self, lo, hi, shape):
        return jax.random.randint(self._next(), shape, lo, hi, dtype=jnp.int32)
    def uniform(self, shape, lo=0.0, hi=1.0):
        return jax.random.uniform(self._next(), shape, jnp.bfloat16, lo, hi)
    def permutation(self, n):
        return jax.random.permutation(self._next(), n)


kernel_name = 'standalone__batchnorm__sampling'

def setup_inputs():
    _rng = _Rng(jax.random.key(int.from_bytes(__import__("os").urandom(4), "little")))
    _w = (lambda a: (lambda t: t.astype(jnp.bfloat16) if jnp.issubdtype(t.dtype, jnp.floating) else t)(jnp.asarray(a)))
    B, S, C = 1024, 32, 576
    K = 3
    return {
        "x": _w((lambda *s: _rng.normal(s) * 0.05)(B, S, C)),
        "w": _w((lambda *s: _rng.normal(s) * 0.05)(K, C, C) * (1.0 / (K * C) ** 0.5)),
        "mean": _w((lambda *s: _rng.normal(s) * 0.05)(C) * 0.1),
        "var": _w(jnp.abs((lambda *s: _rng.normal(s) * 0.05)(C)) + 0.5),
        "g": _w((lambda *s: _rng.normal(s) * 0.05)(C) + 1.0),
        "b": _w((lambda *s: _rng.normal(s) * 0.05)(C) * 0.1),
    }

def reference(x, w, mean, var, g, b):
    K = 3
    P = K // 2
    S = x.shape[1]
    xp = jnp.pad(x, ((0, 0), (P, P), (0, 0)))
    y = sum(jnp.einsum('bsc,cd->bsd', xp[:, k:k + S, :], w[k]) for k in range(K))
    inv_std = 1.0 / jnp.sqrt(var + 1e-5)
    y = (y - mean) * (g * inv_std) + b
    return _silu(y)
```

```python
import functools
import jax
import jax.numpy as jnp
import jax.experimental.pallas as pl
import jax.experimental.pallas.tpu as pltpu

NB = 128
PA = 2.0 / 3.0
PB = 1.5
UNROLL = 6

def _g_rows():
    pts = [0.0, PA, -PA, PB, -PB]
    rows = []
    for i, p in enumerate(pts):
        den = 1.0
        for j, q in enumerate(pts):
            if j != i:
                den *= (p - q)
        rows.append((1.0 / den, p / den, p * p / den))
    rows.append((0.0, 0.0, 1.0))
    return rows


def _kernel(x_ref, w_ref, p_ref, o_ref, wt_ref, sc_ref, sh_ref):
    S, C, NBk = x_ref.shape
    f32 = jnp.float32

    @pl.when(pl.program_id(0) == 0)
    def _():
        wt = [w_ref[k].astype(f32).T for k in range(3)]
        for i, (a, b, c) in enumerate(_g_rows()):
            acc = None
            for coef, m in zip((a, b, c), wt):
                if coef != 0.0:
                    t = m * coef if coef != 1.0 else m
                    acc = t if acc is None else acc + t
            wt_ref[i] = acc.astype(jnp.bfloat16)
        p = p_ref[...].astype(f32)
        scale = p[:, 2:3] * jax.lax.rsqrt(p[:, 1:2] + 1e-5)
        shift = p[:, 3:4] - p[:, 0:1] * scale
        sc_ref[...] = jnp.broadcast_to(0.5 * scale, (C, NBk))
        sh_ref[...] = jnp.broadcast_to(0.5 * shift, (C, NBk))

    def epi(y, s):
        h = y * sc_ref[...] + sh_ref[...]
        o_ref[s] = (h * jnp.tanh(h) + h).astype(o_ref.dtype)

    a, b = PA, PB
    a2, b2 = a * a, b * b

    def group(s0, first=False, last=False):
        d = [None] * 6
        for i in range(6):
            if (first and i == 0) or (last and i == 5):
                continue
            d[i] = x_ref[s0 - 1 + i].astype(f32)
        a2d2 = a2 * d[2]
        t1 = d[4] - b2 * d[2]
        t3 = d[4] - a2d2
        t2 = a * d[3] - (a * b2) * d[1]
        t4 = b * d[3] - (b * a2) * d[1]
        u0 = t1 - a2d2
        if not first:
            u0 = u0 + (a2 * b2) * d[0] if abs(a2 * b2 - 1.0) > 1e-9 else u0 + d[0]
        u5 = d[1] - (a2 + b2) * d[3]
        if not last:
            u5 = u5 + d[5]
        u = [u0, t1 + t2, t1 - t2, t3 + t4, t3 - t4, u5]
        m = [jnp.dot(wt_ref[i], u[i].astype(jnp.bfloat16), preferred_element_type=f32) for i in range(6)]
        p = m[1] + m[2]
        q = m[1] - m[2]
        r = m[3] + m[4]
        t = m[3] - m[4]
        epi(m[0] + p + r, s0)
        epi(a * q + b * t, s0 + 1)
        epi(a2 * p + b2 * r, s0 + 2)
        epi((a * a2) * q + (b * b2) * t + m[5], s0 + 3)

    group(0, first=True)

    def body(j, c):
        group(j * 4)
        return c
    jax.lax.fori_loop(1, S // 4 - 1, body, 0, unroll=UNROLL)
    group(S - 4, last=True)


@jax.jit
def pallas_standalone__batchnorm__sampling_kernel(x, w, mean, var, g, b):
    B, S, C = x.shape
    xt = jnp.transpose(x, (1, 2, 0))
    p = jnp.stack([mean, var, g, b], axis=1)
    ot = pl.pallas_call(
        _kernel,
        grid=(B // NB,),
        in_specs=[pl.BlockSpec((S, C, NB), lambda i: (0, 0, i)),
                  pl.BlockSpec((3, C, C), lambda i: (0, 0, 0)),
                  pl.BlockSpec((C, 4), lambda i: (0, 0))],
        out_specs=pl.BlockSpec((S, C, NB), lambda i: (0, 0, i)),
        out_shape=jax.ShapeDtypeStruct((S, C, B), x.dtype),
        scratch_shapes=[pltpu.VMEM((6, C, C), jnp.bfloat16),
                        pltpu.VMEM((C, NB), jnp.float32),
                        pltpu.VMEM((C, NB), jnp.float32)],
        compiler_params=pltpu.CompilerParams(dimension_semantics=("arbitrary",),
                                             vmem_limit_bytes=96 * 1024 * 1024),
    )(xt, w, p)
    return jnp.transpose(ot, (2, 0, 1))
```

```python
import functools
import jax
import jax.numpy as jnp
import jax.experimental.pallas as pl
import jax.experimental.pallas.tpu as pltpu

NB = 128
PA = 2.0 / 3.0
PB = 1.5
CM = 512

_PTS = (0.0, PA, -PA, PB, -PB)


def _den(i):
    d = 1.0
    for j, q in enumerate(_PTS):
        if j != i:
            d *= (_PTS[i] - q)
    return d


def _kernel(x_hbm, w_hbm, p_ref, o_hbm, xbuf, obuf, wbuf, wt_ref, sc_ref, sh_ref, in_sem, out_sem, w_sem):
    S, C, B = x_hbm.shape
    NT = B // NB
    NG = S // 4
    CR = C - CM
    f32 = jnp.float32
    bf16 = jnp.bfloat16

    def lanes(bt):
        return pl.ds(pl.multiple_of(bt * NB, NB), NB)

    def in_copy(bt, slot):
        return pltpu.make_async_copy(x_hbm.at[:, :, lanes(bt)], xbuf.at[slot], in_sem.at[slot])

    def out_copy(bt, slot, lo, hi):
        return pltpu.make_async_copy(obuf.at[slot, lo:hi], o_hbm.at[lo:hi, :, lanes(bt)], out_sem.at[slot])

    w_copy = pltpu.make_async_copy(w_hbm, wbuf, w_sem.at[0])
    w_copy.start()
    in_copy(0, 0).start()

    p = p_ref[...].astype(f32)
    scale = p[:, 2:3] * jax.lax.rsqrt(p[:, 1:2] + 1e-5)
    shift = p[:, 3:4] - p[:, 0:1] * scale
    sc_ref[...] = jnp.broadcast_to(0.5 * scale, (C, NB))
    sh_ref[...] = jnp.broadcast_to(0.5 * shift, (C, NB))

    w_copy.wait()

    for d0 in range(0, C, 128):
        dn = min(128, C - d0)
        for c0 in range(0, CM, 128):
            g0, g1, g2 = [wbuf[k, c0:c0 + 128, d0:d0 + dn].T for k in range(3)]
            wt_ref[0, d0:d0 + dn, c0:c0 + 128] = g0
            wt_ref[5, d0:d0 + dn, c0:c0 + 128] = g2
            g0, g1, g2 = g0.astype(f32), g1.astype(f32), g2.astype(f32)
            for i in (1, 3):
                pt, den = _PTS[i], _den(i)
                ev = g0 * (1.0 / den) + g2 * (pt * pt / den)
                od = g1 * (pt / den)
                wt_ref[i, d0:d0 + dn, c0:c0 + 128] = (ev + od).astype(bf16)
                wt_ref[i + 1, d0:d0 + dn, c0:c0 + 128] = (ev - od).astype(bf16)
        w0r = wbuf[0, CM:C, d0:d0 + dn]
        xa = jnp.concatenate([w0r, jnp.zeros_like(w0r)], axis=0).T
        xb = jnp.concatenate([wbuf[1, CM:C, d0:d0 + dn], wbuf[2, CM:C, d0:d0 + dn]], axis=0).T
        wt_ref[0, d0:d0 + dn, CM:CM + 128] = xa
        xa, xb = xa.astype(f32), xb.astype(f32)
        for i in (1, 3):
            pt, den = _PTS[i], _den(i)
            ev = xa * (1.0 / den)
            od = xb * (pt / den)
            wt_ref[i, d0:d0 + dn, CM:CM + 128] = (ev + od).astype(bf16)
            wt_ref[i + 1, d0:d0 + dn, CM:CM + 128] = (ev - od).astype(bf16)

    a, b = PA, PB
    a2, b2 = a * a, b * b

    def body(bt, carry):
        slot = bt % 2

        in_copy(bt, slot).wait()

        @pl.when(bt >= 2)
        def _():
            out_copy(bt - 2, slot, 0, S).wait()

        @pl.when(bt + 1 < NT)
        def _():
            in_copy(bt + 1, 1 - slot).start()

        def epi(y, s):
            h = y * sc_ref[...] + sh_ref[...]
            obuf[slot, s] = (h * jnp.tanh(h) + h).astype(obuf.dtype)

        for j in range(NG):
            first, last = j == 0, j == NG - 1
            s0 = 4 * j
            d = [None] * 6
            for i in range(6):
                if (first and i == 0) or (last and i == 5):
                    continue
                d[i] = xbuf[slot, s0 - 1 + i].astype(f32)
            a2d2 = a2 * d[2]
            t1 = d[4] - b2 * d[2]
            t3 = d[4] - a2d2
            t2 = a * d[3] - (a * b2) * d[1]
            t4 = b * d[3] - (b * a2) * d[1]
            u0 = t1 - a2d2
            if not first:
                u0 = u0 + d[0]
            u5 = d[1] - (a2 + b2) * d[3]
            if not last:
                u5 = u5 + d[5]
            u = [u0, t1 + t2, t1 - t2, t3 + t4, t3 - t4, u5]
            m = []
            for i in range(6):
                if i == 0:
                    rhs, lhs = u[0].astype(bf16), wt_ref[0, :, 0:C]
                elif i == 5:
                    rhs, lhs = u[5][0:CM].astype(bf16), wt_ref[5, :, 0:CM]
                else:
                    ext = u5[CM:C] + _PTS[i] * u[i][CM:C]
                    rhs, lhs = jnp.concatenate([u[i].astype(bf16), ext.astype(bf16)], axis=0), wt_ref[i]
                m.append(jnp.dot(lhs, rhs, preferred_element_type=f32))
            p = m[1] + m[2]
            q = m[1] - m[2]
            r = m[3] + m[4]
            t = m[3] - m[4]
            epi(m[0] + p + r, s0)
            epi(a * q + b * t, s0 + 1)
            epi(a2 * p + b2 * r, s0 + 2)
            epi((a * a2) * q + (b * b2) * t + m[5], s0 + 3)
            out_copy(bt, slot, s0, s0 + 4).start()
        return carry

    jax.lax.fori_loop(0, NT, body, 0)
    for bt in (NT - 2, NT - 1):
        out_copy(bt, bt % 2, 0, S).wait()


@jax.jit
def pallas_standalone__batchnorm__sampling_kernel(x, w, mean, var, g, b):
    B, S, C = x.shape
    xt = jnp.transpose(x, (1, 2, 0))
    p = jnp.stack([mean, var, g, b], axis=1)
    ot = pl.pallas_call(
        _kernel,
        in_specs=[pl.BlockSpec(memory_space=pl.ANY),
                  pl.BlockSpec(memory_space=pl.ANY),
                  pl.BlockSpec(memory_space=pltpu.VMEM)],
        out_specs=pl.BlockSpec(memory_space=pl.ANY),
        out_shape=jax.ShapeDtypeStruct((S, C, B), x.dtype),
        scratch_shapes=[pltpu.VMEM((2, S, C, NB), jnp.bfloat16),
                        pltpu.VMEM((2, S, C, NB), jnp.bfloat16),
                        pltpu.VMEM((3, C, C), jnp.bfloat16),
                        pltpu.VMEM((6, C, CM + 128), jnp.bfloat16),
                        pltpu.VMEM((C, NB), jnp.float32),
                        pltpu.VMEM((C, NB), jnp.float32),
                        pltpu.SemaphoreType.DMA((2,)),
                        pltpu.SemaphoreType.DMA((2,)),
                        pltpu.SemaphoreType.DMA((1,))],
        compiler_params=pltpu.CompilerParams(vmem_limit_bytes=96 * 1024 * 1024),
    )(xt, w, p)
    return jnp.transpose(ot, (2, 0, 1))
```

```python
import functools
import jax
import jax.numpy as jnp
import jax.experimental.pallas as pl
import jax.experimental.pallas.tpu as pltpu

NB = 128
PA = 2.0 / 3.0
PB = 1.5
CM = 512
K_PRO = 4
N_PER = 6
STASH = (1,)
TCH = 32

_PTS = (0.0, PA, -PA, PB, -PB)


def _den(i):
    d = 1.0
    for j, q in enumerate(_PTS):
        if j != i:
            d *= (_PTS[i] - q)
    return d


def _kernel(x_hbm, w_hbm, mean_hbm, var_hbm, g_hbm, b_hbm, o_hbm,
            xall, oall, wbuf, pm, pv, pg, pb, w1t, wt_ref, sc_ref, sh_ref, u2,
            in_sem, out_sem, misc_sem):
    S, C, B = x_hbm.shape
    NT = B // NB
    NG = S // 4
    NGT = NT * NG
    N_IT = (NGT - K_PRO) // N_PER
    TS = S + 1
    KT = CM // 128 + 1
    CR = C - CM
    f32 = jnp.float32
    bf16 = jnp.bfloat16
    pk = lambda v: pltpu.bitcast(v, jnp.uint32)
    upk = lambda v: pltpu.bitcast(v, bf16)

    def in_copy(bt, lo, hi, sem):
        return pltpu.make_async_copy(x_hbm.at[lo:hi, :, bt * NB:(bt + 1) * NB],
                                     xall.at[bt * TS + 1 + lo:bt * TS + 1 + hi], sem)

    p_copies = [pltpu.make_async_copy(src, dst, misc_sem.at[6 + i])
                for i, (src, dst) in enumerate(((mean_hbm, pm), (var_hbm, pv), (g_hbm, pg), (b_hbm, pb)))]
    w_copies = [pltpu.make_async_copy(w_hbm.at[k], wbuf.at[k], misc_sem.at[k]) for k in range(3)]
    xa_copy = in_copy(0, 0, 5, misc_sem.at[3])
    xb_copy = in_copy(0, 5, 4 * K_PRO + 1, misc_sem.at[4])
    xc_copy = in_copy(0, 4 * K_PRO + 1, 4 * K_PRO + 8, misc_sem.at[5])
    for cp in [w_copies[0], xa_copy, w_copies[2], w_copies[1]] + p_copies + [xb_copy, xc_copy]:
        cp.start()
    for it in range(N_IT):
        lo = 4 * (K_PRO + 2 + N_PER * it)
        hi = min(lo + 4 * N_PER, NT * S)
        while lo < hi:
            bt = lo // S
            e = min(hi, (bt + 1) * S)
            in_copy(bt, lo - bt * S, e - bt * S, in_sem.at[it]).start()
            lo = e
    n_full = 4 * N_PER
    n_last = NT * S - 4 * (K_PRO + 2 + N_PER * (N_IT - 1))

    for bt in range(NT + 1):
        xall[bt * TS] = jnp.zeros((C, NB), bf16)

    a, b = PA, PB
    a2, b2 = a * a, b * b
    k_rows = (C, CM + 128, CM + 128, CM + 128, CM + 128, CM)

    def split(gi):
        if isinstance(gi, int):
            return gi // NG, gi % NG
        return jax.lax.shift_right_logical(gi, 3), jnp.bitwise_and(gi, NG - 1)

    def data_transform(d):
        a2d2 = a2 * d[2]
        t1 = d[4] - b2 * d[2]
        t3 = d[4] - a2d2
        t2 = a * d[3] - (a * b2) * d[1]
        t4 = b * d[3] - (b * a2) * d[1]
        u0 = t1 - a2d2 + d[0]
        u5 = d[1] - (a2 + b2) * d[3] + d[5]
        return [u0, t1 + t2, t1 - t2, t3 + t4, t3 - t4, u5]

    def transform(gi):
        bt, j = split(gi)
        base = bt * TS + 4 * j
        u = data_transform([xall[base + i].astype(f32) for i in range(6)])
        rhs = [u[0].astype(bf16)]
        for i in range(1, 5):
            ext = u[5][CM:C] + _PTS[i] * u[i][CM:C]
            rhs.append(jnp.concatenate([u[i], ext], axis=0).astype(bf16))
        rhs.append(u[5][0:CM].astype(bf16))
        return rhs

    def transform_to(dst, gi):
        bt, j = split(gi)
        base = bt * TS + 4 * j
        for c0 in range(0, C, TCH):
            u = data_transform([xall[base + i, c0:c0 + TCH, :].astype(f32) for i in range(6)])
            for n, i in enumerate(STASH):
                dst[n, c0 // 2:(c0 + TCH) // 2, :] = pk(u[i].astype(bf16))
                if c0 >= CM:
                    dst[n, (c0 + CR) // 2:(c0 + CR + TCH) // 2, :] = pk((u[5] + _PTS[i] * u[i]).astype(bf16))

    def prod(i, rhs_i):
        nk = (k_rows[i] + 127) // 128
        lhs = jnp.concatenate([upk(wt_ref[i, kt]) for kt in range(nk)], axis=1)[:, :k_rows[i]]
        return jnp.dot(lhs, rhs_i, preferred_element_type=f32)

    def epilogue(gi, m, split_out=False):
        bt, j = split(gi)

        def epi(y, s):
            h = y * sc_ref[...] + sh_ref[...]
            oall[4 * gi + s] = (h * jnp.tanh(h) + h).astype(oall.dtype)

        def out_copy(lo, hi):
            if isinstance(gi, int):
                ln = pl.ds(bt * NB, NB)
            else:
                ln = pl.ds(pl.multiple_of(bt * NB, NB), NB)
            pltpu.make_async_copy(oall.at[pl.ds(4 * gi + lo, hi - lo)],
                                  o_hbm.at[pl.ds(4 * j + lo, hi - lo), :, ln], out_sem.at[0]).start()

        p = m[1] + m[2]
        q = m[1] - m[2]
        r = m[3] + m[4]
        t = m[3] - m[4]
        epi(a * q + b * t, 1)
        epi(a2 * p + b2 * r, 2)
        epi((a * a2) * q + (b * b2) * t + m[5], 3)
        if split_out:
            out_copy(1, 4)
        epi(m[0] + p + r, 0)
        out_copy(0, 1 if split_out else 4)

    def finish(gi, rhs, split_out=False):
        epilogue(gi, [prod(i, rhs[i]) for i in range(6)], split_out)

    dblocks = [(d0, min(128, C - d0)) for d0 in range(0, C, 128)]

    def transpose_tap(k, dst):
        for d0, dn in dblocks:
            rows = slice(d0 // 2, (d0 + dn) // 2)
            for kt in range(KT - 1):
                dst[kt, rows, :] = pk(wbuf[k, kt * 128:(kt + 1) * 128, d0:d0 + dn].T)
            if k == 0:
                w0r = wbuf[0, CM:C, d0:d0 + dn]
                dst[KT - 1, rows, :] = pk(jnp.concatenate([w0r, jnp.zeros_like(w0r)], axis=0).T)
            elif k == 1:
                dst[KT - 1, rows, :] = pk(jnp.concatenate(
                    [wbuf[1, CM:C, d0:d0 + dn], wbuf[2, CM:C, d0:d0 + dn]], axis=0).T)

    def combine(i):
        pt, den = _PTS[i], _den(i)
        for kt in range(KT):
            for d0 in range(0, C, 64):
                rows = slice(d0 // 2, (d0 + 64) // 2)
                ev = upk(wt_ref[0, kt, rows, :]).astype(f32) * (1.0 / den)
                if kt < KT - 1:
                    ev = ev + upk(wt_ref[5, kt, rows, :]).astype(f32) * (pt * pt / den)
                od = upk(w1t[kt, rows, :]).astype(f32) * (pt / den)
                wt_ref[i, kt, rows, :] = pk((ev + od).astype(bf16))
                wt_ref[i + 1, kt, rows, :] = pk((ev - od).astype(bf16))

    m = [None] * 6
    w_copies[0].wait()
    transpose_tap(0, wt_ref.at[0])
    xa_copy.wait()
    rhs = transform(0)
    m[0] = prod(0, rhs[0])
    w_copies[2].wait()
    transpose_tap(2, wt_ref.at[5])
    m[5] = prod(5, rhs[5])
    w_copies[1].wait()
    transpose_tap(1, w1t)
    combine(1)
    for cp in p_copies:
        cp.wait()
    combine(3)
    m[1] = prod(1, rhs[1])
    m[2] = prod(2, rhs[2])
    row = lambda r: r[...].astype(f32).reshape(1, C)
    scale = row(pg) * jax.lax.rsqrt(row(pv) + 1e-5)
    shift = row(pb) - row(pm) * scale
    sc_ref[...] = jnp.broadcast_to(0.5 * scale, (NB, C)).T
    sh_ref[...] = jnp.broadcast_to(0.5 * shift, (NB, C)).T
    m[3] = prod(3, rhs[3])
    m[4] = prod(4, rhs[4])
    epilogue(0, m)

    xb_copy.wait()
    for gi in range(1, K_PRO):
        finish(gi, transform(gi))
    xc_copy.wait()
    transform_to(u2, K_PRO)

    def body(it, carry):
        g0 = K_PRO + N_PER * it
        pltpu.make_async_copy(xall.at[0:n_last], xall.at[0:n_last], in_sem.at[it]).wait()

        @pl.when(it < N_IT - 1)
        def _():
            n = n_full - n_last
            pltpu.make_async_copy(xall.at[0:n], xall.at[0:n], in_sem.at[it]).wait()

        rhs = transform(g0)
        for n, i in enumerate(STASH):
            rhs[i] = upk(u2[n, 0:k_rows[i] // 2, :])
        finish(g0, rhs)
        for r in range(1, N_PER):
            finish(g0 + r, transform(g0 + r), r == N_PER - 1)
        transform_to(u2, jnp.minimum(g0 + N_PER, NGT - 1))
        return carry

    jax.lax.fori_loop(0, N_IT, body, 0)
    pltpu.make_async_copy(oall, oall, out_sem.at[0]).wait()


@jax.jit
def pallas_standalone__batchnorm__sampling_kernel(x, w, mean, var, g, b):
    B, S, C = x.shape
    NT = B // NB
    n_it = (NT * (S // 4) - K_PRO) // N_PER
    xt = jnp.transpose(x, (1, 2, 0))
    ot = pl.pallas_call(
        _kernel,
        in_specs=[pl.BlockSpec(memory_space=pl.ANY)] * 6,
        out_specs=pl.BlockSpec(memory_space=pl.ANY),
        out_shape=jax.ShapeDtypeStruct((S, C, B), x.dtype),
        scratch_shapes=[pltpu.VMEM((NT * (S + 1) + 1, C, NB), jnp.bfloat16),
                        pltpu.VMEM((NT * S, C, NB), jnp.bfloat16),
                        pltpu.VMEM((3, C, C), jnp.bfloat16),
                        pltpu.VMEM((C,), jnp.bfloat16),
                        pltpu.VMEM((C,), jnp.bfloat16),
                        pltpu.VMEM((C,), jnp.bfloat16),
                        pltpu.VMEM((C,), jnp.bfloat16),
                        pltpu.VMEM((CM // 128 + 1, C // 2, 128), jnp.uint32),
                        pltpu.VMEM((6, CM // 128 + 1, C // 2, 128), jnp.uint32),
                        pltpu.VMEM((C, NB), jnp.float32),
                        pltpu.VMEM((C, NB), jnp.float32),
                        pltpu.VMEM((len(STASH), (CM + 128) // 2, NB), jnp.uint32),
                        pltpu.SemaphoreType.DMA((n_it,)),
                        pltpu.SemaphoreType.DMA((1,)),
                        pltpu.SemaphoreType.DMA((10,))],
        compiler_params=pltpu.CompilerParams(vmem_limit_bytes=110 * 1024 * 1024, disable_bounds_checks=True),
    )(xt, w, mean, var, g, b)
    return jnp.transpose(ot, (2, 0, 1))
```

```python
import jax
import jax.numpy as jnp
import jax.experimental.pallas as pl
import jax.experimental.pallas.tpu as pltpu

NB = 128
PA = 2.0 / 3.0
PB = 1.5
CM = 512
K_PRO = 4
N_PER = 6
TCH = 32

_PTS = (0.0, PA, -PA, PB, -PB)


def _den(i):
    d = 1.0
    for j, q in enumerate(_PTS):
        if j != i:
            d *= (_PTS[i] - q)
    return d


def _kernel(x_hbm, w_hbm, mean_hbm, var_hbm, g_hbm, b_hbm, o_hbm,
            xall, oall, wbuf, pm, pv, pg, pb, wt_ref, sc_ref, sh_ref, u_scr, m_scr,
            in_sem, out_sem, misc_sem):
    S, C, B = x_hbm.shape
    NT = B // NB
    NG = S // 4
    NGT = NT * NG
    N_IT = (NGT - K_PRO) // N_PER
    TS = S + 1
    KT = CM // 128 + 1
    CR = C - CM
    f32 = jnp.float32
    bf16 = jnp.bfloat16
    pk = lambda v: pltpu.bitcast(v, jnp.uint32)
    upk = lambda v: pltpu.bitcast(v, bf16)

    def in_copy(bt, lo, hi, sem):
        return pltpu.make_async_copy(x_hbm.at[lo:hi, :, bt * NB:(bt + 1) * NB],
                                     xall.at[bt * TS + 1 + lo:bt * TS + 1 + hi], sem)

    p_copies = [pltpu.make_async_copy(src, dst, misc_sem.at[KT + 3 + i])
                for i, (src, dst) in enumerate(((mean_hbm, pm), (var_hbm, pv), (g_hbm, pg), (b_hbm, pb)))]
    w_copies = [pltpu.make_async_copy(w_hbm.at[:, kt * 128:min(C, (kt + 1) * 128), :],
                                      wbuf.at[:, kt * 128:min(C, (kt + 1) * 128), :], misc_sem.at[kt])
                for kt in range(KT)]
    need0 = 4 * K_PRO + 5
    xa_copy = in_copy(0, 0, 5, misc_sem.at[KT])
    xb_copy = in_copy(0, 5, 9, misc_sem.at[KT + 1])
    xc_copy = in_copy(0, 9, need0 - 4, misc_sem.at[KT + 2])
    xd_copy = in_copy(0, need0 - 4, need0, misc_sem.at[KT + 7])
    for cp in p_copies + [xa_copy] + w_copies + [xb_copy, xc_copy, xd_copy]:
        cp.start()
    for it in range(N_IT):
        lo = need0 + 4 * N_PER * it
        hi = min(lo + 4 * N_PER, NT * S)
        while lo < hi:
            bt = lo // S
            e = min(hi, (bt + 1) * S)
            in_copy(bt, lo - bt * S, e - bt * S, in_sem.at[it]).start()
            lo = e
    n_full = 4 * N_PER
    n_last = NT * S - (need0 + 4 * N_PER * (N_IT - 1))

    for bt in range(NT + 1):
        xall[bt * TS] = jnp.zeros((C, NB), bf16)

    a, b = PA, PB
    a2, b2 = a * a, b * b
    k_rows = (C, CM + 128, CM + 128, CM + 128, CM + 128, CM)

    def split(gi):
        if isinstance(gi, int):
            return gi // NG, gi % NG
        return jax.lax.shift_right_logical(gi, 3), jnp.bitwise_and(gi, NG - 1)

    def lanes(bt):
        if isinstance(bt, int):
            return pl.ds(bt * NB, NB)
        return pl.ds(pl.multiple_of(bt * NB, NB), NB)

    def data_transform(d):
        a2d2 = a2 * d[2]
        t1 = d[4] - b2 * d[2]
        t3 = d[4] - a2d2
        t2 = a * d[3] - (a * b2) * d[1]
        t4 = b * d[3] - (b * a2) * d[1]
        u0 = t1 - a2d2 + d[0]
        u5 = d[1] - (a2 + b2) * d[3] + d[5]
        return [u0, t1 + t2, t1 - t2, t3 + t4, t3 - t4, u5]

    def transform(gi):
        bt, j = split(gi)
        base = bt * TS + 4 * j
        u = data_transform([xall[base + i].astype(f32) for i in range(6)])
        rhs = [u[0].astype(bf16)]
        for i in range(1, 5):
            ext = u[5][CM:C] + _PTS[i] * u[i][CM:C]
            rhs.append(jnp.concatenate([u[i], ext], axis=0).astype(bf16))
        rhs.append(u[5][0:CM].astype(bf16))
        return rhs

    def transform_to_scratch(gi, which):
        bt, j = split(gi)
        base = bt * TS + 4 * j
        for c0 in range(0, C, TCH):
            u = data_transform([xall[base + i, c0:c0 + TCH, :].astype(f32) for i in range(6)])
            for i in which:
                if i < 5 or c0 < CM:
                    u_scr[i, c0 // 2:(c0 + TCH) // 2, :] = pk(u[i].astype(bf16))
                if 1 <= i <= 4 and c0 >= CM:
                    u_scr[i, (c0 + CR) // 2:(c0 + CR + TCH) // 2, :] = pk((u[5] + _PTS[i] * u[i]).astype(bf16))

    def prod(i, rhs_i):
        nk = (k_rows[i] + 127) // 128
        lhs = jnp.concatenate([upk(wt_ref[i, kt]) for kt in range(nk)], axis=1)[:, :k_rows[i]]
        return jnp.dot(lhs, rhs_i, preferred_element_type=f32)

    def out_copy(gi, lo, hi):
        bt, j = split(gi)
        pltpu.make_async_copy(oall.at[pl.ds(4 * gi + lo, hi - lo)],
                              o_hbm.at[pl.ds(4 * j + lo, hi - lo), :, lanes(bt)], out_sem.at[0]).start()

    def epilogue(gi, m, mode):
        def epi(y, s):
            h = y * sc_ref[...] + sh_ref[...]
            oall[4 * gi + s] = (h * jnp.tanh(h) + h).astype(oall.dtype)

        p = m[1] + m[2]
        q = m[1] - m[2]
        r = m[3] + m[4]
        t = m[3] - m[4]
        epi(a * q + b * t, 1)
        epi(a2 * p + b2 * r, 2)
        epi((a * a2) * q + (b * b2) * t + m[5], 3)
        if mode == "split":
            out_copy(gi, 1, 4)
        epi(m[0] + p + r, 0)
        if mode != "defer":
            out_copy(gi, 0, 1 if mode == "split" else 4)

    def finish(gi, rhs, mode):
        epilogue(gi, [prod(i, rhs[i]) for i in range(6)], mode)

    def weight_prep(kt):
        for d0 in range(0, C, 128):
            dn = min(128, C - d0)
            rows = slice(d0 // 2, (d0 + dn) // 2)
            if kt < KT - 1:
                g0, g1, g2 = [wbuf[k, kt * 128:(kt + 1) * 128, d0:d0 + dn].T for k in range(3)]
                wt_ref[5, kt, rows, :] = pk(g2)
                g2 = g2.astype(f32)
            else:
                w0r = wbuf[0, CM:C, d0:d0 + dn]
                g0 = jnp.concatenate([w0r, jnp.zeros_like(w0r)], axis=0).T
                g1 = jnp.concatenate([wbuf[1, CM:C, d0:d0 + dn], wbuf[2, CM:C, d0:d0 + dn]], axis=0).T
                g2 = None
            wt_ref[0, kt, rows, :] = pk(g0)
            g0, g1 = g0.astype(f32), g1.astype(f32)
            for i in (1, 3):
                pt, den = _PTS[i], _den(i)
                ev = g0 * (1.0 / den)
                if g2 is not None:
                    ev = ev + g2 * (pt * pt / den)
                od = g1 * (pt / den)
                wt_ref[i, kt, rows, :] = pk((ev + od).astype(bf16))
                wt_ref[i + 1, kt, rows, :] = pk((ev - od).astype(bf16))

    def partial_prod(i, kt):
        n = min(128, k_rows[i] - kt * 128)
        return jnp.dot(upk(wt_ref[i, kt])[:, :n], upk(u_scr[i, kt * 64:kt * 64 + n // 2, :]),
                       preferred_element_type=f32)

    for cp in p_copies:
        cp.wait()
    row = lambda r: r[...].astype(f32).reshape(1, C)
    scale = row(pg) * jax.lax.rsqrt(row(pv) + 1e-5)
    shift = row(pb) - row(pm) * scale
    sc_ref[...] = jnp.broadcast_to(0.5 * scale, (NB, C)).T
    sh_ref[...] = jnp.broadcast_to(0.5 * shift, (NB, C)).T

    xa_copy.wait()
    transform_to_scratch(0, range(6))
    for kt in range(KT):
        w_copies[kt].wait()
        if kt == KT - 1:
            xb_copy.wait()
        weight_prep(kt)
        if 1 <= kt < KT - 1:
            for i in range(6):
                part = partial_prod(i, kt - 1)
                m_scr[i] = part if kt == 1 else m_scr[i] + part
    m = []
    for i in range(6):
        acc = m_scr[i] + partial_prod(i, KT - 2)
        if k_rows[i] > CM:
            acc = acc + partial_prod(i, KT - 1)
        m.append(acc)
    epilogue(0, m, "defer")

    finish(1, transform(1), "defer")
    xc_copy.wait()
    for gi in range(2, K_PRO):
        finish(gi, transform(gi), "defer")
    xd_copy.wait()
    transform_to_scratch(K_PRO, (1,))

    def body(it, carry):
        g0 = K_PRO + N_PER * it
        pltpu.make_async_copy(xall.at[0:n_last], xall.at[0:n_last], in_sem.at[it]).wait()

        @pl.when(it < N_IT - 1)
        def _():
            n = n_full - n_last
            pltpu.make_async_copy(xall.at[0:n], xall.at[0:n], in_sem.at[it]).wait()

        @pl.when(it == 0)
        def _():
            out_copy(0, 0, 4 * K_PRO)

        rhs = transform(g0)
        rhs[1] = upk(u_scr[1])
        finish(g0, rhs, "whole")
        for r in range(1, N_PER):
            finish(g0 + r, transform(g0 + r), "split" if r == N_PER - 1 else "whole")
        transform_to_scratch(jnp.minimum(g0 + N_PER, NGT - 1), (1,))
        return carry

    jax.lax.fori_loop(0, N_IT, body, 0)
    pltpu.make_async_copy(oall, oall, out_sem.at[0]).wait()


@jax.jit
def pallas_standalone__batchnorm__sampling_kernel(x, w, mean, var, g, b):
    B, S, C = x.shape
    NT = B // NB
    KT = CM // 128 + 1
    n_it = (NT * (S // 4) - K_PRO) // N_PER
    xt = jnp.transpose(x, (1, 2, 0))
    ot = pl.pallas_call(
        _kernel,
        in_specs=[pl.BlockSpec(memory_space=pl.ANY)] * 6,
        out_specs=pl.BlockSpec(memory_space=pl.ANY),
        out_shape=jax.ShapeDtypeStruct((S, C, B), x.dtype),
        scratch_shapes=[pltpu.VMEM((NT * (S + 1) + 1, C, NB), jnp.bfloat16),
                        pltpu.VMEM((NT * S, C, NB), jnp.bfloat16),
                        pltpu.VMEM((3, C, C), jnp.bfloat16),
                        pltpu.VMEM((C,), jnp.bfloat16),
                        pltpu.VMEM((C,), jnp.bfloat16),
                        pltpu.VMEM((C,), jnp.bfloat16),
                        pltpu.VMEM((C,), jnp.bfloat16),
                        pltpu.VMEM((6, KT, C // 2, 128), jnp.uint32),
                        pltpu.VMEM((C, NB), jnp.float32),
                        pltpu.VMEM((C, NB), jnp.float32),
                        pltpu.VMEM((6, KT * 64, NB), jnp.uint32),
                        pltpu.VMEM((6, C, NB), jnp.float32),
                        pltpu.SemaphoreType.DMA((n_it,)),
                        pltpu.SemaphoreType.DMA((1,)),
                        pltpu.SemaphoreType.DMA((KT + 8,))],
        compiler_params=pltpu.CompilerParams(vmem_limit_bytes=110 * 1024 * 1024,
                                             disable_bounds_checks=True),
    )(xt, w, mean, var, g, b)
    return jnp.transpose(ot, (2, 0, 1))
```

```python
import jax
import jax.numpy as jnp
import jax.experimental.pallas as pl
import jax.experimental.pallas.tpu as pltpu

NB = 128
PA = 0.4375
PB = 1.0 / PA
CM = 512
M = 6
NP = M + 2
K_PRO = 4
N_PER = 5
TCH = 32
STASH = 1

_PTS = (0.0, PA, -PA, 1.0, -1.0, PB, -PB)


def _den(i):
    d = 1.0
    for j, q in enumerate(_PTS):
        if j != i:
            d *= (_PTS[i] - q)
    return d


def _kernel(x_hbm, w_hbm, mean_hbm, var_hbm, g_hbm, b_hbm, o_hbm,
            xall, oall, wbuf, pm, pv, pg, pb, wt_ref, sc_ref, sh_ref, u_scr, m_scr, c_scr, z_ref,
            in_sem, out_sem, misc_sem):
    S, C, B = x_hbm.shape
    NT = B // NB
    TS = S + 1
    NGT = NT * TS // M
    N_IT = (NGT - K_PRO) // N_PER
    KT = CM // 128 + 1
    CR = C - CM
    f32 = jnp.float32
    bf16 = jnp.bfloat16
    pk = lambda v: pltpu.bitcast(v, jnp.uint32)
    upk = lambda v: pltpu.bitcast(v, bf16)

    def slot_ranges(lo, hi):
        out = []
        for bt in range(NT):
            a0, a1 = max(lo, bt * TS + 1), min(hi, (bt + 1) * TS)
            if a0 < a1:
                out.append((bt, a0 - bt * TS - 1, a1 - bt * TS - 1))
        return out

    def in_copies(lo, hi, sem):
        return [pltpu.make_async_copy(x_hbm.at[s0:s1, :, bt * NB:(bt + 1) * NB],
                                      xall.at[bt * TS + 1 + s0:bt * TS + 1 + s1], sem)
                for bt, s0, s1 in slot_ranges(lo, hi)]

    p_copies = [pltpu.make_async_copy(src, dst, misc_sem.at[KT + 4 + i])
                for i, (src, dst) in enumerate(((mean_hbm, pm), (var_hbm, pv), (g_hbm, pg), (b_hbm, pb)))]
    w_copies = [pltpu.make_async_copy(w_hbm.at[:, kt * 128:min(C, (kt + 1) * 128), :],
                                      wbuf.at[:, kt * 128:min(C, (kt + 1) * 128), :], misc_sem.at[kt])
                for kt in range(KT)]
    need = lambda g: M * (g + 1) + 1
    (xa_copy,) = in_copies(0, need(0), misc_sem.at[KT])
    (xb_copy,) = in_copies(need(0), need(1), misc_sem.at[KT + 1])
    (xc_copy,) = in_copies(need(1), need(K_PRO - 1), misc_sem.at[KT + 2])
    (xd_copy,) = in_copies(need(K_PRO - 1), need(K_PRO), misc_sem.at[KT + 3])
    for cp in p_copies + [xa_copy] + w_copies + [xb_copy, xc_copy, xd_copy]:
        cp.start()
    counts = []
    for it in range(N_IT):
        lo, hi = need(K_PRO + N_PER * it), need(K_PRO + N_PER * (it + 1))
        for cp in in_copies(lo, hi, in_sem.at[it]):
            cp.start()
        counts.append(sum(s1 - s0 for _, s0, s1 in slot_ranges(lo, hi)))
    n_min = min(counts)

    for bt in range(NT + 1):
        xall[bt * TS] = jnp.zeros((C, NB), bf16)

    for i in range(4):
        z_ref[i] = 0
    a, b = PA, PB
    a2, b2 = a * a, b * b
    ee = a2 + 1.0 + b2
    kap = 2.0 - a2 - b2
    k_rows = (C,) + (CM + 128,) * M + (CM,)

    def pair(d, i):
        p = _PTS[i]
        if p == 1.0:
            ev = d[0] + d[2] + d[4]
            od = d[1] + d[3] + d[5]
        else:
            ev = d[0] + (p ** 2) * d[2] + (p ** 4) * d[4]
            od = p * d[1] + (p ** 3) * d[3] + (p ** 5) * d[5]
        return ev + od, ev - od

    def ext_rows(i, u_i, d_prev, d_last):
        p = _PTS[i]
        if p == 1.0:
            return d_prev + u_i - d_last
        if p == -1.0:
            return d_prev - u_i - d_last
        return d_prev + p * u_i - (p ** M) * d_last

    def transform(gi):
        base = M * gi
        rhs = [xall[base + 1]]
        for i in range(1, M, 2):
            bz = base + z_ref[i // 2]
            d = [xall[bz + 1 + k].astype(f32) for k in range(M)]
            d_prev = xall[bz, CM:C, :].astype(f32)
            for k, u in enumerate(pair(d, i)):
                ext = ext_rows(i + k, u[CM:C], d_prev, d[M - 1][CM:C])
                rhs.append(jnp.concatenate([u, ext], axis=0).astype(bf16))
        rhs.append(xall[base + M, 0:CM, :])
        return rhs

    def transform_to_scratch(gi, which):
        base = M * gi
        for c0 in range(0, C, TCH):
            d = [xall[base + 1 + i, c0:c0 + TCH, :].astype(f32) for i in range(M)]
            for i in range(1, M, 2):
                for k, u in enumerate(pair(d, i)):
                    if i + k in which:
                        u_scr[i + k, c0 // 2:(c0 + TCH) // 2, :] = pk(u.astype(bf16))
                        if c0 >= CM:
                            d_prev = xall[base, c0:c0 + TCH, :].astype(f32)
                            ext = ext_rows(i + k, u, d_prev, d[M - 1])
                            u_scr[i + k, (c0 + CR) // 2:(c0 + CR + TCH) // 2, :] = pk(ext.astype(bf16))

    def prod(i, rhs_i):
        nk = (k_rows[i] + 127) // 128
        lhs = jnp.concatenate([upk(wt_ref[i, kt]) for kt in range(nk)], axis=1)[:, :k_rows[i]]
        return jnp.dot(lhs, rhs_i, preferred_element_type=f32)

    def out_copy_static(lo, hi):
        for bt, s0, s1 in slot_ranges(lo, hi):
            pltpu.make_async_copy(oall.at[bt * TS + 1 + s0:bt * TS + 1 + s1],
                                  o_hbm.at[s0:s1, :, bt * NB:(bt + 1) * NB], out_sem.at[0]).start()

    def out_copy_slot(slot):
        bt = jax.lax.shift_right_logical(slot * 1986, 16)
        s1 = slot - bt * TS

        @pl.when(s1 > 0)
        def _():
            pltpu.make_async_copy(oall.at[pl.ds(slot, 1)],
                                  o_hbm.at[pl.ds(s1 - 1, 1), :, pl.ds(pl.multiple_of(bt * NB, NB), NB)],
                                  out_sem.at[0]).start()

    def epilogue(gi, m, carry, copy_out):
        def epi(y, k):
            h = y * sc_ref[...] + sh_ref[...]
            oall[M * gi + k] = (h * jnp.tanh(h) + h).astype(oall.dtype)

        sa, ta = m[1] + m[2], m[1] - m[2]
        s1, t1 = m[3] + m[4], m[3] - m[4]
        sb, tb = m[5] + m[6], m[5] - m[6]
        o6 = sa + s1 + sb - m[0]
        o2 = b2 * sa + s1 + a2 * sb - ee * m[0]
        o4 = kap * s1 - m[0] - o2 - o6
        o5 = a * ta + t1 + b * tb - ee * m[7]
        o1 = b * ta + t1 + a * tb - m[7]
        o3 = kap * t1 - m[7] - o1 - o5
        if carry is None:
            epi(o1, 1)
        else:
            epi(m[0] + carry[0], 0)
            epi(o1 + carry[1], 1)
        epi(o2, 2)
        epi(o3, 3)
        epi(o4, 4)
        epi(o5, 5)
        if copy_out:
            for k in range(M):
                out_copy_slot(M * gi + k)
        return o6, m[7]

    def finish(gi, rhs, carry, copy_out):
        return epilogue(gi, [prod(i, rhs[i]) for i in range(NP)], carry, copy_out)

    def weight_prep(kt):
        for d0 in range(0, C, 128):
            dn = min(128, C - d0)
            rows = slice(d0 // 2, (d0 + dn) // 2)
            if kt < KT - 1:
                g0, g1, g2 = [wbuf[2 - k, kt * 128:(kt + 1) * 128, d0:d0 + dn].T for k in range(3)]
                wt_ref[NP - 1, kt, rows, :] = pk(g2)
                g2 = g2.astype(f32)
            else:
                w0r = wbuf[2, CM:C, d0:d0 + dn]
                g0 = jnp.concatenate([w0r, jnp.zeros_like(w0r)], axis=0).T
                g1 = jnp.concatenate([wbuf[1, CM:C, d0:d0 + dn], wbuf[0, CM:C, d0:d0 + dn]], axis=0).T
                g2 = None
            wt_ref[0, kt, rows, :] = pk(g0)
            g0, g1 = g0.astype(f32), g1.astype(f32)
            for i in range(1, M, 2):
                pt, den = _PTS[i], _den(i)
                ev = g0 * (1.0 / den)
                if g2 is not None:
                    ev = ev + g2 * (pt * pt / den)
                od = g1 * (pt / den)
                wt_ref[i, kt, rows, :] = pk((ev + od).astype(bf16))
                wt_ref[i + 1, kt, rows, :] = pk((ev - od).astype(bf16))

    def partial_prod(i, kt):
        n = min(128, k_rows[i] - kt * 128)
        if i == 0:
            rhs = xall[1, kt * 128:kt * 128 + n, :]
        elif i == NP - 1:
            rhs = xall[M, kt * 128:kt * 128 + n, :]
        else:
            rhs = upk(u_scr[i, kt * 64:kt * 64 + n // 2, :])
        return jnp.dot(upk(wt_ref[i, kt])[:, :n], rhs, preferred_element_type=f32)

    for cp in p_copies:
        cp.wait()
    row = lambda r: r[...].astype(f32).reshape(1, C)
    scale = row(pg) * jax.lax.rsqrt(row(pv) + 1e-5)
    shift = row(pb) - row(pm) * scale
    sc_ref[...] = jnp.broadcast_to(0.5 * scale, (NB, C)).T
    sh_ref[...] = jnp.broadcast_to(0.5 * shift, (NB, C)).T

    xa_copy.wait()
    transform_to_scratch(0, range(1, M + 1))
    for kt in range(KT):
        w_copies[kt].wait()
        if kt == KT - 1:
            xb_copy.wait()
        weight_prep(kt)
        if 1 <= kt < KT - 1:
            for i in range(NP):
                part = partial_prod(i, kt - 1)
                m_scr[i] = part if kt == 1 else m_scr[i] + part
    m = []
    for i in range(NP):
        acc = m_scr[i] + partial_prod(i, KT - 2)
        if k_rows[i] > CM:
            acc = acc + partial_prod(i, KT - 1)
        m.append(acc)
    carry = epilogue(0, m, None, False)
    carry = finish(1, transform(1), carry, False)
    xc_copy.wait()
    for gi in range(2, K_PRO):
        carry = finish(gi, transform(gi), carry, False)
    c_scr[0] = carry[0]
    c_scr[1] = carry[1]
    xd_copy.wait()
    transform_to_scratch(K_PRO, (STASH,))

    def body(it, c):
        g0 = K_PRO + N_PER * it
        pltpu.make_async_copy(xall.at[0:n_min], xall.at[0:n_min], in_sem.at[it]).wait()
        for n in sorted(set(counts)):
            if n > n_min:
                hit = None
                for k, cnt in enumerate(counts):
                    if cnt == n:
                        hit = (it == k) if hit is None else jnp.logical_or(hit, it == k)

                @pl.when(hit)
                def _():
                    pltpu.make_async_copy(xall.at[0:n - n_min], xall.at[0:n - n_min], in_sem.at[it]).wait()

        @pl.when(it == 0)
        def _():
            out_copy_static(0, M * K_PRO)

        rhs = transform(g0)
        rhs[STASH] = upk(u_scr[STASH])
        carry = finish(g0, rhs, (c_scr[0], c_scr[1]), True)
        for r in range(1, N_PER):
            carry = finish(g0 + r, transform(g0 + r), carry, True)
        c_scr[0] = carry[0]
        c_scr[1] = carry[1]
        transform_to_scratch(jnp.minimum(g0 + N_PER, NGT - 1), (STASH,))
        return c

    jax.lax.fori_loop(0, N_IT, body, 0)
    pltpu.make_async_copy(oall.at[0:NT * S], oall.at[0:NT * S], out_sem.at[0]).wait()


@jax.jit
def pallas_standalone__batchnorm__sampling_kernel(x, w, mean, var, g, b):
    B, S, C = x.shape
    NT = B // NB
    KT = CM // 128 + 1
    n_it = (NT * (S + 1) // M - K_PRO) // N_PER
    xt = jnp.transpose(x, (1, 2, 0))
    ot = pl.pallas_call(
        _kernel,
        in_specs=[pl.BlockSpec(memory_space=pl.ANY)] * 6,
        out_specs=pl.BlockSpec(memory_space=pl.ANY),
        out_shape=jax.ShapeDtypeStruct((S, C, B), x.dtype),
        scratch_shapes=[pltpu.VMEM((NT * (S + 1) + 1, C, NB), jnp.bfloat16),
                        pltpu.VMEM((NT * (S + 1), C, NB), jnp.bfloat16),
                        pltpu.VMEM((3, C, C), jnp.bfloat16),
                        pltpu.VMEM((C,), jnp.bfloat16),
                        pltpu.VMEM((C,), jnp.bfloat16),
                        pltpu.VMEM((C,), jnp.bfloat16),
                        pltpu.VMEM((C,), jnp.bfloat16),
                        pltpu.VMEM((NP, KT, C // 2, 128), jnp.uint32),
                        pltpu.VMEM((C, NB), jnp.float32),
                        pltpu.VMEM((C, NB), jnp.float32),
                        pltpu.VMEM((NP, KT * 64, NB), jnp.uint32),
                        pltpu.VMEM((NP, C, NB), jnp.float32),
                        pltpu.VMEM((2, C, NB), jnp.float32),
                        pltpu.SMEM((4,), jnp.int32),
                        pltpu.SemaphoreType.DMA((n_it,)),
                        pltpu.SemaphoreType.DMA((1,)),
                        pltpu.SemaphoreType.DMA((KT + 8,))],
        compiler_params=pltpu.CompilerParams(vmem_limit_bytes=110 * 1024 * 1024,
                                             disable_bounds_checks=True),
    )(xt, w, mean, var, g, b)
    return jnp.transpose(ot, (2, 0, 1))
```

```python
import jax
import jax.numpy as jnp
import jax.experimental.pallas as pl
import jax.experimental.pallas.tpu as pltpu

NB = 128
PA = 0.4375
PB = 1.0 / PA
CM = 512
M = 6
NP = M + 2
K_PRO = 4
N_PER = 5
TCH = 32
STASH = 1

_PTS = (0.0, PA, -PA, 1.0, -1.0, PB, -PB)


def _den(i):
    d = 1.0
    for j, q in enumerate(_PTS):
        if j != i:
            d *= (_PTS[i] - q)
    return d


def _kernel(x_hbm, w_hbm, mean_hbm, var_hbm, g_hbm, b_hbm, o_hbm,
            xall, oall, wbuf, pm, pv, pg, pb, wt_ref, sc_ref, sh_ref, sh3_ref, u_scr, m_scr, c_scr, z_ref,
            in_sem, out_sem, misc_sem):
    S, C, B = x_hbm.shape
    NT = B // NB
    TS = S + 1
    NGT = NT * TS // M
    N_IT = (NGT - K_PRO) // N_PER
    KT = CM // 128 + 1
    CR = C - CM
    f32 = jnp.float32
    bf16 = jnp.bfloat16
    pk = lambda v: pltpu.bitcast(v, jnp.uint32)
    upk = lambda v: pltpu.bitcast(v, bf16)

    def slot_ranges(lo, hi):
        out = []
        for bt in range(NT):
            a0, a1 = max(lo, bt * TS + 1), min(hi, (bt + 1) * TS)
            if a0 < a1:
                out.append((bt, a0 - bt * TS - 1, a1 - bt * TS - 1))
        return out

    def in_copies(lo, hi, sem):
        return [pltpu.make_async_copy(x_hbm.at[s0:s1, :, bt * NB:(bt + 1) * NB],
                                      xall.at[bt * TS + 1 + s0:bt * TS + 1 + s1], sem)
                for bt, s0, s1 in slot_ranges(lo, hi)]

    p_copies = [pltpu.make_async_copy(src, dst, misc_sem.at[KT + 4 + i])
                for i, (src, dst) in enumerate(((mean_hbm, pm), (var_hbm, pv), (g_hbm, pg), (b_hbm, pb)))]
    w_copies = [pltpu.make_async_copy(w_hbm.at[:, kt * 128:min(C, (kt + 1) * 128), :],
                                      wbuf.at[:, kt * 128:min(C, (kt + 1) * 128), :], misc_sem.at[kt])
                for kt in range(KT)]
    need = lambda g: M * (g + 1) + 1
    (xa_copy,) = in_copies(0, need(0), misc_sem.at[KT])
    (xb_copy,) = in_copies(need(0), need(1), misc_sem.at[KT + 1])
    (xc_copy,) = in_copies(need(1), need(K_PRO - 1), misc_sem.at[KT + 2])
    for cp in p_copies + [xa_copy] + w_copies + [xb_copy, xc_copy]:
        cp.start()
    counts = []
    for it in range(N_IT):
        lo, hi = need(K_PRO - 1 + N_PER * it), need(K_PRO - 1 + N_PER * (it + 1))
        for cp in in_copies(lo, hi, in_sem.at[it]):
            cp.start()
        counts.append(sum(s1 - s0 for _, s0, s1 in slot_ranges(lo, hi)))
    n_min = min(counts)

    for bt in range(NT + 1):
        xall[bt * TS] = jnp.zeros((C, NB), bf16)

    for i in range(4):
        z_ref[i] = 0
    a, b = PA, PB
    a2, b2 = a * a, b * b
    ee = a2 + 1.0 + b2
    kap = 2.0 - a2 - b2
    k_rows = (C,) + (CM + 128,) * M + (CM,)

    def pair(d, i):
        p = _PTS[i]
        if p == 1.0:
            ev = d[0] + d[2] + d[4]
            od = d[1] + d[3] + d[5]
        else:
            ev = d[0] + (p ** 2) * d[2] + (p ** 4) * d[4]
            od = p * d[1] + (p ** 3) * d[3] + (p ** 5) * d[5]
        return ev + od, ev - od

    def ext_rows(i, u_i, d_prev, d_last):
        p = _PTS[i]
        if p == 1.0:
            return d_prev + u_i - d_last
        if p == -1.0:
            return d_prev - u_i - d_last
        return d_prev + p * u_i - (p ** M) * d_last

    def transform(gi):
        base = M * gi
        rhs = [xall[base + 1]]
        for i in range(1, M, 2):
            bz = base + z_ref[i // 2]
            d = [xall[bz + 1 + k].astype(f32) for k in range(M)]
            d_prev = xall[bz, CM:C, :].astype(f32)
            for k, u in enumerate(pair(d, i)):
                ext = ext_rows(i + k, u[CM:C], d_prev, d[M - 1][CM:C])
                rhs.append(jnp.concatenate([u, ext], axis=0).astype(bf16))
        rhs.append(xall[base + M, 0:CM, :])
        return rhs

    def transform_to_scratch(gi, which):
        base = M * gi
        for c0 in range(0, C, TCH):
            d = [xall[base + 1 + i, c0:c0 + TCH, :].astype(f32) for i in range(M)]
            for i in range(1, M, 2):
                for k, u in enumerate(pair(d, i)):
                    if i + k in which:
                        u_scr[i + k, c0 // 2:(c0 + TCH) // 2, :] = pk(u.astype(bf16))
                        if c0 >= CM:
                            d_prev = xall[base, c0:c0 + TCH, :].astype(f32)
                            ext = ext_rows(i + k, u, d_prev, d[M - 1])
                            u_scr[i + k, (c0 + CR) // 2:(c0 + CR + TCH) // 2, :] = pk(ext.astype(bf16))

    def prod(i, rhs_i):
        nk = (k_rows[i] + 127) // 128
        lhs = jnp.concatenate([upk(wt_ref[i, kt]) for kt in range(nk)], axis=1)[:, :k_rows[i]]
        return jnp.dot(lhs, rhs_i, preferred_element_type=f32)

    def out_copy_static(lo, hi):
        for bt, s0, s1 in slot_ranges(lo, hi):
            pltpu.make_async_copy(oall.at[bt * TS + 1 + s0:bt * TS + 1 + s1],
                                  o_hbm.at[s0:s1, :, bt * NB:(bt + 1) * NB], out_sem.at[0]).start()

    def out_copy_slot(slot):
        bt = jax.lax.shift_right_logical(slot * 1986, 16)
        s1 = slot - bt * TS

        @pl.when(s1 > 0)
        def _():
            pltpu.make_async_copy(oall.at[pl.ds(slot, 1)],
                                  o_hbm.at[pl.ds(s1 - 1, 1), :, pl.ds(pl.multiple_of(bt * NB, NB), NB)],
                                  out_sem.at[0]).start()

    def epilogue(gi, m, carry, copy_out):
        def epi(h, k):
            oall[M * gi + k] = (h * jnp.tanh(h) + h).astype(oall.dtype)

        sh = sh_ref[...]
        m0 = m[0] * sc_ref[...]
        em0 = ee * m0
        sa, ta = m[1] + m[2], m[1] - m[2]
        s1s, t1s = (m[3] + m[4]) + sh, (m[3] - m[4]) + sh
        sb, tb = m[5] + m[6], m[5] - m[6]
        o6 = ((s1s - m0) + sa) + sb
        o2 = ((s1s - em0) + b2 * sa) + a2 * sb
        o4 = ((sh3_ref[...] - m0) + kap * s1s) - o2 - o6
        q5 = (a * ta + t1s) + b * tb
        q1 = (b * ta + t1s) + a * tb
        q3 = (kap * t1s + sh3_ref[...]) - q1 - q5
        if carry is not None:
            q1 = q1 + carry[1]
        m7 = m[7] * sc_ref[...]
        em7 = ee * m7
        if carry is not None:
            epi(m0 + carry[0], 0)
        epi(o2, 2)
        epi(o4, 4)
        epi(q1 - m7, 1)
        epi(q3 + em7, 3)
        epi(q5 - em7, 5)
        if copy_out:
            for k in range(M):
                out_copy_slot(M * gi + k)
        return o6, m7

    def finish(gi, rhs, carry, copy_out):
        return epilogue(gi, [prod(i, rhs[i]) for i in range(NP)], carry, copy_out)

    def weight_prep(kt):
        for d0 in range(0, C, 128):
            dn = min(128, C - d0)
            rows = slice(d0 // 2, (d0 + dn) // 2)
            if kt < KT - 1:
                g0, g1, g2 = [wbuf[2 - k, kt * 128:(kt + 1) * 128, d0:d0 + dn].T for k in range(3)]
                wt_ref[NP - 1, kt, rows, :] = pk(g2)
                g2 = g2.astype(f32)
            else:
                w0r = wbuf[2, CM:C, d0:d0 + dn]
                g0 = jnp.concatenate([w0r, jnp.zeros_like(w0r)], axis=0).T
                g1 = jnp.concatenate([wbuf[1, CM:C, d0:d0 + dn], wbuf[0, CM:C, d0:d0 + dn]], axis=0).T
                g2 = None
            wt_ref[0, kt, rows, :] = pk(g0)
            scl = sc_ref[d0:d0 + dn, :]
            g0, g1 = g0.astype(f32) * scl, g1.astype(f32) * scl
            if g2 is not None:
                g2 = g2 * scl
            for i in range(1, M, 2):
                pt, den = _PTS[i], _den(i)
                ev = g0 * (1.0 / den)
                if g2 is not None:
                    ev = ev + g2 * (pt * pt / den)
                od = g1 * (pt / den)
                wt_ref[i, kt, rows, :] = pk((ev + od).astype(bf16))
                wt_ref[i + 1, kt, rows, :] = pk((ev - od).astype(bf16))

    def partial_prod(i, kt):
        n = min(128, k_rows[i] - kt * 128)
        if i == 0:
            rhs = xall[1, kt * 128:kt * 128 + n, :]
        elif i == NP - 1:
            rhs = xall[M, kt * 128:kt * 128 + n, :]
        else:
            rhs = upk(u_scr[i, kt * 64:kt * 64 + n // 2, :])
        return jnp.dot(upk(wt_ref[i, kt])[:, :n], rhs, preferred_element_type=f32)

    for cp in p_copies:
        cp.wait()
    row = lambda r: r[...].astype(f32).reshape(1, C)
    scale = row(pg) * jax.lax.rsqrt(row(pv) + 1e-5)
    shift = row(pb) - row(pm) * scale
    sc_ref[...] = jnp.broadcast_to(0.5 * scale, (NB, C)).T
    sh_t = jnp.broadcast_to(0.5 * shift, (NB, C)).T
    sh_ref[...] = sh_t
    sh3_ref[...] = (3.0 - kap) * sh_t

    xa_copy.wait()
    transform_to_scratch(0, range(1, M + 1))
    for kt in range(KT):
        w_copies[kt].wait()
        if kt == KT - 1:
            xb_copy.wait()
        weight_prep(kt)
        if 1 <= kt < KT - 1:
            for i in range(NP):
                part = partial_prod(i, kt - 1)
                m_scr[i] = part if kt == 1 else m_scr[i] + part
    m = []
    for i in range(NP):
        acc = m_scr[i] + partial_prod(i, KT - 2)
        if k_rows[i] > CM:
            acc = acc + partial_prod(i, KT - 1)
        m.append(acc)
    carry = epilogue(0, m, None, False)
    carry = finish(1, transform(1), carry, False)
    xc_copy.wait()
    for gi in range(2, K_PRO):
        carry = finish(gi, transform(gi), carry, False)
    c_scr[0] = carry[0]
    c_scr[1] = carry[1]

    def body(it, c):
        g0 = K_PRO + N_PER * it
        pltpu.make_async_copy(xall.at[0:n_min], xall.at[0:n_min], in_sem.at[it]).wait()
        for n in sorted(set(counts)):
            if n > n_min:
                hit = None
                for k, cnt in enumerate(counts):
                    if cnt == n:
                        hit = (it == k) if hit is None else jnp.logical_or(hit, it == k)

                @pl.when(hit)
                def _():
                    pltpu.make_async_copy(xall.at[0:n - n_min], xall.at[0:n - n_min], in_sem.at[it]).wait()

        @pl.when(it == 0)
        def _():
            out_copy_static(0, M * K_PRO)

        carry = (c_scr[0], c_scr[1])
        for r in range(N_PER):
            carry = finish(g0 + r, transform(g0 + r), carry, True)
        c_scr[0] = carry[0]
        c_scr[1] = carry[1]
        return c

    jax.lax.fori_loop(0, N_IT, body, 0)
    pltpu.make_async_copy(oall.at[0:NT * S], oall.at[0:NT * S], out_sem.at[0]).wait()


@jax.jit
def pallas_standalone__batchnorm__sampling_kernel(x, w, mean, var, g, b):
    B, S, C = x.shape
    NT = B // NB
    KT = CM // 128 + 1
    n_it = (NT * (S + 1) // M - K_PRO) // N_PER
    xt = jnp.transpose(x, (1, 2, 0))
    ot = pl.pallas_call(
        _kernel,
        in_specs=[pl.BlockSpec(memory_space=pl.ANY)] * 6,
        out_specs=pl.BlockSpec(memory_space=pl.ANY),
        out_shape=jax.ShapeDtypeStruct((S, C, B), x.dtype),
        scratch_shapes=[pltpu.VMEM((NT * (S + 1) + 1, C, NB), jnp.bfloat16),
                        pltpu.VMEM((NT * (S + 1), C, NB), jnp.bfloat16),
                        pltpu.VMEM((3, C, C), jnp.bfloat16),
                        pltpu.VMEM((C,), jnp.bfloat16),
                        pltpu.VMEM((C,), jnp.bfloat16),
                        pltpu.VMEM((C,), jnp.bfloat16),
                        pltpu.VMEM((C,), jnp.bfloat16),
                        pltpu.VMEM((NP, KT, C // 2, 128), jnp.uint32),
                        pltpu.VMEM((C, NB), jnp.float32),
                        pltpu.VMEM((C, NB), jnp.float32),
                        pltpu.VMEM((C, NB), jnp.float32),
                        pltpu.VMEM((NP, KT * 64, NB), jnp.uint32),
                        pltpu.VMEM((NP, C, NB), jnp.float32),
                        pltpu.VMEM((2, C, NB), jnp.float32),
                        pltpu.SMEM((4,), jnp.int32),
                        pltpu.SemaphoreType.DMA((n_it,)),
                        pltpu.SemaphoreType.DMA((1,)),
                        pltpu.SemaphoreType.DMA((KT + 8,))],
        compiler_params=pltpu.CompilerParams(vmem_limit_bytes=110 * 1024 * 1024,
                                             disable_bounds_checks=True),
    )(xt, w, mean, var, g, b)
    return jnp.transpose(ot, (2, 0, 1))
```

```python
import jax
import jax.numpy as jnp
import jax.experimental.pallas as pl
import jax.experimental.pallas.tpu as pltpu

NB = 128
PA = 0.4375
PB = 1.0 / PA
CM = 512
M = 6
NP = M + 2
K_PRO = 4
N_PER = 5
TCH = 32
EARLY = (0, 3, 4, 1)
FINE_ROWS = ((0, 320), (320, 576))

_PTS = (0.0, PA, -PA, 1.0, -1.0, PB, -PB)


def _den(i):
    d = 1.0
    for j, q in enumerate(_PTS):
        if j != i:
            d *= (_PTS[i] - q)
    return d


def _kernel(x_hbm, w_hbm, mean_hbm, var_hbm, g_hbm, b_hbm, o_hbm,
            xall, oall, wbuf, pm, pv, pg, pb, wt_ref, sc_ref, sh_ref, sh3_ref, u_scr, m_scr, c_scr, z_ref,
            in_sem, out_sem, misc_sem):
    S, C, B = x_hbm.shape
    NT = B // NB
    TS = S + 1
    NGT = NT * TS // M
    N_IT = (NGT - K_PRO) // N_PER
    KT = CM // 128 + 1
    CR = C - CM
    f32 = jnp.float32
    bf16 = jnp.bfloat16
    pk = lambda v: pltpu.bitcast(v, jnp.uint32)
    upk = lambda v: pltpu.bitcast(v, bf16)

    wt16, u16 = wt_ref, u_scr
    wt_ref = wt16.bitcast(jnp.uint32)
    u_scr = u16.bitcast(jnp.uint32)

    def slot_ranges(lo, hi):
        out = []
        for bt in range(NT):
            a0, a1 = max(lo, bt * TS + 1), min(hi, (bt + 1) * TS)
            if a0 < a1:
                out.append((bt, a0 - bt * TS - 1, a1 - bt * TS - 1))
        return out

    def in_copies(lo, hi, sem):
        return [pltpu.make_async_copy(x_hbm.at[s0:s1, :, bt * NB:(bt + 1) * NB],
                                      xall.at[bt * TS + 1 + s0:bt * TS + 1 + s1], sem)
                for bt, s0, s1 in slot_ranges(lo, hi)]

    p_copies = [pltpu.make_async_copy(src, dst, misc_sem.at[KT + 4 + i])
                for i, (src, dst) in enumerate(((mean_hbm, pm), (var_hbm, pv), (g_hbm, pg), (b_hbm, pb)))]
    w_copies = [pltpu.make_async_copy(w_hbm.at[:, kt * 128:min(C, (kt + 1) * 128), :],
                                      wbuf.at[:, kt * 128:min(C, (kt + 1) * 128), :], misc_sem.at[kt])
                for kt in range(KT)]
    need = lambda g: M * (g + 1) + 1
    (xa_copy,) = in_copies(0, need(0), misc_sem.at[KT])
    (xb_copy,) = in_copies(need(0), need(1), misc_sem.at[KT + 1])
    (xc_copy,) = in_copies(need(1), need(K_PRO - 1), misc_sem.at[KT + 2])
    for cp in p_copies + [xa_copy] + w_copies + [xb_copy, xc_copy]:
        cp.start()
    counts = []
    for it in range(N_IT):
        lo, hi = need(K_PRO - 1 + N_PER * it), need(K_PRO - 1 + N_PER * (it + 1))
        for cp in in_copies(lo, hi, in_sem.at[it]):
            cp.start()
        counts.append(sum(s1 - s0 for _, s0, s1 in slot_ranges(lo, hi)))
    n_min = min(counts)

    for bt in range(NT + 1):
        xall[bt * TS] = jnp.zeros((C, NB), bf16)

    for i in range(4):
        z_ref[i] = 0
    a, b = PA, PB
    a2, b2 = a * a, b * b
    ee = a2 + 1.0 + b2
    kap = 2.0 - a2 - b2
    k_rows = (C,) + (CM + 128,) * M + (CM,)

    def pair(d, i):
        p = _PTS[i]
        if p == 1.0:
            ev = d[0] + d[2] + d[4]
            od = d[1] + d[3] + d[5]
        else:
            ev = d[0] + (p ** 2) * d[2] + (p ** 4) * d[4]
            od = p * d[1] + (p ** 3) * d[3] + (p ** 5) * d[5]
        return ev + od, ev - od

    def ext_rows(i, u_i, d_prev, d_last):
        p = _PTS[i]
        if p == 1.0:
            return d_prev + u_i - d_last
        if p == -1.0:
            return d_prev - u_i - d_last
        return d_prev + p * u_i - (p ** M) * d_last

    def transform(gi):
        base = M * gi
        rhs = [xall[base + 1]]
        for i in range(1, M, 2):
            bz = base + z_ref[i // 2]
            d = [xall[bz + 1 + k].astype(f32) for k in range(M)]
            d_prev = xall[bz, CM:C, :].astype(f32)
            for k, u in enumerate(pair(d, i)):
                ext = ext_rows(i + k, u[CM:C], d_prev, d[M - 1][CM:C])
                rhs.append(jnp.concatenate([u, ext], axis=0).astype(bf16))
        rhs.append(xall[base + M, 0:CM, :])
        return rhs

    def transform_to_scratch(gi, which):
        base = M * gi
        for c0 in range(0, C, TCH):
            d = [xall[base + 1 + i, c0:c0 + TCH, :].astype(f32) for i in range(M)]
            for i in range(1, M, 2):
                for k, u in enumerate(pair(d, i)):
                    if i + k in which:
                        u16[i + k, c0:c0 + TCH, :] = u.astype(bf16)
                        if c0 >= CM:
                            d_prev = xall[base, c0:c0 + TCH, :].astype(f32)
                            ext = ext_rows(i + k, u, d_prev, d[M - 1])
                            u16[i + k, c0 + CR:c0 + CR + TCH, :] = ext.astype(bf16)

    def prod(i, rhs_i):
        nk = (k_rows[i] + 127) // 128
        lhs = jnp.concatenate([upk(wt_ref[i, kt]) for kt in range(nk)], axis=1)[:, :k_rows[i]]
        return jnp.dot(lhs, rhs_i, preferred_element_type=f32)

    def out_copy_static(lo, hi):
        for bt, s0, s1 in slot_ranges(lo, hi):
            pltpu.make_async_copy(oall.at[bt * TS + 1 + s0:bt * TS + 1 + s1],
                                  o_hbm.at[s0:s1, :, bt * NB:(bt + 1) * NB], out_sem.at[0]).start()

    def out_copy_slot(slot, r0=0, r1=None):
        r1 = C if r1 is None else r1
        bt = jax.lax.shift_right_logical(slot * 1986, 16)
        s1 = slot - bt * TS

        @pl.when(s1 > 0)
        def _():
            pltpu.make_async_copy(oall.at[pl.ds(slot, 1), r0:r1],
                                  o_hbm.at[pl.ds(s1 - 1, 1), r0:r1, pl.ds(pl.multiple_of(bt * NB, NB), NB)],
                                  out_sem.at[0]).start()

    def epilogue(gi, m, carry, copy_out):
        def epi(h, k, r0=0, r1=C):
            h = h[r0:r1]
            oall[M * gi + k, r0:r1, :] = (h * jnp.tanh(h) + h).astype(oall.dtype)

        sh = sh_ref[...]
        m0 = m[0] * sc_ref[...]
        em0 = ee * m0
        sa, ta = m[1] + m[2], m[1] - m[2]
        s1s, t1s = (m[3] + m[4]) + sh, (m[3] - m[4]) + sh
        sb, tb = m[5] + m[6], m[5] - m[6]
        o6 = ((s1s - m0) + sa) + sb
        o2 = ((s1s - em0) + b2 * sa) + a2 * sb
        o4 = ((sh3_ref[...] - m0) + kap * s1s) - o2 - o6
        q5 = (a * ta + t1s) + b * tb
        q1 = (b * ta + t1s) + a * tb
        q3 = (kap * t1s + sh3_ref[...]) - q1 - q5
        if carry is not None:
            q1 = q1 + carry[1]
        m7 = m[7] * sc_ref[...]
        em7 = ee * m7
        if carry is not None:
            epi(m0 + carry[0], 0)
        epi(o2, 2)
        epi(o4, 4)
        odd = ((q1 - m7, 1), (q3 + em7, 3), (q5 - em7, 5))
        if copy_out == "fine":
            for k in (0, 2, 4):
                out_copy_slot(M * gi + k)
            for r0, r1 in FINE_ROWS:
                for h, k in odd:
                    epi(h, k, r0, r1)
                for h, k in odd:
                    out_copy_slot(M * gi + k, r0, r1)
        else:
            for h, k in odd:
                epi(h, k)
            if copy_out:
                for k in range(M):
                    out_copy_slot(M * gi + k)
        return o6, m7

    def finish(gi, rhs, carry, copy_out):
        return epilogue(gi, [prod(i, rhs[i]) for i in range(NP)], carry, copy_out)

    def weight_prep(kt):
        for d0 in range(0, C, 128):
            dn = min(128, C - d0)
            rows = slice(d0 // 2, (d0 + dn) // 2)
            if kt < KT - 1:
                g0, g1, g2 = [wbuf[2 - k, kt * 128:(kt + 1) * 128, d0:d0 + dn].T for k in range(3)]
                wt16[NP - 1, kt, d0:d0 + dn, :] = g2
                g2 = g2.astype(f32)
            else:
                w0r = wbuf[2, CM:C, d0:d0 + dn]
                g0 = jnp.concatenate([w0r, jnp.zeros_like(w0r)], axis=0).T
                g1 = jnp.concatenate([wbuf[1, CM:C, d0:d0 + dn], wbuf[0, CM:C, d0:d0 + dn]], axis=0).T
                g2 = None
            wt16[0, kt, d0:d0 + dn, :] = g0
            scl = sc_ref[d0:d0 + dn, :]
            g0, g1 = g0.astype(f32) * scl, g1.astype(f32) * scl
            if g2 is not None:
                g2 = g2 * scl
            for i in range(1, M, 2):
                pt, den = _PTS[i], _den(i)
                ev = g0 * (1.0 / den)
                if g2 is not None:
                    ev = ev + g2 * (pt * pt / den)
                od = g1 * (pt / den)
                wt16[i, kt, d0:d0 + dn, :] = (ev + od).astype(bf16)
                wt16[i + 1, kt, d0:d0 + dn, :] = (ev - od).astype(bf16)

    def partial_prod(i, kt0, kt1, rhs=None):
        hi = min(kt1 * 128, k_rows[i])
        nk = (hi + 127) // 128
        lhs = jnp.concatenate([upk(wt_ref[i, kt]) for kt in range(kt0, nk)], axis=1)[:, :hi - kt0 * 128]
        if rhs is not None:
            rhs = rhs[kt0 * 128:hi]
        elif i == 0:
            rhs = xall[1, kt0 * 128:hi, :]
        elif i == NP - 1:
            rhs = xall[M, kt0 * 128:hi, :]
        else:
            rhs = upk(u_scr[i, kt0 * 64:hi // 2, :])
        return jnp.dot(lhs, rhs, preferred_element_type=f32)

    for cp in p_copies:
        cp.wait()
    row = lambda r: r[...].astype(f32).reshape(1, C)
    scale = row(pg) * jax.lax.rsqrt(row(pv) + 1e-5)
    shift = row(pb) - row(pm) * scale
    sc_ref[...] = jnp.broadcast_to(0.5 * scale, (NB, C)).T
    sh_t = jnp.broadcast_to(0.5 * shift, (NB, C)).T
    sh_ref[...] = sh_t
    sh3_ref[...] = (3.0 - kap) * sh_t

    xa_copy.wait()
    transform_to_scratch(0, range(1, M + 1))
    for kt in range(KT - 1):
        w_copies[kt].wait()
        if kt == KT - 2:
            w_copies[KT - 1].wait()
        weight_prep(kt)
        if kt == KT - 2:
            weight_prep(KT - 1)
        if kt >= 1:
            for i in range(NP):
                part = partial_prod(i, kt - 1, kt + 1 if (kt == KT - 2 and i in EARLY) else kt)
                m_scr[i] = part if kt == 1 else m_scr[i] + part
    xb_copy.wait()
    m = [m_scr[i] + partial_prod(i, KT - 1 if i in EARLY else KT - 2, KT) if (i not in EARLY or k_rows[i] > CM) else m_scr[i]
         for i in range(NP)]
    carry = epilogue(0, m, None, False)
    rhs = transform(1)
    m = [prod(i, rhs[i]) for i in range(NP - 1)]
    m_scr[0] = partial_prod(NP - 1, 0, 2, rhs[NP - 1])
    for i in range(NP - 1):
        m_scr[i + 1] = m[i]
    xc_copy.wait()
    m = [m_scr[i + 1] for i in range(NP - 1)]
    m.append(m_scr[0] + partial_prod(NP - 1, 2, KT - 1, xall[2 * M]))
    carry = epilogue(1, m, carry, False)
    for gi in range(2, K_PRO):
        carry = finish(gi, transform(gi), carry, False)
    c_scr[0] = carry[0]
    c_scr[1] = carry[1]

    def body(it, c):
        g0 = K_PRO + N_PER * it
        pltpu.make_async_copy(xall.at[0:n_min], xall.at[0:n_min], in_sem.at[it]).wait()
        for n in sorted(set(counts)):
            if n > n_min:
                hit = None
                for k, cnt in enumerate(counts):
                    if cnt == n:
                        hit = (it == k) if hit is None else jnp.logical_or(hit, it == k)

                @pl.when(hit)
                def _():
                    pltpu.make_async_copy(xall.at[0:n - n_min], xall.at[0:n - n_min], in_sem.at[it]).wait()

        @pl.when(it == 0)
        def _():
            out_copy_static(0, M * K_PRO)

        carry = (c_scr[0], c_scr[1])
        for r in range(N_PER):
            carry = finish(g0 + r, transform(g0 + r), carry, "fine" if r == N_PER - 1 else True)
        c_scr[0] = carry[0]
        c_scr[1] = carry[1]
        return c

    jax.lax.fori_loop(0, N_IT, body, 0)
    pltpu.make_async_copy(oall.at[0:NT * S], oall.at[0:NT * S], out_sem.at[0]).wait()


@jax.jit
def pallas_standalone__batchnorm__sampling_kernel(x, w, mean, var, g, b):
    B, S, C = x.shape
    NT = B // NB
    KT = CM // 128 + 1
    n_it = (NT * (S + 1) // M - K_PRO) // N_PER
    xt = jnp.transpose(x, (1, 2, 0))
    ot = pl.pallas_call(
        _kernel,
        in_specs=[pl.BlockSpec(memory_space=pl.ANY)] * 6,
        out_specs=pl.BlockSpec(memory_space=pl.ANY),
        out_shape=jax.ShapeDtypeStruct((S, C, B), x.dtype),
        scratch_shapes=[pltpu.VMEM((NT * (S + 1) + 1, C, NB), jnp.bfloat16),
                        pltpu.VMEM((NT * (S + 1), C, NB), jnp.bfloat16),
                        pltpu.VMEM((3, C, C), jnp.bfloat16),
                        pltpu.VMEM((C,), jnp.bfloat16),
                        pltpu.VMEM((C,), jnp.bfloat16),
                        pltpu.VMEM((C,), jnp.bfloat16),
                        pltpu.VMEM((C,), jnp.bfloat16),
                        pltpu.VMEM((NP, KT, C, 128), jnp.bfloat16),
                        pltpu.VMEM((C, NB), jnp.float32),
                        pltpu.VMEM((C, NB), jnp.float32),
                        pltpu.VMEM((C, NB), jnp.float32),
                        pltpu.VMEM((NP, KT * 128, NB), jnp.bfloat16),
                        pltpu.VMEM((NP, C, NB), jnp.float32),
                        pltpu.VMEM((2, C, NB), jnp.float32),
                        pltpu.SMEM((4,), jnp.int32),
                        pltpu.SemaphoreType.DMA((n_it,)),
                        pltpu.SemaphoreType.DMA((1,)),
                        pltpu.SemaphoreType.DMA((KT + 8,))],
        compiler_params=pltpu.CompilerParams(vmem_limit_bytes=110 * 1024 * 1024,
                                             disable_bounds_checks=True),
    )(xt, w, mean, var, g, b)
    return jnp.transpose(ot, (2, 0, 1))
```

```python
import jax
import jax.numpy as jnp
import jax.experimental.pallas as pl
import jax.experimental.pallas.tpu as pltpu

NB = 128
PA = 0.4375
PB = 1.0 / PA
CM = 512
M = 6
NP = M + 2
K_PRO = 4
N_PER = 5
TCH = 32
HALVES = ((0, 432), (432, 576))
G1_SPLIT = False
EARLY = (0, 3, 4, 1)
FINE_ROWS = ((0, 320), (320, 576))

_PTS = (0.0, PA, -PA, 1.0, -1.0, PB, -PB)


def _den(i):
    d = 1.0
    for j, q in enumerate(_PTS):
        if j != i:
            d *= (_PTS[i] - q)
    return d


def _kernel(x_hbm, w_hbm, mean_hbm, var_hbm, g_hbm, b_hbm, o_hbm,
            xall, oall, wbuf, pm, pv, pg, pb, wt_ref, sc_ref, sh_ref, sh3_ref, u_scr, m_scr, c_scr, z_ref,
            in_sem, out_sem, misc_sem):
    S, C, B = x_hbm.shape
    NT = B // NB
    TS = S + 1
    NGT = NT * TS // M
    N_IT = (NGT - K_PRO) // N_PER
    KT = CM // 128 + 1
    CR = C - CM
    f32 = jnp.float32
    bf16 = jnp.bfloat16
    pk = lambda v: pltpu.bitcast(v, jnp.uint32)
    upk = lambda v: pltpu.bitcast(v, bf16)

    wt16, u16 = wt_ref, u_scr
    wt_ref = wt16.bitcast(jnp.uint32)
    u_scr = u16.bitcast(jnp.uint32)

    def slot_ranges(lo, hi):
        out = []
        for bt in range(NT):
            a0, a1 = max(lo, bt * TS + 1), min(hi, (bt + 1) * TS)
            if a0 < a1:
                out.append((bt, a0 - bt * TS - 1, a1 - bt * TS - 1))
        return out

    def in_copies(lo, hi, sem):
        return [pltpu.make_async_copy(x_hbm.at[s0:s1, :, bt * NB:(bt + 1) * NB],
                                      xall.at[bt * TS + 1 + s0:bt * TS + 1 + s1], sem)
                for bt, s0, s1 in slot_ranges(lo, hi)]

    p_copies = [pltpu.make_async_copy(src, dst, misc_sem.at[KT + 4 + i])
                for i, (src, dst) in enumerate(((mean_hbm, pm), (var_hbm, pv), (g_hbm, pg), (b_hbm, pb)))]
    w_copies = [pltpu.make_async_copy(w_hbm.at[:, kt * 128:min(C, (kt + 1) * 128), :],
                                      wbuf.at[:, kt * 128:min(C, (kt + 1) * 128), :], misc_sem.at[kt])
                for kt in range(KT)]
    need = lambda g: M * (g + 1) + 1
    (xa_copy,) = in_copies(0, need(0), misc_sem.at[KT])
    (xb_copy,) = in_copies(need(0), need(1), misc_sem.at[KT + 1])
    (xc_copy,) = in_copies(need(1), need(K_PRO - 1), misc_sem.at[KT + 2])
    for cp in p_copies + [xa_copy] + w_copies + [xb_copy, xc_copy]:
        cp.start()
    counts = []
    for it in range(N_IT):
        lo, hi = need(K_PRO - 1 + N_PER * it), need(K_PRO - 1 + N_PER * (it + 1))
        for cp in in_copies(lo, hi, in_sem.at[it]):
            cp.start()
        counts.append(sum(s1 - s0 for _, s0, s1 in slot_ranges(lo, hi)))
    n_min = min(counts)

    for bt in range(NT + 1):
        xall[bt * TS] = jnp.zeros((C, NB), bf16)

    for i in range(4):
        z_ref[i] = 0
    a, b = PA, PB
    a2, b2 = a * a, b * b
    ee = a2 + 1.0 + b2
    kap = 2.0 - a2 - b2
    k_rows = (C,) + (CM + 128,) * M + (CM,)

    def pair(d, i):
        p = _PTS[i]
        if p == 1.0:
            ev = d[0] + d[2] + d[4]
            od = d[1] + d[3] + d[5]
        else:
            ev = d[0] + (p ** 2) * d[2] + (p ** 4) * d[4]
            od = p * d[1] + (p ** 3) * d[3] + (p ** 5) * d[5]
        return ev + od, ev - od

    def ext_rows(i, u_i, d_prev, d_last):
        p = _PTS[i]
        if p == 1.0:
            return d_prev + u_i - d_last
        if p == -1.0:
            return d_prev - u_i - d_last
        return d_prev + p * u_i - (p ** M) * d_last

    def transform(gi):
        base = M * gi
        rhs = [xall[base + 1]]
        for i in range(1, M, 2):
            bz = base + z_ref[i // 2]
            d = [xall[bz + 1 + k].astype(f32) for k in range(M)]
            d_prev = xall[bz, CM:C, :].astype(f32)
            for k, u in enumerate(pair(d, i)):
                ext = ext_rows(i + k, u[CM:C], d_prev, d[M - 1][CM:C])
                rhs.append(jnp.concatenate([u, ext], axis=0).astype(bf16))
        rhs.append(xall[base + M, 0:CM, :])
        return rhs

    def transform_to_scratch(gi, which):
        base = M * gi
        for c0 in range(0, C, TCH):
            d = [xall[base + 1 + i, c0:c0 + TCH, :].astype(f32) for i in range(M)]
            for i in range(1, M, 2):
                for k, u in enumerate(pair(d, i)):
                    if i + k in which:
                        u16[i + k, c0:c0 + TCH, :] = u.astype(bf16)
                        if c0 >= CM:
                            d_prev = xall[base, c0:c0 + TCH, :].astype(f32)
                            ext = ext_rows(i + k, u, d_prev, d[M - 1])
                            u16[i + k, c0 + CR:c0 + CR + TCH, :] = ext.astype(bf16)

    def prod(i, rhs_i):
        nk = (k_rows[i] + 127) // 128
        lhs = jnp.concatenate([upk(wt_ref[i, kt]) for kt in range(nk)], axis=1)[:, :k_rows[i]]
        return jnp.dot(lhs, rhs_i, preferred_element_type=f32)

    def out_copy_static(lo, hi):
        for bt, s0, s1 in slot_ranges(lo, hi):
            pltpu.make_async_copy(oall.at[bt * TS + 1 + s0:bt * TS + 1 + s1],
                                  o_hbm.at[s0:s1, :, bt * NB:(bt + 1) * NB], out_sem.at[0]).start()

    def out_copy_slot(slot, r0=0, r1=None):
        r1 = C if r1 is None else r1
        bt = jax.lax.shift_right_logical(slot * 1986, 16)
        s1 = slot - bt * TS

        @pl.when(s1 > 0)
        def _():
            pltpu.make_async_copy(oall.at[pl.ds(slot, 1), r0:r1],
                                  o_hbm.at[pl.ds(s1 - 1, 1), r0:r1, pl.ds(pl.multiple_of(bt * NB, NB), NB)],
                                  out_sem.at[0]).start()

    def epilogue(gi, m, carry, copy_out, R0=0, R1=C):
        def epi(h, k):
            oall[M * gi + k, R0:R1, :] = (h * jnp.tanh(h) + h).astype(oall.dtype)

        sh = sh_ref[R0:R1, :]
        sc = sc_ref[R0:R1, :]
        sh3 = sh3_ref[R0:R1, :]
        m0 = m[0] * sc
        em0 = ee * m0
        sa, ta = m[1] + m[2], m[1] - m[2]
        s1s, t1s = (m[3] + m[4]) + sh, (m[3] - m[4]) + sh
        sb, tb = m[5] + m[6], m[5] - m[6]
        o6 = ((s1s - m0) + sa) + sb
        o2 = ((s1s - em0) + b2 * sa) + a2 * sb
        o4 = ((sh3 - m0) + kap * s1s) - o2 - o6
        q5 = (a * ta + t1s) + b * tb
        q1 = (b * ta + t1s) + a * tb
        q3 = (kap * t1s + sh3) - q1 - q5
        if carry is not None:
            q1 = q1 + carry[1]
        m7 = m[7] * sc
        em7 = ee * m7
        if carry is not None:
            epi(m0 + carry[0], 0)
        epi(o2, 2)
        epi(o4, 4)
        epi(q1 - m7, 1)
        epi(q3 + em7, 3)
        epi(q5 - em7, 5)
        if copy_out:
            for k in range(M):
                out_copy_slot(M * gi + k, R0, R1)
        return o6, m7

    def finish(gi, rhs, carry, copy_out):
        return epilogue(gi, [prod(i, rhs[i]) for i in range(NP)], carry, copy_out)

    def finish_h(gi, rhs, carry, copy_out=True, between=None):
        res = []
        for h, (R0, R1) in enumerate(HALVES):
            if h == 1 and between is not None:
                between()
            m = []
            for i in range(NP):
                nk = (k_rows[i] + 127) // 128
                lhs = jnp.concatenate([upk(wt_ref[i, kt, R0 // 2:R1 // 2, :]) for kt in range(nk)], axis=1)[:, :k_rows[i]]
                m.append(jnp.dot(lhs, rhs[i], preferred_element_type=f32))
            res.append(epilogue(gi, m, carry[h], copy_out, R0, R1))
        return res

    def weight_prep(kt):
        for d0 in range(0, C, 128):
            dn = min(128, C - d0)
            rows = slice(d0 // 2, (d0 + dn) // 2)
            if kt < KT - 1:
                g0, g1, g2 = [wbuf[2 - k, kt * 128:(kt + 1) * 128, d0:d0 + dn].T for k in range(3)]
                wt16[NP - 1, kt, d0:d0 + dn, :] = g2
                g2 = g2.astype(f32)
            else:
                w0r = wbuf[2, CM:C, d0:d0 + dn]
                g0 = jnp.concatenate([w0r, jnp.zeros_like(w0r)], axis=0).T
                g1 = jnp.concatenate([wbuf[1, CM:C, d0:d0 + dn], wbuf[0, CM:C, d0:d0 + dn]], axis=0).T
                g2 = None
            wt16[0, kt, d0:d0 + dn, :] = g0
            scl = sc_ref[d0:d0 + dn, :]
            g0, g1 = g0.astype(f32) * scl, g1.astype(f32) * scl
            if g2 is not None:
                g2 = g2 * scl
            for i in range(1, M, 2):
                pt, den = _PTS[i], _den(i)
                ev = g0 * (1.0 / den)
                if g2 is not None:
                    ev = ev + g2 * (pt * pt / den)
                od = g1 * (pt / den)
                wt16[i, kt, d0:d0 + dn, :] = (ev + od).astype(bf16)
                wt16[i + 1, kt, d0:d0 + dn, :] = (ev - od).astype(bf16)

    def partial_prod(i, kt0, kt1, rhs=None):
        hi = min(kt1 * 128, k_rows[i])
        nk = (hi + 127) // 128
        lhs = jnp.concatenate([upk(wt_ref[i, kt]) for kt in range(kt0, nk)], axis=1)[:, :hi - kt0 * 128]
        if rhs is not None:
            rhs = rhs[kt0 * 128:hi]
        elif i == 0:
            rhs = xall[1, kt0 * 128:hi, :]
        elif i == NP - 1:
            rhs = xall[M, kt0 * 128:hi, :]
        else:
            rhs = upk(u_scr[i, kt0 * 64:hi // 2, :])
        return jnp.dot(lhs, rhs, preferred_element_type=f32)

    for cp in p_copies:
        cp.wait()
    row = lambda r: r[...].astype(f32).reshape(1, C)
    scale = row(pg) * jax.lax.rsqrt(row(pv) + 1e-5)
    shift = row(pb) - row(pm) * scale
    sc_ref[...] = jnp.broadcast_to(0.5 * scale, (NB, C)).T
    sh_t = jnp.broadcast_to(0.5 * shift, (NB, C)).T
    sh_ref[...] = sh_t
    sh3_ref[...] = (3.0 - kap) * sh_t

    xa_copy.wait()
    transform_to_scratch(0, range(1, M + 1))
    for kt in range(KT - 1):
        w_copies[kt].wait()
        if kt == KT - 2:
            w_copies[KT - 1].wait()
        weight_prep(kt)
        if kt == KT - 2:
            weight_prep(KT - 1)
        if kt >= 1:
            for i in range(NP):
                part = partial_prod(i, kt - 1, kt + 1 if (kt == KT - 2 and i in EARLY) else kt)
                m_scr[i] = part if kt == 1 else m_scr[i] + part
    xb_copy.wait()
    m = [m_scr[i] + partial_prod(i, KT - 1 if i in EARLY else KT - 2, KT) if (i not in EARLY or k_rows[i] > CM) else m_scr[i]
         for i in range(NP)]
    carry = epilogue(0, m, None, False)
    carry = [(carry[0][R0:R1], carry[1][R0:R1]) for R0, R1 in HALVES]
    carry = finish_h(1, transform(1), carry, False, xc_copy.wait if G1_SPLIT else None)
    if not G1_SPLIT:
        xc_copy.wait()
    for gi in range(2, K_PRO):
        carry = finish_h(gi, transform(gi), carry, False)
    for h, (R0, R1) in enumerate(HALVES):
        c_scr[0, R0:R1, :] = carry[h][0]
        c_scr[1, R0:R1, :] = carry[h][1]

    def body(it, c):
        g0 = K_PRO + N_PER * it
        pltpu.make_async_copy(xall.at[0:n_min], xall.at[0:n_min], in_sem.at[it]).wait()
        for n in sorted(set(counts)):
            if n > n_min:
                hit = None
                for k, cnt in enumerate(counts):
                    if cnt == n:
                        hit = (it == k) if hit is None else jnp.logical_or(hit, it == k)

                @pl.when(hit)
                def _():
                    pltpu.make_async_copy(xall.at[0:n - n_min], xall.at[0:n - n_min], in_sem.at[it]).wait()

        @pl.when(it == 0)
        def _():
            out_copy_static(0, M * K_PRO)

        carry = [(c_scr[0, R0:R1, :], c_scr[1, R0:R1, :]) for R0, R1 in HALVES]
        for r in range(N_PER):
            carry = finish_h(g0 + r, transform(g0 + r), carry)
        for h, (R0, R1) in enumerate(HALVES):
            c_scr[0, R0:R1, :] = carry[h][0]
            c_scr[1, R0:R1, :] = carry[h][1]
        return c

    jax.lax.fori_loop(0, N_IT, body, 0)
    pltpu.make_async_copy(oall.at[0:NT * S], oall.at[0:NT * S], out_sem.at[0]).wait()


@jax.jit
def pallas_standalone__batchnorm__sampling_kernel(x, w, mean, var, g, b):
    B, S, C = x.shape
    NT = B // NB
    KT = CM // 128 + 1
    n_it = (NT * (S + 1) // M - K_PRO) // N_PER
    xt = jnp.transpose(x, (1, 2, 0))
    ot = pl.pallas_call(
        _kernel,
        in_specs=[pl.BlockSpec(memory_space=pl.ANY)] * 6,
        out_specs=pl.BlockSpec(memory_space=pl.ANY),
        out_shape=jax.ShapeDtypeStruct((S, C, B), x.dtype),
        scratch_shapes=[pltpu.VMEM((NT * (S + 1) + 1, C, NB), jnp.bfloat16),
                        pltpu.VMEM((NT * (S + 1), C, NB), jnp.bfloat16),
                        pltpu.VMEM((3, C, C), jnp.bfloat16),
                        pltpu.VMEM((C,), jnp.bfloat16),
                        pltpu.VMEM((C,), jnp.bfloat16),
                        pltpu.VMEM((C,), jnp.bfloat16),
                        pltpu.VMEM((C,), jnp.bfloat16),
                        pltpu.VMEM((NP, KT, C, 128), jnp.bfloat16),
                        pltpu.VMEM((C, NB), jnp.float32),
                        pltpu.VMEM((C, NB), jnp.float32),
                        pltpu.VMEM((C, NB), jnp.float32),
                        pltpu.VMEM((NP, KT * 128, NB), jnp.bfloat16),
                        pltpu.VMEM((NP, C, NB), jnp.float32),
                        pltpu.VMEM((2, C, NB), jnp.float32),
                        pltpu.SMEM((4,), jnp.int32),
                        pltpu.SemaphoreType.DMA((n_it,)),
                        pltpu.SemaphoreType.DMA((1,)),
                        pltpu.SemaphoreType.DMA((KT + 8,))],
        compiler_params=pltpu.CompilerParams(vmem_limit_bytes=110 * 1024 * 1024,
                                             disable_bounds_checks=True),
    )(xt, w, mean, var, g, b)
    return jnp.transpose(ot, (2, 0, 1))
```

```python
import jax
import jax.numpy as jnp
import jax.experimental.pallas as pl
import jax.experimental.pallas.tpu as pltpu

NB = 128
PA = 0.4375
PB = 1.0 / PA
CM = 512
M = 6
NP = M + 2
K_PRO = 4
N_PER = 5
TCH = 32
HALVES = ((0, 432), (432, 576))
G1_SPLIT = False
PLAN = ((0, 7, 3, 4), (1, 2, 5, 6))
FINE_ROWS = ((0, 320), (320, 576))

_PTS = (0.0, PA, -PA, 1.0, -1.0, PB, -PB)


def _den(i):
    d = 1.0
    for j, q in enumerate(_PTS):
        if j != i:
            d *= (_PTS[i] - q)
    return d


def _kernel(x_hbm, w_hbm, mean_hbm, var_hbm, g_hbm, b_hbm, o_hbm,
            xall, oall, wbuf, pm, pv, pg, pb, wt_ref, sc_ref, sh_ref, sh3_ref, u_scr, m_scr, c_scr, z_ref,
            in_sem, out_sem, misc_sem):
    S, C, B = x_hbm.shape
    NT = B // NB
    TS = S + 1
    NGT = NT * TS // M
    N_IT = (NGT - K_PRO) // N_PER
    KT = CM // 128 + 1
    CR = C - CM
    f32 = jnp.float32
    bf16 = jnp.bfloat16
    pk = lambda v: pltpu.bitcast(v, jnp.uint32)
    upk = lambda v: pltpu.bitcast(v, bf16)

    wt16, u16 = wt_ref, u_scr
    wt_ref = wt16.bitcast(jnp.uint32)
    u_scr = u16.bitcast(jnp.uint32)

    def slot_ranges(lo, hi):
        out = []
        for bt in range(NT):
            a0, a1 = max(lo, bt * TS + 1), min(hi, (bt + 1) * TS)
            if a0 < a1:
                out.append((bt, a0 - bt * TS - 1, a1 - bt * TS - 1))
        return out

    def in_copies(lo, hi, sem):
        return [pltpu.make_async_copy(x_hbm.at[s0:s1, :, bt * NB:(bt + 1) * NB],
                                      xall.at[bt * TS + 1 + s0:bt * TS + 1 + s1], sem)
                for bt, s0, s1 in slot_ranges(lo, hi)]

    p_copies = [pltpu.make_async_copy(src, dst, misc_sem.at[KT + 4 + i])
                for i, (src, dst) in enumerate(((mean_hbm, pm), (var_hbm, pv), (g_hbm, pg), (b_hbm, pb)))]
    w_copies = [pltpu.make_async_copy(w_hbm.at[:, kt * 128:min(C, (kt + 1) * 128), :],
                                      wbuf.at[:, kt * 128:min(C, (kt + 1) * 128), :], misc_sem.at[kt])
                for kt in range(KT)]
    need = lambda g: M * (g + 1) + 1
    xa_copies = [pltpu.make_async_copy(x_hbm.at[0:M, kt * 128:min(C, (kt + 1) * 128), 0:NB],
                                       xall.at[1:M + 1, kt * 128:min(C, (kt + 1) * 128), :],
                                       misc_sem.at[KT + 8 + kt]) for kt in range(KT)]
    (xb_copy,) = in_copies(need(0), need(1), misc_sem.at[KT + 1])
    (xc_copy,) = in_copies(need(1), need(K_PRO - 1), misc_sem.at[KT + 2])
    for cp in p_copies + [c for wx in zip(w_copies, xa_copies) for c in wx] + [xb_copy, xc_copy]:
        cp.start()
    counts = []
    for it in range(N_IT):
        lo, hi = need(K_PRO - 1 + N_PER * it), need(K_PRO - 1 + N_PER * (it + 1))
        for cp in in_copies(lo, hi, in_sem.at[it]):
            cp.start()
        counts.append(sum(s1 - s0 for _, s0, s1 in slot_ranges(lo, hi)))
    n_min = min(counts)

    for bt in range(NT + 1):
        xall[bt * TS] = jnp.zeros((C, NB), bf16)

    for i in range(4):
        z_ref[i] = 0
    a, b = PA, PB
    a2, b2 = a * a, b * b
    ee = a2 + 1.0 + b2
    kap = 2.0 - a2 - b2
    k_rows = (C,) + (CM + 128,) * M + (CM,)

    def pair(d, i):
        p = _PTS[i]
        if p == 1.0:
            ev = d[0] + d[2] + d[4]
            od = d[1] + d[3] + d[5]
        else:
            ev = d[0] + (p ** 2) * d[2] + (p ** 4) * d[4]
            od = p * d[1] + (p ** 3) * d[3] + (p ** 5) * d[5]
        return ev + od, ev - od

    def ext_rows(i, u_i, d_prev, d_last):
        p = _PTS[i]
        if p == 1.0:
            return d_prev + u_i - d_last
        if p == -1.0:
            return d_prev - u_i - d_last
        return d_prev + p * u_i - (p ** M) * d_last

    def transform(gi):
        base = M * gi
        rhs = [xall[base + 1]]
        for i in range(1, M, 2):
            bz = base + z_ref[i // 2]
            d = [xall[bz + 1 + k].astype(f32) for k in range(M)]
            d_prev = xall[bz, CM:C, :].astype(f32)
            for k, u in enumerate(pair(d, i)):
                ext = ext_rows(i + k, u[CM:C], d_prev, d[M - 1][CM:C])
                rhs.append(jnp.concatenate([u, ext], axis=0).astype(bf16))
        rhs.append(xall[base + M, 0:CM, :])
        return rhs

    def transform_to_scratch(gi, which, kt):
        base = M * gi
        for c0 in range(kt * 128, min(C, (kt + 1) * 128), TCH):
            d = [xall[base + 1 + i, c0:c0 + TCH, :].astype(f32) for i in range(M)]
            for i in range(1, M, 2):
                for k, u in enumerate(pair(d, i)):
                    if i + k in which:
                        u16[i + k, c0:c0 + TCH, :] = u.astype(bf16)
                        if c0 >= CM:
                            d_prev = xall[base, c0:c0 + TCH, :].astype(f32)
                            ext = ext_rows(i + k, u, d_prev, d[M - 1])
                            u16[i + k, c0 + CR:c0 + CR + TCH, :] = ext.astype(bf16)

    def prod(i, rhs_i):
        nk = (k_rows[i] + 127) // 128
        lhs = jnp.concatenate([upk(wt_ref[i, kt]) for kt in range(nk)], axis=1)[:, :k_rows[i]]
        return jnp.dot(lhs, rhs_i, preferred_element_type=f32)

    def out_copy_static(lo, hi):
        for bt, s0, s1 in slot_ranges(lo, hi):
            pltpu.make_async_copy(oall.at[bt * TS + 1 + s0:bt * TS + 1 + s1],
                                  o_hbm.at[s0:s1, :, bt * NB:(bt + 1) * NB], out_sem.at[0]).start()

    def out_copy_slot(slot, r0=0, r1=None):
        r1 = C if r1 is None else r1
        bt = jax.lax.shift_right_logical(slot * 1986, 16)
        s1 = slot - bt * TS

        @pl.when(s1 > 0)
        def _():
            pltpu.make_async_copy(oall.at[pl.ds(slot, 1), r0:r1],
                                  o_hbm.at[pl.ds(s1 - 1, 1), r0:r1, pl.ds(pl.multiple_of(bt * NB, NB), NB)],
                                  out_sem.at[0]).start()

    def epilogue(gi, m, carry, copy_out, R0=0, R1=C):
        def epi(h, k):
            oall[M * gi + k, R0:R1, :] = (h * jnp.tanh(h) + h).astype(oall.dtype)

        sh = sh_ref[R0:R1, :]
        sc = sc_ref[R0:R1, :]
        sh3 = sh3_ref[R0:R1, :]
        m0 = m[0] * sc
        em0 = ee * m0
        sa, ta = m[1] + m[2], m[1] - m[2]
        s1s, t1s = (m[3] + m[4]) + sh, (m[3] - m[4]) + sh
        sb, tb = m[5] + m[6], m[5] - m[6]
        o6 = ((s1s - m0) + sa) + sb
        o2 = ((s1s - em0) + b2 * sa) + a2 * sb
        o4 = ((sh3 - m0) + kap * s1s) - o2 - o6
        q5 = (a * ta + t1s) + b * tb
        q1 = (b * ta + t1s) + a * tb
        q3 = (kap * t1s + sh3) - q1 - q5
        if carry is not None:
            q1 = q1 + carry[1]
        m7 = m[7] * sc
        em7 = ee * m7
        if carry is not None:
            epi(m0 + carry[0], 0)
        epi(o2, 2)
        epi(o4, 4)
        epi(q1 - m7, 1)
        epi(q3 + em7, 3)
        epi(q5 - em7, 5)
        if copy_out:
            for k in range(M):
                out_copy_slot(M * gi + k, R0, R1)
        return o6, m7

    def finish(gi, rhs, carry, copy_out):
        return epilogue(gi, [prod(i, rhs[i]) for i in range(NP)], carry, copy_out)

    def finish_h(gi, rhs, carry, copy_out=True, between=None):
        res = []
        for h, (R0, R1) in enumerate(HALVES):
            if h == 1 and between is not None:
                between()
            m = []
            for i in range(NP):
                nk = (k_rows[i] + 127) // 128
                lhs = jnp.concatenate([upk(wt_ref[i, kt, R0 // 2:R1 // 2, :]) for kt in range(nk)], axis=1)[:, :k_rows[i]]
                m.append(jnp.dot(lhs, rhs[i], preferred_element_type=f32))
            res.append(epilogue(gi, m, carry[h], copy_out, R0, R1))
        return res

    def weight_prep(kt):
        for d0 in range(0, C, 128):
            dn = min(128, C - d0)
            rows = slice(d0 // 2, (d0 + dn) // 2)
            if kt < KT - 1:
                g0, g1, g2 = [wbuf[2 - k, kt * 128:(kt + 1) * 128, d0:d0 + dn].T for k in range(3)]
                wt_ref[NP - 1, kt, rows, :] = pk(g2)
                g2 = g2.astype(f32)
            else:
                w0r = wbuf[2, CM:C, d0:d0 + dn]
                g0 = jnp.concatenate([w0r, jnp.zeros_like(w0r)], axis=0).T
                g1 = jnp.concatenate([wbuf[1, CM:C, d0:d0 + dn], wbuf[0, CM:C, d0:d0 + dn]], axis=0).T
                g2 = None
            wt_ref[0, kt, rows, :] = pk(g0)
            scl = sc_ref[d0:d0 + dn, :]
            g0, g1 = g0.astype(f32) * scl, g1.astype(f32) * scl
            if g2 is not None:
                g2 = g2 * scl
            for i in range(1, M, 2):
                pt, den = _PTS[i], _den(i)
                ev = g0 * (1.0 / den)
                if g2 is not None:
                    ev = ev + g2 * (pt * pt / den)
                od = g1 * (pt / den)
                wt16[i, kt, d0:d0 + dn, :] = (ev + od).astype(bf16)
                wt16[i + 1, kt, d0:d0 + dn, :] = (ev - od).astype(bf16)

    def partial_prod(i, kt0, kt1, rhs=None):
        hi = min(kt1 * 128, k_rows[i])
        nk = (hi + 127) // 128
        lhs = jnp.concatenate([upk(wt_ref[i, kt]) for kt in range(kt0, nk)], axis=1)[:, :hi - kt0 * 128]
        if rhs is not None:
            rhs = rhs[kt0 * 128:hi]
        elif i == 0:
            rhs = xall[1, kt0 * 128:hi, :]
        elif i == NP - 1:
            rhs = xall[M, kt0 * 128:hi, :]
        else:
            rhs = upk(u_scr[i, kt0 * 64:hi // 2, :])
        return jnp.dot(lhs, rhs, preferred_element_type=f32)

    for cp in p_copies:
        cp.wait()
    row = lambda r: r[...].astype(f32).reshape(1, C)
    scale = row(pg) * jax.lax.rsqrt(row(pv) + 1e-5)
    shift = row(pb) - row(pm) * scale
    sc_ref[...] = jnp.broadcast_to(0.5 * scale, (NB, C)).T
    sh_t = jnp.broadcast_to(0.5 * shift, (NB, C)).T
    sh_ref[...] = sh_t
    sh3_ref[...] = (3.0 - kap) * sh_t

    done = [0] * NP

    def advance(steps):
        acc = {}
        for i, kt1 in steps:
            part = partial_prod(i, done[i], kt1)
            if i in acc:
                acc[i] = acc[i] + part
            else:
                acc[i] = part if done[i] == 0 else m_scr[i] + part
            done[i] = kt1
        for i, v in acc.items():
            m_scr[i] = v

    SF, SG = PLAN
    allp = range(1, M + 1)
    w_copies[0].wait()
    weight_prep(0)
    xa_copies[0].wait()
    transform_to_scratch(0, allp, 0)
    advance([(i, 1) for i in SF])
    w_copies[1].wait()
    xa_copies[1].wait()
    weight_prep(1)
    transform_to_scratch(0, allp, 1)
    advance([(i, 1) for i in SG] + [(i, 2) for i in SG])
    w_copies[2].wait()
    xa_copies[2].wait()
    weight_prep(2)
    transform_to_scratch(0, allp, 2)
    advance([(i, 2) for i in SF] + [(i, 3) for i in SF])
    for kt in (3, 4):
        w_copies[kt].wait()
        xa_copies[kt].wait()
    for kt in (3, 4):
        weight_prep(kt)
        transform_to_scratch(0, allp, kt)
    advance([(i, 3) for i in SG] + [(i, 4) for i in SF])
    xb_copy.wait()
    m = [m_scr[i] + partial_prod(i, done[i], KT) if done[i] * 128 < k_rows[i] else m_scr[i] for i in range(NP)]
    carry = epilogue(0, m, None, False)
    carry = [(carry[0][R0:R1], carry[1][R0:R1]) for R0, R1 in HALVES]
    carry = finish_h(1, transform(1), carry, False, xc_copy.wait if G1_SPLIT else None)
    if not G1_SPLIT:
        xc_copy.wait()
    for gi in range(2, K_PRO):
        carry = finish_h(gi, transform(gi), carry, False)
    for h, (R0, R1) in enumerate(HALVES):
        c_scr[0, R0:R1, :] = carry[h][0]
        c_scr[1, R0:R1, :] = carry[h][1]

    def body(it, c):
        g0 = K_PRO + N_PER * it
        pltpu.make_async_copy(xall.at[0:n_min], xall.at[0:n_min], in_sem.at[it]).wait()
        for n in sorted(set(counts)):
            if n > n_min:
                hit = None
                for k, cnt in enumerate(counts):
                    if cnt == n:
                        hit = (it == k) if hit is None else jnp.logical_or(hit, it == k)

                @pl.when(hit)
                def _():
                    pltpu.make_async_copy(xall.at[0:n - n_min], xall.at[0:n - n_min], in_sem.at[it]).wait()

        @pl.when(it == 0)
        def _():
            out_copy_static(0, M * K_PRO)

        carry = [(c_scr[0, R0:R1, :], c_scr[1, R0:R1, :]) for R0, R1 in HALVES]
        for r in range(N_PER):
            carry = finish_h(g0 + r, transform(g0 + r), carry)
        for h, (R0, R1) in enumerate(HALVES):
            c_scr[0, R0:R1, :] = carry[h][0]
            c_scr[1, R0:R1, :] = carry[h][1]
        return c

    jax.lax.fori_loop(0, N_IT, body, 0)
    pltpu.make_async_copy(oall.at[0:NT * S], oall.at[0:NT * S], out_sem.at[0]).wait()


@jax.jit
def pallas_standalone__batchnorm__sampling_kernel(x, w, mean, var, g, b):
    B, S, C = x.shape
    NT = B // NB
    KT = CM // 128 + 1
    n_it = (NT * (S + 1) // M - K_PRO) // N_PER
    xt = jnp.transpose(x, (1, 2, 0))
    ot = pl.pallas_call(
        _kernel,
        in_specs=[pl.BlockSpec(memory_space=pl.ANY)] * 6,
        out_specs=pl.BlockSpec(memory_space=pl.ANY),
        out_shape=jax.ShapeDtypeStruct((S, C, B), x.dtype),
        scratch_shapes=[pltpu.VMEM((NT * (S + 1) + 1, C, NB), jnp.bfloat16),
                        pltpu.VMEM((NT * (S + 1), C, NB), jnp.bfloat16),
                        pltpu.VMEM((3, C, C), jnp.bfloat16),
                        pltpu.VMEM((C,), jnp.bfloat16),
                        pltpu.VMEM((C,), jnp.bfloat16),
                        pltpu.VMEM((C,), jnp.bfloat16),
                        pltpu.VMEM((C,), jnp.bfloat16),
                        pltpu.VMEM((NP, KT, C, 128), jnp.bfloat16),
                        pltpu.VMEM((C, NB), jnp.float32),
                        pltpu.VMEM((C, NB), jnp.float32),
                        pltpu.VMEM((C, NB), jnp.float32),
                        pltpu.VMEM((NP, KT * 128, NB), jnp.bfloat16),
                        pltpu.VMEM((NP, C, NB), jnp.float32),
                        pltpu.VMEM((2, C, NB), jnp.float32),
                        pltpu.SMEM((4,), jnp.int32),
                        pltpu.SemaphoreType.DMA((n_it,)),
                        pltpu.SemaphoreType.DMA((1,)),
                        pltpu.SemaphoreType.DMA((2 * KT + 8,))],
        compiler_params=pltpu.CompilerParams(vmem_limit_bytes=110 * 1024 * 1024,
                                             disable_bounds_checks=True),
    )(xt, w, mean, var, g, b)
    return jnp.transpose(ot, (2, 0, 1))
```

```python
import jax
import jax.numpy as jnp
import jax.experimental.pallas as pl
import jax.experimental.pallas.tpu as pltpu

NB = 128
PA = 0.4375
PB = 1.0 / PA
CM = 512
M = 6
NP = M + 2
K_PRO = 4
N_PER = 5
TCH = 32
ROWS = ((0, 432), (432, 576))
PRO_ROWS = ((0, 512), (512, 576))
SET_F, SET_G = (0, 7, 3, 4), (1, 2, 5, 6)

_PTS = (0.0, PA, -PA, 1.0, -1.0, PB, -PB)


def _den(i):
    d = 1.0
    for j, q in enumerate(_PTS):
        if j != i:
            d *= (_PTS[i] - q)
    return d


def _kernel(x_hbm, w_hbm, mean_hbm, var_hbm, g_hbm, b_hbm, o_hbm,
            xall, oall, wbuf, pm, pv, pg, pb, wt_ref, sc_ref, sh_ref, shx_ref, u_scr, m_scr, c_scr,
            in_sem, out_sem, w_sem, xa_sem, misc_sem):
    S, C, B = x_hbm.shape
    NT = B // NB
    TS = S + 1
    NGT = NT * TS // M
    N_IT = (NGT - K_PRO) // N_PER
    KT = CM // 128 + 1
    CR = C - CM
    f32 = jnp.float32
    bf16 = jnp.bfloat16
    pk = lambda v: pltpu.bitcast(v, jnp.uint32)
    upk = lambda v: pltpu.bitcast(v, bf16)
    k_rows = (C,) + (CM + 128,) * M + (CM,)

    a, b = PA, PB
    a2, b2 = a * a, b * b
    ee = a2 + 1.0 + b2
    kap = 2.0 - a2 - b2

    def krange(kt):
        return slice(kt * 128, min(C, (kt + 1) * 128))

    def slot_ranges(lo, hi):
        out = []
        for bt in range(NT):
            a0, a1 = max(lo, bt * TS + 1), min(hi, (bt + 1) * TS)
            if a0 < a1:
                out.append((bt, a0 - bt * TS - 1, a1 - bt * TS - 1))
        return out

    def in_copies(lo, hi, sem):
        return [pltpu.make_async_copy(x_hbm.at[s0:s1, :, bt * NB:(bt + 1) * NB],
                                      xall.at[bt * TS + 1 + s0:bt * TS + 1 + s1], sem)
                for bt, s0, s1 in slot_ranges(lo, hi)]

    need = lambda g: M * (g + 1) + 1
    p_copies = [pltpu.make_async_copy(src, dst, misc_sem.at[2 + i])
                for i, (src, dst) in enumerate(((mean_hbm, pm), (var_hbm, pv), (g_hbm, pg), (b_hbm, pb)))]
    w_copies = [pltpu.make_async_copy(w_hbm.at[:, krange(kt), :], wbuf.at[:, krange(kt), :], w_sem.at[kt])
                for kt in range(KT)]
    xa_copies = [pltpu.make_async_copy(x_hbm.at[0:M, krange(kt), 0:NB], xall.at[1:M + 1, krange(kt), :],
                                       xa_sem.at[kt]) for kt in range(KT)]
    (xb_copy,) = in_copies(need(0), need(1), misc_sem.at[0])
    (xc_copy,) = in_copies(need(1), need(K_PRO - 1), misc_sem.at[1])
    for cp in p_copies + [c for wx in zip(w_copies, xa_copies) for c in wx] + [xb_copy, xc_copy]:
        cp.start()
    counts = []
    for it in range(N_IT):
        lo, hi = need(K_PRO - 1 + N_PER * it), need(K_PRO - 1 + N_PER * (it + 1))
        for cp in in_copies(lo, hi, in_sem.at[it]):
            cp.start()
        counts.append(sum(s1 - s0 for _, s0, s1 in slot_ranges(lo, hi)))

    for bt in range(NT + 1):
        xall[bt * TS] = jnp.zeros((C, NB), bf16)

    def pair(d, i):
        p = _PTS[i]
        if p == 1.0:
            ev = d[0] + d[2] + d[4]
            od = d[1] + d[3] + d[5]
        else:
            ev = d[0] + (p ** 2) * d[2] + (p ** 4) * d[4]
            od = p * d[1] + (p ** 3) * d[3] + (p ** 5) * d[5]
        return ev + od, ev - od

    def ext_rows(i, u_i, d_prev, d_last):
        p = _PTS[i]
        if p == 1.0:
            return d_prev + u_i - d_last
        if p == -1.0:
            return d_prev - u_i - d_last
        return d_prev + p * u_i - (p ** M) * d_last

    def transform(gi, zs=(0, 0, 0)):
        base = M * gi
        rhs = [xall[base + 1]]
        for i in range(1, M, 2):
            bz = base + zs[i // 2]
            d = [xall[bz + 1 + k].astype(f32) for k in range(M)]
            d_prev = xall[bz, CM:C, :].astype(f32)
            for k, u in enumerate(pair(d, i)):
                ext = ext_rows(i + k, u[CM:C], d_prev, d[M - 1][CM:C])
                rhs.append(jnp.concatenate([u, ext], axis=0).astype(bf16))
        rhs.append(xall[base + M, 0:CM, :])
        return rhs

    def transform0(kt):
        for c0 in range(krange(kt).start, krange(kt).stop, TCH):
            d = [xall[1 + i, c0:c0 + TCH, :].astype(f32) for i in range(M)]
            for i in range(1, M, 2):
                for k, u in enumerate(pair(d, i)):
                    u_scr[i + k, c0 // 2:(c0 + TCH) // 2, :] = pk(u.astype(bf16))
                    if c0 >= CM:
                        ext = ext_rows(i + k, u, xall[0, c0:c0 + TCH, :].astype(f32), d[M - 1])
                        u_scr[i + k, (c0 + CR) // 2:(c0 + CR + TCH) // 2, :] = pk(ext.astype(bf16))

    def weight_prep(kt):
        for d0 in range(0, C, 128):
            dn = min(128, C - d0)
            rows = slice(d0 // 2, (d0 + dn) // 2)
            if kt < KT - 1:
                g0, g1, g2 = [wbuf[2 - k, krange(kt), d0:d0 + dn].T for k in range(3)]
                wt_ref[NP - 1, kt, rows, :] = pk(g2)
                g2 = g2.astype(f32)
            else:
                g0r = wbuf[2, CM:C, d0:d0 + dn]
                g0 = jnp.concatenate([g0r, jnp.zeros_like(g0r)], axis=0).T
                g1 = jnp.concatenate([wbuf[1, CM:C, d0:d0 + dn], wbuf[0, CM:C, d0:d0 + dn]], axis=0).T
                g2 = None
            wt_ref[0, kt, rows, :] = pk(g0)
            scl = sc_ref[d0:d0 + dn, :]
            g0, g1 = g0.astype(f32) * scl, g1.astype(f32) * scl
            if g2 is not None:
                g2 = g2 * scl
            for i in range(1, M, 2):
                pt, den = _PTS[i], _den(i)
                ev = g0 * (1.0 / den)
                if g2 is not None:
                    ev = ev + g2 * (pt * pt / den)
                od = g1 * (pt / den)
                wt_ref[i, kt, rows, :] = pk((ev + od).astype(bf16))
                wt_ref[i + 1, kt, rows, :] = pk((ev - od).astype(bf16))

    def prod(i, rhs, r0, r1, kt0=0, kt1=KT):
        hi = min(kt1 * 128, k_rows[i])
        lhs = jnp.concatenate([upk(wt_ref[i, kt, r0 // 2:r1 // 2, :]) for kt in range(kt0, (hi + 127) // 128)],
                              axis=1)[:, :hi - kt0 * 128]
        return jnp.dot(lhs, rhs(kt0 * 128, hi), preferred_element_type=f32)

    def out_copy(slot, r0, r1):
        bt = jax.lax.shift_right_logical(slot * 1986, 16)
        s1 = slot - bt * TS

        @pl.when(s1 > 0)
        def _():
            pltpu.make_async_copy(oall.at[pl.ds(slot, 1), r0:r1],
                                  o_hbm.at[pl.ds(s1 - 1, 1), r0:r1, pl.ds(pl.multiple_of(bt * NB, NB), NB)],
                                  out_sem.at[0]).start()

    def epilogue(gi, m, carry, r0, r1, copy_out):
        def act(h, k):
            oall[M * gi + k, r0:r1, :] = (h * jnp.tanh(h) + h).astype(bf16)

        sc, sh, shx = sc_ref[r0:r1, :], sh_ref[r0:r1, :], shx_ref[r0:r1, :]
        m0 = m[0] * sc
        em0 = ee * m0
        sa, ta = m[1] + m[2], m[1] - m[2]
        s1, t1 = (m[3] + m[4]) + sh, (m[3] - m[4]) + sh
        sb, tb = m[5] + m[6], m[5] - m[6]
        o6 = ((s1 - m0) + sa) + sb
        o2 = ((s1 - em0) + b2 * sa) + a2 * sb
        o4 = ((shx - m0) + kap * s1) - o2 - o6
        q5 = (a * ta + t1) + b * tb
        q1 = (b * ta + t1) + a * tb
        q3 = (kap * t1 + shx) - q1 - q5
        if carry is not None:
            q1 = q1 + carry[1]
        m7 = m[7] * sc
        em7 = ee * m7
        if carry is not None:
            act(m0 + carry[0], 0)
        act(o2, 2)
        act(o4, 4)
        act(q1 - m7, 1)
        act(q3 + em7, 3)
        act(q5 - em7, 5)
        if copy_out:
            for k in range(M):
                out_copy(M * gi + k, r0, r1)
        return o6, m7

    def group(gi, rhs, carry, rows, copy_out):
        return [epilogue(gi, [prod(i, lambda lo, hi, v=rhs[i]: v, r0, r1) for i in range(NP)],
                         carry[h], r0, r1, copy_out)
                for h, (r0, r1) in enumerate(rows)]

    def save_carry(carry, rows):
        for h, (r0, r1) in enumerate(rows):
            c_scr[0, r0:r1, :] = carry[h][0]
            c_scr[1, r0:r1, :] = carry[h][1]

    for cp in p_copies:
        cp.wait()
    row = lambda r: r[...].astype(f32).reshape(1, C)
    scale = row(pg) * jax.lax.rsqrt(row(pv) + 1e-5)
    shift = row(pb) - row(pm) * scale
    sc_ref[...] = jnp.broadcast_to(0.5 * scale, (NB, C)).T
    sh_t = jnp.broadcast_to(0.5 * shift, (NB, C)).T
    sh_ref[...] = sh_t
    shx_ref[...] = (3.0 - kap) * sh_t

    def rhs0(i):
        if i == 0:
            return lambda lo, hi: xall[1, lo:hi, :]
        if i == NP - 1:
            return lambda lo, hi: xall[M, lo:hi, :]
        return lambda lo, hi: upk(u_scr[i, lo // 2:hi // 2, :])

    done = [0] * NP

    def advance(steps):
        acc = {}
        for i, kt1 in steps:
            part = prod(i, rhs0(i), 0, C, done[i], kt1)
            if i in acc:
                acc[i] = acc[i] + part
            else:
                acc[i] = part if done[i] == 0 else m_scr[i] + part
            done[i] = kt1
        for i, v in acc.items():
            m_scr[i] = v

    w_copies[0].wait()
    weight_prep(0)
    xa_copies[0].wait()
    transform0(0)
    advance([(i, 1) for i in SET_F])
    w_copies[1].wait()
    xa_copies[1].wait()
    weight_prep(1)
    transform0(1)
    advance([(i, 1) for i in SET_G] + [(i, 2) for i in SET_G])
    w_copies[2].wait()
    xa_copies[2].wait()
    weight_prep(2)
    transform0(2)
    advance([(i, 2) for i in SET_F] + [(i, 3) for i in SET_F])
    for kt in (3, 4):
        w_copies[kt].wait()
        xa_copies[kt].wait()
    for kt in (3, 4):
        weight_prep(kt)
        transform0(kt)
    advance([(i, 3) for i in SET_G] + [(i, 4) for i in SET_F])
    xb_copy.wait()
    cs = []
    for r0, r1 in ROWS:
        m = [m_scr[i, r0:r1, :] + prod(i, rhs0(i), r0, r1, done[i]) if done[i] * 128 < k_rows[i]
             else m_scr[i, r0:r1, :] for i in range(NP)]
        cs.append(epilogue(0, m, None, r0, r1, False))
    carry = [jnp.concatenate([c[k] for c in cs], axis=0) for k in range(2)]
    carry = [(carry[0][r0:r1], carry[1][r0:r1]) for r0, r1 in PRO_ROWS]
    carry = group(1, transform(1), carry, PRO_ROWS, False)
    xc_copy.wait()
    for gi in range(2, K_PRO):
        carry = group(gi, transform(gi), carry, PRO_ROWS, False)
    save_carry(carry, PRO_ROWS)

    n_min = min(counts)

    def body(it, c):
        g0 = K_PRO + N_PER * it
        pltpu.make_async_copy(xall.at[0:n_min], xall.at[0:n_min], in_sem.at[it]).wait()
        for n in sorted(set(counts) - {n_min}):
            hit = None
            for k, cnt in enumerate(counts):
                if cnt == n:
                    hit = (it == k) if hit is None else jnp.logical_or(hit, it == k)

            @pl.when(hit)
            def _():
                pltpu.make_async_copy(xall.at[0:n - n_min], xall.at[0:n - n_min], in_sem.at[it]).wait()

        @pl.when(it == 0)
        def _():
            for bt, s0, s1 in slot_ranges(0, M * K_PRO):
                pltpu.make_async_copy(oall.at[bt * TS + 1 + s0:bt * TS + 1 + s1],
                                      o_hbm.at[s0:s1, :, bt * NB:(bt + 1) * NB], out_sem.at[0]).start()

        zs = (0, jax.lax.shift_right_logical(it, 8), jax.lax.shift_right_logical(it, 9))
        carry = [(c_scr[0, r0:r1, :], c_scr[1, r0:r1, :]) for r0, r1 in ROWS]
        for r in range(N_PER):
            gi = g0 + r
            carry = group(gi, transform(gi, zs), carry, ROWS, True)
        save_carry(carry, ROWS)
        return c

    jax.lax.fori_loop(0, N_IT, body, 0)
    pltpu.make_async_copy(oall.at[0:NT * S], oall.at[0:NT * S], out_sem.at[0]).wait()


@jax.jit
def pallas_standalone__batchnorm__sampling_kernel(
    x: jax.Array,
    w: jax.Array,
    mean: jax.Array,
    var: jax.Array,
    g: jax.Array,
    b: jax.Array,
):
    B, S, C = x.shape
    assert (B, S, C) == (1024, 32, 576) and w.shape == (3, C, C)
    NT = B // NB
    KT = CM // 128 + 1
    n_it = (NT * (S + 1) // M - K_PRO) // N_PER
    xt = jnp.transpose(x, (1, 2, 0))
    ot = pl.pallas_call(
        _kernel,
        in_specs=[pl.BlockSpec(memory_space=pl.ANY)] * 6,
        out_specs=pl.BlockSpec(memory_space=pl.ANY),
        out_shape=jax.ShapeDtypeStruct((S, C, B), x.dtype),
        scratch_shapes=[pltpu.VMEM((NT * (S + 1) + 1, C, NB), jnp.bfloat16),
                        pltpu.VMEM((NT * (S + 1), C, NB), jnp.bfloat16),
                        pltpu.VMEM((3, C, C), jnp.bfloat16),
                        pltpu.VMEM((C,), jnp.bfloat16),
                        pltpu.VMEM((C,), jnp.bfloat16),
                        pltpu.VMEM((C,), jnp.bfloat16),
                        pltpu.VMEM((C,), jnp.bfloat16),
                        pltpu.VMEM((NP, KT, C // 2, 128), jnp.uint32),
                        pltpu.VMEM((C, NB), jnp.float32),
                        pltpu.VMEM((C, NB), jnp.float32),
                        pltpu.VMEM((C, NB), jnp.float32),
                        pltpu.VMEM((NP - 1, KT * 64, NB), jnp.uint32),
                        pltpu.VMEM((NP, C, NB), jnp.float32),
                        pltpu.VMEM((2, C, NB), jnp.float32),
                        pltpu.SemaphoreType.DMA((n_it,)),
                        pltpu.SemaphoreType.DMA((1,)),
                        pltpu.SemaphoreType.DMA((KT,)),
                        pltpu.SemaphoreType.DMA((KT,)),
                        pltpu.SemaphoreType.DMA((6,))],
        compiler_params=pltpu.CompilerParams(vmem_limit_bytes=110 * 1024 * 1024,
                                             disable_bounds_checks=True),
    )(xt, w, mean, var, g, b)
    return jnp.transpose(ot, (2, 0, 1))
```

```python
import jax
import jax.numpy as jnp
import jax.experimental.pallas as pl
import jax.experimental.pallas.tpu as pltpu

NB = 128
PA = 0.4375
PB = 1.0 / PA
CM = 512
M = 6
NP = M + 2
K_PRO = 4
N_PER = 5
TCH = 32
ROWS = ((0, 432), (432, 576))
LAST_ROWS = ((0, 368), (368, 512), (512, 576))
PRO_ROWS = ((0, 512), (512, 576))
SET_F, SET_G = (0, 7, 1, 2), (3, 4, 5, 6)

_PTS = (0.0, PA, -PA, 1.0, -1.0, PB, -PB)


def _den(i):
    d = 1.0
    for j, q in enumerate(_PTS):
        if j != i:
            d *= (_PTS[i] - q)
    return d


def _kernel(x_hbm, w_hbm, mean_hbm, var_hbm, g_hbm, b_hbm, o_hbm,
            xall, oall, wbuf, pm, pv, pg, pb, wt_ref, sc_ref, sh_ref, shx_ref, u_scr, m_scr, c_scr,
            in_sem, out_sem, w_sem, xa_sem, misc_sem):
    S, C, B = x_hbm.shape
    NT = B // NB
    TS = S + 1
    NGT = NT * TS // M
    N_IT = (NGT - K_PRO) // N_PER
    KT = CM // 128 + 1
    CR = C - CM
    f32 = jnp.float32
    bf16 = jnp.bfloat16
    pk = lambda v: pltpu.bitcast(v, jnp.uint32)
    upk = lambda v: pltpu.bitcast(v, bf16)
    k_rows = (C,) + (CM + 128,) * M + (CM,)

    a, b = PA, PB
    a2, b2 = a * a, b * b
    ee = a2 + 1.0 + b2
    kap = 2.0 - a2 - b2

    def krange(kt):
        return slice(kt * 128, min(C, (kt + 1) * 128))

    def slot_ranges(lo, hi):
        out = []
        for bt in range(NT):
            a0, a1 = max(lo, bt * TS + 1), min(hi, (bt + 1) * TS)
            if a0 < a1:
                out.append((bt, a0 - bt * TS - 1, a1 - bt * TS - 1))
        return out

    def in_copies(lo, hi, sem):
        return [pltpu.make_async_copy(x_hbm.at[s0:s1, :, bt * NB:(bt + 1) * NB],
                                      xall.at[bt * TS + 1 + s0:bt * TS + 1 + s1], sem)
                for bt, s0, s1 in slot_ranges(lo, hi)]

    need = lambda g: M * (g + 1) + 1
    p_copies = [pltpu.make_async_copy(src, dst, misc_sem.at[2 + i])
                for i, (src, dst) in enumerate(((mean_hbm, pm), (var_hbm, pv), (g_hbm, pg), (b_hbm, pb)))]
    w_copies = [pltpu.make_async_copy(w_hbm.at[:, krange(kt), :], wbuf.at[:, krange(kt), :], w_sem.at[kt])
                for kt in range(KT)]
    xa_copies = [pltpu.make_async_copy(x_hbm.at[0:M, krange(kt), 0:NB], xall.at[1:M + 1, krange(kt), :],
                                       xa_sem.at[kt]) for kt in range(KT)]
    (xb_copy,) = in_copies(need(0), need(1), misc_sem.at[0])
    (xc_copy,) = in_copies(need(1), need(K_PRO - 1), misc_sem.at[1])
    for cp in p_copies + [c for wx in zip(w_copies, xa_copies) for c in wx] + [xb_copy, xc_copy]:
        cp.start()
    counts = []
    for it in range(N_IT):
        lo, hi = need(K_PRO - 1 + N_PER * it), need(K_PRO - 1 + N_PER * (it + 1))
        for cp in in_copies(lo, hi, in_sem.at[it]):
            cp.start()
        counts.append(sum(s1 - s0 for _, s0, s1 in slot_ranges(lo, hi)))

    for bt in range(NT + 1):
        xall[bt * TS] = jnp.zeros((C, NB), bf16)

    def pair(d, i):
        p = _PTS[i]
        if p == 1.0:
            ev = d[0] + d[2] + d[4]
            od = d[1] + d[3] + d[5]
        else:
            ev = d[0] + (p ** 2) * d[2] + (p ** 4) * d[4]
            od = p * d[1] + (p ** 3) * d[3] + (p ** 5) * d[5]
        return ev + od, ev - od

    def ext_rows(i, u_i, d_prev, d_last):
        p = _PTS[i]
        if p == 1.0:
            return d_prev + u_i - d_last
        if p == -1.0:
            return d_prev - u_i - d_last
        return d_prev + p * u_i - (p ** M) * d_last

    def transform(gi, zs=(0, 0, 0)):
        base = M * gi
        rhs = [xall[base + 1]]
        for i in range(1, M, 2):
            bz = base + zs[i // 2]
            d = [xall[bz + 1 + k].astype(f32) for k in range(M)]
            d_prev = xall[bz, CM:C, :].astype(f32)
            for k, u in enumerate(pair(d, i)):
                ext = ext_rows(i + k, u[CM:C], d_prev, d[M - 1][CM:C])
                rhs.append(jnp.concatenate([u, ext], axis=0).astype(bf16))
        rhs.append(xall[base + M, 0:CM, :])
        return rhs

    def transform0(kt):
        for c0 in range(krange(kt).start, krange(kt).stop, TCH):
            d = [xall[1 + i, c0:c0 + TCH, :].astype(f32) for i in range(M)]
            for i in range(1, M, 2):
                for k, u in enumerate(pair(d, i)):
                    u_scr[i + k, c0 // 2:(c0 + TCH) // 2, :] = pk(u.astype(bf16))
                    if c0 >= CM:
                        ext = ext_rows(i + k, u, xall[0, c0:c0 + TCH, :].astype(f32), d[M - 1])
                        u_scr[i + k, (c0 + CR) // 2:(c0 + CR + TCH) // 2, :] = pk(ext.astype(bf16))

    def weight_prep(kt):
        for d0 in range(0, C, 128):
            dn = min(128, C - d0)
            rows = slice(d0 // 2, (d0 + dn) // 2)
            if kt < KT - 1:
                g0, g1, g2 = [wbuf[2 - k, krange(kt), d0:d0 + dn].T for k in range(3)]
                wt_ref[NP - 1, kt, rows, :] = pk(g2)
                g2 = g2.astype(f32)
            else:
                g0r = wbuf[2, CM:C, d0:d0 + dn]
                g0 = jnp.concatenate([g0r, jnp.zeros_like(g0r)], axis=0).T
                g1 = jnp.concatenate([wbuf[1, CM:C, d0:d0 + dn], wbuf[0, CM:C, d0:d0 + dn]], axis=0).T
                g2 = None
            wt_ref[0, kt, rows, :] = pk(g0)
            scl = sc_ref[d0:d0 + dn, :]
            g0, g1 = g0.astype(f32) * scl, g1.astype(f32) * scl
            if g2 is not None:
                g2 = g2 * scl
            for i in range(1, M, 2):
                pt, den = _PTS[i], _den(i)
                ev = g0 * (1.0 / den)
                if g2 is not None:
                    ev = ev + g2 * (pt * pt / den)
                od = g1 * (pt / den)
                wt_ref[i, kt, rows, :] = pk((ev + od).astype(bf16))
                wt_ref[i + 1, kt, rows, :] = pk((ev - od).astype(bf16))

    def prod(i, rhs, r0, r1, kt0=0, kt1=KT):
        hi = min(kt1 * 128, k_rows[i])
        lhs = jnp.concatenate([upk(wt_ref[i, kt, r0 // 2:r1 // 2, :]) for kt in range(kt0, (hi + 127) // 128)],
                              axis=1)[:, :hi - kt0 * 128]
        return jnp.dot(lhs, rhs(kt0 * 128, hi), preferred_element_type=f32)

    def out_copy(slot, r0, r1):
        bt = jax.lax.shift_right_logical(slot * 1986, 16)
        s1 = slot - bt * TS

        @pl.when(s1 > 0)
        def _():
            pltpu.make_async_copy(oall.at[pl.ds(slot, 1), r0:r1],
                                  o_hbm.at[pl.ds(s1 - 1, 1), r0:r1, pl.ds(pl.multiple_of(bt * NB, NB), NB)],
                                  out_sem.at[0]).start()

    def epilogue(gi, m, carry, r0, r1, copy_out):
        def act(h, k):
            oall[M * gi + k, r0:r1, :] = (h * jnp.tanh(h) + h).astype(bf16)

        sc, sh, shx = sc_ref[r0:r1, :], sh_ref[r0:r1, :], shx_ref[r0:r1, :]
        m0 = m[0] * sc
        em0 = ee * m0
        sa, ta = m[1] + m[2], m[1] - m[2]
        s1, t1 = (m[3] + m[4]) + sh, (m[3] - m[4]) + sh
        sb, tb = m[5] + m[6], m[5] - m[6]
        o6 = ((s1 - m0) + sa) + sb
        o2 = ((s1 - em0) + b2 * sa) + a2 * sb
        o4 = ((shx - m0) + kap * s1) - o2 - o6
        q5 = (a * ta + t1) + b * tb
        q1 = (b * ta + t1) + a * tb
        q3 = (kap * t1 + shx) - q1 - q5
        if carry is not None:
            q1 = q1 + carry[1]
        m7 = m[7] * sc
        em7 = ee * m7
        if carry is not None:
            act(m0 + carry[0], 0)
        act(o2, 2)
        act(o4, 4)
        act(q1 - m7, 1)
        act(q3 + em7, 3)
        act(q5 - em7, 5)
        if copy_out:
            for k in range(M):
                out_copy(M * gi + k, r0, r1)
        return o6, m7

    def group(gi, rhs, carry, rows, copy_out):
        return [epilogue(gi, [prod(i, lambda lo, hi, v=rhs[i]: v, r0, r1) for i in range(NP)],
                         carry[h], r0, r1, copy_out)
                for h, (r0, r1) in enumerate(rows)]

    def save_carry(carry, rows):
        for h, (r0, r1) in enumerate(rows):
            c_scr[0, r0:r1, :] = carry[h][0]
            c_scr[1, r0:r1, :] = carry[h][1]

    for cp in p_copies:
        cp.wait()
    row = lambda r: r[...].astype(f32).reshape(1, C)
    scale = row(pg) * jax.lax.rsqrt(row(pv) + 1e-5)
    shift = row(pb) - row(pm) * scale
    sc_ref[...] = jnp.broadcast_to(0.5 * scale, (NB, C)).T
    sh_t = jnp.broadcast_to(0.5 * shift, (NB, C)).T
    sh_ref[...] = sh_t
    shx_ref[...] = (3.0 - kap) * sh_t

    def rhs0(i):
        if i == 0:
            return lambda lo, hi: xall[1, lo:hi, :]
        if i == NP - 1:
            return lambda lo, hi: xall[M, lo:hi, :]
        return lambda lo, hi: upk(u_scr[i, lo // 2:hi // 2, :])

    done = [0] * NP

    def advance(steps):
        acc = {}
        for i, kt1 in steps:
            part = prod(i, rhs0(i), 0, C, done[i], kt1)
            if i in acc:
                acc[i] = acc[i] + part
            else:
                acc[i] = part if done[i] == 0 else m_scr[i] + part
            done[i] = kt1
        for i, v in acc.items():
            m_scr[i] = v

    w_copies[0].wait()
    weight_prep(0)
    xa_copies[0].wait()
    transform0(0)
    advance([(i, 1) for i in SET_F])
    w_copies[1].wait()
    xa_copies[1].wait()
    weight_prep(1)
    transform0(1)
    advance([(i, 1) for i in SET_G] + [(i, 2) for i in SET_G])
    w_copies[2].wait()
    xa_copies[2].wait()
    weight_prep(2)
    transform0(2)
    advance([(i, 2) for i in SET_F] + [(i, 3) for i in SET_F])
    for kt in (3, 4):
        w_copies[kt].wait()
        xa_copies[kt].wait()
    for kt in (3, 4):
        weight_prep(kt)
        transform0(kt)
    advance([(i, 3) for i in SET_G] + [(i, 4) for i in SET_F])
    xb_copy.wait()
    cs = []
    for r0, r1 in ROWS:
        m = [m_scr[i, r0:r1, :] + prod(i, rhs0(i), r0, r1, done[i]) if done[i] * 128 < k_rows[i]
             else m_scr[i, r0:r1, :] for i in range(NP)]
        cs.append(epilogue(0, m, None, r0, r1, False))
    carry = [jnp.concatenate([c[k] for c in cs], axis=0) for k in range(2)]
    carry = [(carry[0][r0:r1], carry[1][r0:r1]) for r0, r1 in PRO_ROWS]
    carry = group(1, transform(1), carry, PRO_ROWS, False)
    xc_copy.wait()
    for gi in range(2, K_PRO):
        carry = group(gi, transform(gi), carry, PRO_ROWS, False)
    save_carry(carry, PRO_ROWS)

    (n_in,) = set(counts)

    def body(it, c):
        g0 = K_PRO + N_PER * it
        pltpu.make_async_copy(xall.at[0:n_in], xall.at[0:n_in], in_sem.at[it]).wait()

        @pl.when(it == 0)
        def _():
            for bt, s0, s1 in slot_ranges(0, M * K_PRO):
                pltpu.make_async_copy(oall.at[bt * TS + 1 + s0:bt * TS + 1 + s1],
                                      o_hbm.at[s0:s1, :, bt * NB:(bt + 1) * NB], out_sem.at[0]).start()

        zs = (0, jax.lax.shift_right_logical(it, 8), jax.lax.shift_right_logical(it, 9))
        carry = [(c_scr[0, r0:r1, :], c_scr[1, r0:r1, :]) for r0, r1 in ROWS]
        for r in range(N_PER):
            gi = g0 + r
            if r == N_PER - 1:
                full = [jnp.concatenate([c[k] for c in carry], axis=0) for k in range(2)]
                carry = [(full[0][r0:r1], full[1][r0:r1]) for r0, r1 in LAST_ROWS]
                carry = group(gi, transform(gi, zs), carry, LAST_ROWS, True)
            else:
                carry = group(gi, transform(gi, zs), carry, ROWS, True)
        save_carry(carry, LAST_ROWS)
        return c

    jax.lax.fori_loop(0, N_IT, body, 0)
    pltpu.make_async_copy(oall.at[0:NT * S], oall.at[0:NT * S], out_sem.at[0]).wait()


@jax.jit
def pallas_standalone__batchnorm__sampling_kernel(
    x: jax.Array,
    w: jax.Array,
    mean: jax.Array,
    var: jax.Array,
    g: jax.Array,
    b: jax.Array,
):
    B, S, C = x.shape
    assert (B, S, C) == (1024, 32, 576) and w.shape == (3, C, C)
    NT = B // NB
    KT = CM // 128 + 1
    n_it = (NT * (S + 1) // M - K_PRO) // N_PER
    xt = jnp.transpose(x, (1, 2, 0))
    ot = pl.pallas_call(
        _kernel,
        in_specs=[pl.BlockSpec(memory_space=pl.ANY)] * 6,
        out_specs=pl.BlockSpec(memory_space=pl.ANY),
        out_shape=jax.ShapeDtypeStruct((S, C, B), x.dtype),
        scratch_shapes=[pltpu.VMEM((NT * (S + 1) + 1, C, NB), jnp.bfloat16),
                        pltpu.VMEM((NT * (S + 1), C, NB), jnp.bfloat16),
                        pltpu.VMEM((3, C, C), jnp.bfloat16),
                        pltpu.VMEM((C,), jnp.bfloat16),
                        pltpu.VMEM((C,), jnp.bfloat16),
                        pltpu.VMEM((C,), jnp.bfloat16),
                        pltpu.VMEM((C,), jnp.bfloat16),
                        pltpu.VMEM((NP, KT, C // 2, 128), jnp.uint32),
                        pltpu.VMEM((C, NB), jnp.float32),
                        pltpu.VMEM((C, NB), jnp.float32),
                        pltpu.VMEM((C, NB), jnp.float32),
                        pltpu.VMEM((NP - 1, KT * 64, NB), jnp.uint32),
                        pltpu.VMEM((NP, C, NB), jnp.float32),
                        pltpu.VMEM((2, C, NB), jnp.float32),
                        pltpu.SemaphoreType.DMA((n_it,)),
                        pltpu.SemaphoreType.DMA((1,)),
                        pltpu.SemaphoreType.DMA((KT,)),
                        pltpu.SemaphoreType.DMA((KT,)),
                        pltpu.SemaphoreType.DMA((6,))],
        compiler_params=pltpu.CompilerParams(vmem_limit_bytes=110 * 1024 * 1024,
                                             disable_bounds_checks=True,
                                             disable_semaphore_checks=True),
    )(xt, w, mean, var, g, b)
    return jnp.transpose(ot, (2, 0, 1))
```

```python
import jax
import jax.numpy as jnp
import jax.experimental.pallas as pl
import jax.experimental.pallas.tpu as pltpu

NB = 128
PA = 0.4375
PB = 1.0 / PA
CM = 512
M = 6
NP = M + 2
K_PRO = 5
N_PER = 5
TCH = 32
ROWS = ((0, 432), (432, 576))
RAMP_ROWS = ((0, 432), (432, 576))
Z_ROWS = ((0, 240), (240, 288))
ZF_ROWS = ((0, 240), (240, 288))
PRO_ROWS = ((0, 496), (496, 576))
SET_F, SET_G = (0, 7, 1, 2), (3, 4, 5, 6)

_PTS = (0.0, PA, -PA, 1.0, -1.0, PB, -PB)


def _den(i):
    d = 1.0
    for j, q in enumerate(_PTS):
        if j != i:
            d *= (_PTS[i] - q)
    return d


def _kernel(x_hbm, w_hbm, mean_hbm, var_hbm, g_hbm, b_hbm, o_hbm,
            xall, oall, wbuf, pm, pv, pg, pb, wt_ref, sc_ref, sh_ref, shx_ref, u_scr, m_scr, c_scr,
            in_sem, out_sem, w_sem, xa_sem, misc_sem):
    S, C, B = x_hbm.shape
    NT = B // NB
    TS = S + 1
    NGT = NT * TS // M
    GB = 2 * TS // M
    N_IT = NT - 1
    HZ = C // 2
    KT = CM // 128 + 1
    CR = C - CM
    f32 = jnp.float32
    bf16 = jnp.bfloat16
    pk = lambda v: pltpu.bitcast(v, jnp.uint32)
    upk = lambda v: pltpu.bitcast(v, bf16)
    k_rows = (C,) + (CM + 128,) * M + (CM,)

    a, b = PA, PB
    a2, b2 = a * a, b * b
    ee = a2 + 1.0 + b2
    kap = 2.0 - a2 - b2

    def krange(kt):
        return slice(kt * 128, min(C, (kt + 1) * 128))

    def slot_ranges(lo, hi):
        out = []
        for bt in range(NT):
            a0, a1 = max(lo, bt * TS + 1), min(hi, (bt + 1) * TS)
            if a0 < a1:
                out.append((bt, a0 - bt * TS - 1, a1 - bt * TS - 1))
        return out

    def in_copies(lo, hi, sem):
        return [pltpu.make_async_copy(x_hbm.at[s0:s1, :, bt * NB:(bt + 1) * NB],
                                      xall.at[bt * TS + 1 + s0:bt * TS + 1 + s1], sem)
                for bt, s0, s1 in slot_ranges(lo, hi)]

    need = lambda g: M * (g + 1) + 1
    p_copies = [pltpu.make_async_copy(src, dst, misc_sem.at[2 + i])
                for i, (src, dst) in enumerate(((mean_hbm, pm), (var_hbm, pv), (g_hbm, pg), (b_hbm, pb)))]
    w_copies = [pltpu.make_async_copy(w_hbm.at[:, krange(kt), :], wbuf.at[:, krange(kt), :], w_sem.at[kt])
                for kt in range(KT)]
    xa_copies = [pltpu.make_async_copy(x_hbm.at[0:M, krange(kt), 0:NB], xall.at[1:M + 1, krange(kt), :],
                                       xa_sem.at[kt]) for kt in range(KT)]
    (xb_copy,) = in_copies(need(0), need(1), misc_sem.at[0])
    (xc_copy,) = in_copies(need(1), need(K_PRO - 1), misc_sem.at[1])
    for cp in p_copies + [c for wx in zip(w_copies, xa_copies) for c in wx] + [xb_copy, xc_copy]:
        cp.start()
    counts = []
    lo = need(K_PRO - 1)
    for it in range(N_IT):
        blk, j = (it + 1) // 2, (it + 1) % 2
        hi = need(GB * blk + N_PER * j + N_PER - 1 + j)
        for cp in in_copies(lo, hi, in_sem.at[it]):
            cp.start()
        counts.append(sum(s1 - s0 for _, s0, s1 in slot_ranges(lo, hi)))
        lo = hi

    for bt in range(NT + 1):
        xall[bt * TS] = jnp.zeros((C, NB), bf16)

    def pair(d, i):
        p = _PTS[i]
        if p == 1.0:
            ev = d[0] + d[2] + d[4]
            od = d[1] + d[3]
            if len(d) == M:
                od = od + d[5]
        else:
            ev = d[0] + (p ** 2) * d[2] + (p ** 4) * d[4]
            od = p * d[1] + (p ** 3) * d[3]
            if len(d) == M:
                od = od + (p ** 5) * d[5]
        return ev + od, ev - od

    def ext_rows(i, u_i, d_prev, d_last):
        p = _PTS[i]
        if d_last is None:
            return d_prev + p * u_i
        if p == 1.0:
            return d_prev + u_i - d_last
        if p == -1.0:
            return d_prev - u_i - d_last
        return d_prev + p * u_i - (p ** M) * d_last

    def transform(gi, zs=(0, 0, 0), short=False):
        base = M * gi
        rhs = [xall[base + 1]]
        for i in range(1, M, 2):
            bz = base + zs[i // 2]
            d = [xall[bz + 1 + k].astype(f32) for k in range(M - short)]
            d_prev = xall[bz, CM:C, :].astype(f32)
            for k, u in enumerate(pair(d, i)):
                ext = ext_rows(i + k, u[CM:C], d_prev, None if short else d[M - 1][CM:C])
                rhs.append(jnp.concatenate([u, ext], axis=0).astype(bf16))
        if not short:
            rhs.append(xall[base + M, 0:CM, :])
        return rhs

    def transform0(kt):
        for c0 in range(krange(kt).start, krange(kt).stop, TCH):
            d = [xall[1 + i, c0:c0 + TCH, :].astype(f32) for i in range(M)]
            for i in range(1, M, 2):
                for k, u in enumerate(pair(d, i)):
                    u_scr[i + k, c0 // 2:(c0 + TCH) // 2, :] = pk(u.astype(bf16))
                    if c0 >= CM:
                        ext = ext_rows(i + k, u, xall[0, c0:c0 + TCH, :].astype(f32), d[M - 1])
                        u_scr[i + k, (c0 + CR) // 2:(c0 + CR + TCH) // 2, :] = pk(ext.astype(bf16))

    def weight_prep(kt):
        for d0 in range(0, C, 128):
            dn = min(128, C - d0)
            rows = slice(d0 // 2, (d0 + dn) // 2)
            if kt < KT - 1:
                g0, g1, g2 = [wbuf[2 - k, krange(kt), d0:d0 + dn].T for k in range(3)]
                wt_ref[NP - 1, kt, rows, :] = pk(g2)
                g2 = g2.astype(f32)
            else:
                g0r = wbuf[2, CM:C, d0:d0 + dn]
                g0 = jnp.concatenate([g0r, jnp.zeros_like(g0r)], axis=0).T
                g1 = jnp.concatenate([wbuf[1, CM:C, d0:d0 + dn], wbuf[0, CM:C, d0:d0 + dn]], axis=0).T
                g2 = None
            wt_ref[0, kt, rows, :] = pk(g0)
            scl = sc_ref[d0:d0 + dn, :]
            g0, g1 = g0.astype(f32) * scl, g1.astype(f32) * scl
            if g2 is not None:
                g2 = g2 * scl
            for i in range(1, M, 2):
                pt, den = _PTS[i], _den(i)
                ev = g0 * (1.0 / den)
                if g2 is not None:
                    ev = ev + g2 * (pt * pt / den)
                od = g1 * (pt / den)
                wt_ref[i, kt, rows, :] = pk((ev + od).astype(bf16))
                wt_ref[i + 1, kt, rows, :] = pk((ev - od).astype(bf16))

    def rows_of(r0, r1, off=None, div=1):
        if off is None:
            return pl.ds(r0 // div, (r1 - r0) // div)
        return pl.ds(pl.multiple_of(off * (HZ // div) + r0 // div, 16 // div), (r1 - r0) // div)

    def pick(ref, r0, r1, off, div=1):
        if off is None:
            return ref[r0 // div:r1 // div, :]
        return jnp.where(off == 0, ref[r0 // div:r1 // div, :], ref[(HZ + r0) // div:(HZ + r1) // div, :])

    def prod(i, rhs, r0, r1, kt0=0, kt1=KT, off=None):
        hi = min(kt1 * 128, k_rows[i])
        lhs = jnp.concatenate([upk(pick(wt_ref.at[i, kt], r0, r1, off, 2)) for kt in range(kt0, (hi + 127) // 128)],
                              axis=1)[:, :hi - kt0 * 128]
        return jnp.dot(lhs, rhs(kt0 * 128, hi), preferred_element_type=f32)

    def out_copy(slot, rs):
        if isinstance(slot, int):
            bt, s1 = slot // TS, slot % TS
            pltpu.make_async_copy(oall.at[pl.ds(slot, 1), rs], o_hbm.at[pl.ds(s1 - 1, 1), rs, pl.ds(bt * NB, NB)],
                                  out_sem.at[0]).start()
            return
        bt = jax.lax.shift_right_logical(slot * 1986, 16)
        s1 = slot - bt * TS

        @pl.when(s1 > 0)
        def _():
            pltpu.make_async_copy(oall.at[pl.ds(slot, 1), rs],
                                  o_hbm.at[pl.ds(s1 - 1, 1), rs, pl.ds(pl.multiple_of(bt * NB, NB), NB)],
                                  out_sem.at[0]).start()

    def epilogue(gi, m, carry, r0, r1, copy_out, off=None):
        rs = rows_of(r0, r1, off)

        def act(h, k):
            oall[M * gi + k, rs, :] = (h * jnp.tanh(h) + h).astype(bf16)

        sc, sh, shx = [pick(ref, r0, r1, off) for ref in (sc_ref, sh_ref, shx_ref)]
        m0 = m[0] * sc
        em0 = ee * m0
        sa, ta = m[1] + m[2], m[1] - m[2]
        s1, t1 = (m[3] + m[4]) + sh, (m[3] - m[4]) + sh
        sb, tb = m[5] + m[6], m[5] - m[6]
        o6 = ((s1 - m0) + sa) + sb
        o2 = ((s1 - em0) + b2 * sa) + a2 * sb
        o4 = ((shx - m0) + kap * s1) - o2 - o6
        q5 = (a * ta + t1) + b * tb
        q1 = (b * ta + t1) + a * tb
        q3 = (kap * t1 + shx) - q1 - q5
        if isinstance(carry, str):
            for h, k in ((o2, 2), (o4, 4), (q3, 3), (q5, 5)):
                act(h, k)
            for k in range(2, M):
                out_copy(M * gi + k, rs)

            def finish(c0, c1):
                act(m0 + c0, 0)
                act(q1 + c1, 1)
                out_copy(M * gi, rs)
                out_copy(M * gi + 1, rs)
            return finish
        if carry is not None:
            q1 = q1 + carry[1]
        m7 = None
        if len(m) == NP:
            m7 = m[7] * sc
            em7 = ee * m7
            q1, q3, q5 = q1 - m7, q3 + em7, q5 - em7
        if carry is not None:
            act(m0 + carry[0], 0)
        act(o2, 2)
        act(o4, 4)
        act(q1, 1)
        act(q3, 3)
        act(q5, 5)
        if copy_out:
            for k in range(M):
                out_copy(M * gi + k, rs)
        return o6, m7

    def group(gi, rhs, carry, rows, copy_out, after_first=None):
        out = []
        for h, (r0, r1) in enumerate(rows):
            out.append(epilogue(gi, [prod(i, lambda lo, hi, v=rhs[i]: v, r0, r1) for i in range(NP)],
                                carry[h], r0, r1, copy_out))
            if h == 0 and after_first is not None:
                after_first(out[0])
        return out

    def short_half(gi, zs, off, rows, carry):
        rhs = transform(gi, zs, True)
        return [epilogue(gi, [prod(i, lambda lo, hi, v=rhs[i]: v, r0, r1, off=off) for i in range(NP - 1)],
                         carry(r0, r1), r0, r1, True, off) for r0, r1 in rows]

    def save_carry(carry, rows):
        for h, (r0, r1) in enumerate(rows):
            c_scr[0, r0:r1, :] = carry[h][0]
            c_scr[1, r0:r1, :] = carry[h][1]

    for cp in p_copies:
        cp.wait()
    row = lambda r: r[...].astype(f32).reshape(1, C)
    scale = row(pg) * jax.lax.rsqrt(row(pv) + 1e-5)
    shift = row(pb) - row(pm) * scale
    sc_ref[...] = jnp.broadcast_to(0.5 * scale, (NB, C)).T
    sh_t = jnp.broadcast_to(0.5 * shift, (NB, C)).T
    sh_ref[...] = sh_t
    shx_ref[...] = (3.0 - kap) * sh_t

    def rhs0(i):
        if i == 0:
            return lambda lo, hi: xall[1, lo:hi, :]
        if i == NP - 1:
            return lambda lo, hi: xall[M, lo:hi, :]
        return lambda lo, hi: upk(u_scr[i, lo // 2:hi // 2, :])

    done = [0] * NP

    def advance(steps):
        acc = {}
        for i, kt1 in steps:
            part = prod(i, rhs0(i), 0, C, done[i], kt1)
            if i in acc:
                acc[i] = acc[i] + part
            else:
                acc[i] = part if done[i] == 0 else m_scr[i] + part
            done[i] = kt1
        for i, v in acc.items():
            m_scr[i] = v

    w_copies[0].wait()
    weight_prep(0)
    xa_copies[0].wait()
    transform0(0)
    advance([(i, 1) for i in SET_F])
    w_copies[1].wait()
    xa_copies[1].wait()
    weight_prep(1)
    transform0(1)
    advance([(i, 1) for i in SET_G] + [(i, 2) for i in SET_G])
    w_copies[2].wait()
    xa_copies[2].wait()
    weight_prep(2)
    transform0(2)
    advance([(i, 2) for i in SET_F] + [(i, 3) for i in SET_F])
    for kt in (3, 4):
        w_copies[kt].wait()
        xa_copies[kt].wait()
    for kt in (3, 4):
        weight_prep(kt)
        transform0(kt)
    advance([(i, 3) for i in SET_G] + [(i, 4) for i in SET_F])
    xb_copy.wait()
    cs = []
    for r0, r1 in ROWS:
        m = [m_scr[i, r0:r1, :] + prod(i, rhs0(i), r0, r1, done[i]) if done[i] * 128 < k_rows[i]
             else m_scr[i, r0:r1, :] for i in range(NP)]
        cs.append(epilogue(0, m, None, r0, r1, False))
    carry = [jnp.concatenate([c[k] for c in cs], axis=0) for k in range(2)]
    carry = [(carry[0][r0:r1], carry[1][r0:r1]) for r0, r1 in PRO_ROWS]
    carry = group(1, transform(1), carry, PRO_ROWS, False)
    save_carry(carry, PRO_ROWS)
    xc_copy.wait()

    def ramp(gi, c):
        zs = (0, jax.lax.shift_right_logical(gi, 8), jax.lax.shift_right_logical(gi, 9))
        carry = [(c_scr[0, r0:r1, :], c_scr[1, r0:r1, :]) for r0, r1 in RAMP_ROWS]
        save_carry(group(gi, transform(gi, zs), carry, RAMP_ROWS, False), RAMP_ROWS)
        return c

    jax.lax.fori_loop(2, K_PRO, ramp, 0)

    n_lo, n_hi = min(counts), max(counts)

    def body(it, c):
        blk = jax.lax.shift_right_logical(it + 1, 1)
        j = jnp.bitwise_and(it + 1, 1)
        g0 = GB * blk + N_PER * j
        pltpu.make_async_copy(xall.at[0:n_lo], xall.at[0:n_lo], in_sem.at[it]).wait()

        @pl.when(j == 1)
        def _():
            pltpu.make_async_copy(xall.at[0:n_hi - n_lo], xall.at[0:n_hi - n_lo], in_sem.at[it]).wait()

        @pl.when(it == 0)
        def _():
            for bt, s0, s1 in slot_ranges(0, M * K_PRO):
                pltpu.make_async_copy(oall.at[bt * TS + 1 + s0:bt * TS + 1 + s1],
                                      o_hbm.at[s0:s1, :, bt * NB:(bt + 1) * NB], out_sem.at[0]).start()

        zs = (0, jax.lax.shift_right_logical(it, 8), jax.lax.shift_right_logical(it, 9))
        second = j == 1
        fin = short_half(GB * (blk + j) - 1, zs, 1 - j, Z_ROWS, lambda r0, r1: "later")
        c_in = [c_scr[k, HZ:C, :] for k in range(2)]
        carry = [(c_scr[0, r0:r1, :], jnp.where(second, c_scr[1, r0:r1, :], 0.0)) for r0, r1 in ROWS]

        def finish_short(c_out):
            for f, (r0, r1) in zip(fin, Z_ROWS):
                f(*[jnp.where(second, c_out[k][r0:r1], c_in[k][r0:r1]) for k in range(2)])

        for r in range(N_PER):
            gi = g0 + r
            carry = group(gi, transform(gi, zs), carry, ROWS, True, finish_short if r == N_PER - 1 else None)
        save_carry(carry, ROWS)
        return c

    jax.lax.fori_loop(0, N_IT, body, 0)
    short_half(NGT - 1, (0, 0, 0), None, [(HZ + r0, HZ + r1) for r0, r1 in ZF_ROWS],
               lambda r0, r1: (c_scr[0, r0:r1, :], c_scr[1, r0:r1, :]))
    pltpu.make_async_copy(oall.at[0:NT * S], oall.at[0:NT * S], out_sem.at[0]).wait()


@jax.jit
def pallas_standalone__batchnorm__sampling_kernel(
    x: jax.Array,
    w: jax.Array,
    mean: jax.Array,
    var: jax.Array,
    g: jax.Array,
    b: jax.Array,
):
    B, S, C = x.shape
    assert (B, S, C) == (1024, 32, 576) and w.shape == (3, C, C)
    NT = B // NB
    KT = CM // 128 + 1
    n_it = NT - 1
    xt = jnp.transpose(x, (1, 2, 0))
    ot = pl.pallas_call(
        _kernel,
        in_specs=[pl.BlockSpec(memory_space=pl.ANY)] * 6,
        out_specs=pl.BlockSpec(memory_space=pl.ANY),
        out_shape=jax.ShapeDtypeStruct((S, C, B), x.dtype),
        scratch_shapes=[pltpu.VMEM((NT * (S + 1) + 1, C, NB), jnp.bfloat16),
                        pltpu.VMEM((NT * (S + 1), C, NB), jnp.bfloat16),
                        pltpu.VMEM((3, C, C), jnp.bfloat16),
                        pltpu.VMEM((C,), jnp.bfloat16),
                        pltpu.VMEM((C,), jnp.bfloat16),
                        pltpu.VMEM((C,), jnp.bfloat16),
                        pltpu.VMEM((C,), jnp.bfloat16),
                        pltpu.VMEM((NP, KT, C // 2, 128), jnp.uint32),
                        pltpu.VMEM((C, NB), jnp.float32),
                        pltpu.VMEM((C, NB), jnp.float32),
                        pltpu.VMEM((C, NB), jnp.float32),
                        pltpu.VMEM((NP - 1, KT * 64, NB), jnp.uint32),
                        pltpu.VMEM((NP, C, NB), jnp.float32),
                        pltpu.VMEM((2, C, NB), jnp.float32),
                        pltpu.SemaphoreType.DMA((n_it,)),
                        pltpu.SemaphoreType.DMA((1,)),
                        pltpu.SemaphoreType.DMA((KT,)),
                        pltpu.SemaphoreType.DMA((KT,)),
                        pltpu.SemaphoreType.DMA((6,))],
        compiler_params=pltpu.CompilerParams(vmem_limit_bytes=110 * 1024 * 1024,
                                             disable_bounds_checks=True,
                                             disable_semaphore_checks=True),
    )(xt, w, mean, var, g, b)
    return jnp.transpose(ot, (2, 0, 1))
```

```python
import jax
import jax.numpy as jnp
import jax.experimental.pallas as pl
import jax.experimental.pallas.tpu as pltpu

NB = 128
PA = 0.4375
PB = 1.0 / PA
CM = 512
M = 6
NP = M + 2
K_PRO = 5
N_PER = 5
TCH = 32
ROWS = ((0, 432), (432, 576))
PRO_ROWS = ((0, 496), (496, 576))
Z_ROWS = ((0, 240), (240, 288))
ZF_ROWS = ((0, 160), (160, 240), (240, 288))
SET_F, SET_G = (0, 7, 1, 2), (3, 4, 5, 6)

_PTS = (0.0, PA, -PA, 1.0, -1.0, PB, -PB)


def _den(i):
    d = 1.0
    for j, q in enumerate(_PTS):
        if j != i:
            d *= (_PTS[i] - q)
    return d


def _kernel(x_hbm, w_hbm, mean_hbm, var_hbm, g_hbm, b_hbm, o_hbm,
            xall, oall, wbuf, pm, pv, pg, pb, wt_ref, sc_ref, sh_ref, shx_ref, u_scr, m_scr, c_scr,
            in_sem, out_sem, w_sem, xa_sem, misc_sem):
    S, C, B = x_hbm.shape
    NT = B // NB
    TS = S + 1
    NGT = NT * TS // M
    GB = 2 * TS // M
    N_IT = NT - 1
    HZ = C // 2
    KT = CM // 128 + 1
    CR = C - CM
    f32 = jnp.float32
    bf16 = jnp.bfloat16
    pk = lambda v: pltpu.bitcast(v, jnp.uint32)
    upk = lambda v: pltpu.bitcast(v, bf16)
    k_rows = (C,) + (CM + 128,) * M + (CM,)

    a, b = PA, PB
    a2, b2 = a * a, b * b
    ee = a2 + 1.0 + b2
    kap = 2.0 - a2 - b2

    def krange(kt):
        return slice(kt * 128, min(C, (kt + 1) * 128))

    def slot_ranges(lo, hi):
        out = []
        for bt in range(NT):
            a0, a1 = max(lo, bt * TS + 1), min(hi, (bt + 1) * TS)
            if a0 < a1:
                out.append((bt, a0 - bt * TS - 1, a1 - bt * TS - 1))
        return out

    def in_copies(lo, hi, sem):
        return [pltpu.make_async_copy(x_hbm.at[s0:s1, :, bt * NB:(bt + 1) * NB],
                                      xall.at[bt * TS + 1 + s0:bt * TS + 1 + s1], sem)
                for bt, s0, s1 in slot_ranges(lo, hi)]

    need = lambda g: M * (g + 1) + 1
    p_copies = [pltpu.make_async_copy(src, dst, misc_sem.at[2 + i])
                for i, (src, dst) in enumerate(((mean_hbm, pm), (var_hbm, pv), (g_hbm, pg), (b_hbm, pb)))]
    w_copies = [pltpu.make_async_copy(w_hbm.at[:, krange(kt), :], wbuf.at[:, krange(kt), :], w_sem.at[kt])
                for kt in range(KT)]
    xa_copies = [pltpu.make_async_copy(x_hbm.at[0:M, krange(kt), 0:NB], xall.at[1:M + 1, krange(kt), :],
                                       xa_sem.at[kt]) for kt in range(KT)]
    (xb_copy,) = in_copies(need(0), need(1), misc_sem.at[0])
    (xc_copy,) = in_copies(need(1), need(K_PRO - 1), misc_sem.at[1])
    for cp in p_copies + [c for wx in zip(w_copies, xa_copies) for c in wx] + [xb_copy, xc_copy]:
        cp.start()
    counts = []
    lo = need(K_PRO - 1)
    for it in range(N_IT):
        blk, j = (it + 1) // 2, (it + 1) % 2
        hi = need(GB * blk + N_PER * j + N_PER - 1 + j)
        for cp in in_copies(lo, hi, in_sem.at[it]):
            cp.start()
        counts.append(sum(s1 - s0 for _, s0, s1 in slot_ranges(lo, hi)))
        lo = hi

    for bt in range(NT + 1):
        xall[bt * TS] = jnp.zeros((C, NB), bf16)

    def pair(d, i):
        p = _PTS[i]
        if p == 1.0:
            ev = d[0] + d[2] + d[4]
            od = d[1] + d[3]
            if len(d) == M:
                od = od + d[5]
        else:
            ev = d[0] + (p ** 2) * d[2] + (p ** 4) * d[4]
            od = p * d[1] + (p ** 3) * d[3]
            if len(d) == M:
                od = od + (p ** 5) * d[5]
        return ev + od, ev - od

    def ext_rows(i, u_i, d_prev, d_last):
        p = _PTS[i]
        if d_last is None:
            return d_prev + p * u_i
        if p == 1.0:
            return d_prev + u_i - d_last
        if p == -1.0:
            return d_prev - u_i - d_last
        return d_prev + p * u_i - (p ** M) * d_last

    def transform(gi, zs=(0, 0, 0), short=False):
        base = M * gi
        rhs = [xall[base + 1]]
        for i in range(1, M, 2):
            bz = base + zs[i // 2]
            d = [xall[bz + 1 + k].astype(f32) for k in range(M - short)]
            d_prev = xall[bz, CM:C, :].astype(f32)
            for k, u in enumerate(pair(d, i)):
                ext = ext_rows(i + k, u[CM:C], d_prev, None if short else d[M - 1][CM:C])
                rhs.append(jnp.concatenate([u, ext], axis=0).astype(bf16))
        if not short:
            rhs.append(xall[base + M, 0:CM, :])
        return rhs

    def transform0(kt):
        for c0 in range(krange(kt).start, krange(kt).stop, TCH):
            d = [xall[1 + i, c0:c0 + TCH, :].astype(f32) for i in range(M)]
            for i in range(1, M, 2):
                for k, u in enumerate(pair(d, i)):
                    u_scr[i + k, c0 // 2:(c0 + TCH) // 2, :] = pk(u.astype(bf16))
                    if c0 >= CM:
                        ext = ext_rows(i + k, u, xall[0, c0:c0 + TCH, :].astype(f32), d[M - 1])
                        u_scr[i + k, (c0 + CR) // 2:(c0 + CR + TCH) // 2, :] = pk(ext.astype(bf16))

    def weight_prep(kt):
        for d0 in range(0, C, 128):
            dn = min(128, C - d0)
            rows = slice(d0 // 2, (d0 + dn) // 2)
            if kt < KT - 1:
                g0, g1, g2 = [wbuf[2 - k, krange(kt), d0:d0 + dn].T for k in range(3)]
                wt_ref[NP - 1, kt, rows, :] = pk(g2)
                g2 = g2.astype(f32)
            else:
                g0r = wbuf[2, CM:C, d0:d0 + dn]
                g0 = jnp.concatenate([g0r, jnp.zeros_like(g0r)], axis=0).T
                g1 = jnp.concatenate([wbuf[1, CM:C, d0:d0 + dn], wbuf[0, CM:C, d0:d0 + dn]], axis=0).T
                g2 = None
            wt_ref[0, kt, rows, :] = pk(g0)
            scl = sc_ref[d0:d0 + dn, :]
            g0, g1 = g0.astype(f32) * scl, g1.astype(f32) * scl
            if g2 is not None:
                g2 = g2 * scl
            for i in range(1, M, 2):
                pt, den = _PTS[i], _den(i)
                ev = g0 * (1.0 / den)
                if g2 is not None:
                    ev = ev + g2 * (pt * pt / den)
                od = g1 * (pt / den)
                wt_ref[i, kt, rows, :] = pk((ev + od).astype(bf16))
                wt_ref[i + 1, kt, rows, :] = pk((ev - od).astype(bf16))

    def rows_of(r0, r1, off):
        if off is None:
            return pl.ds(r0, r1 - r0)
        return pl.ds(pl.multiple_of(off * HZ + r0, 16), r1 - r0)

    def pick(ref, r0, r1, off, div=1):
        if off is None:
            return ref[r0 // div:r1 // div, :]
        return jnp.where(off == 0, ref[r0 // div:r1 // div, :], ref[(HZ + r0) // div:(HZ + r1) // div, :])

    def prod(i, rhs, r0, r1, kt0=0, kt1=KT, off=None):
        hi = min(kt1 * 128, k_rows[i])
        lhs = jnp.concatenate([upk(pick(wt_ref.at[i, kt], r0, r1, off, 2)) for kt in range(kt0, (hi + 127) // 128)],
                              axis=1)[:, :hi - kt0 * 128]
        return jnp.dot(lhs, rhs(kt0 * 128, hi), preferred_element_type=f32)

    def out_copy(slot, rs):
        if isinstance(slot, int):
            bt, s1 = slot // TS, slot % TS
            pltpu.make_async_copy(oall.at[pl.ds(slot, 1), rs], o_hbm.at[pl.ds(s1 - 1, 1), rs, pl.ds(bt * NB, NB)],
                                  out_sem.at[0]).start()
            return
        bt = jax.lax.shift_right_logical(slot * 1986, 16)
        s1 = slot - bt * TS

        @pl.when(s1 > 0)
        def _():
            pltpu.make_async_copy(oall.at[pl.ds(slot, 1), rs],
                                  o_hbm.at[pl.ds(s1 - 1, 1), rs, pl.ds(pl.multiple_of(bt * NB, NB), NB)],
                                  out_sem.at[0]).start()

    def epilogue(gi, m, carry, r0, r1, copy_out, off=None):
        rs = rows_of(r0, r1, off)

        def act(h, k):
            oall[M * gi + k, rs, :] = (h * jnp.tanh(h) + h).astype(bf16)

        sc, sh, shx = [pick(ref, r0, r1, off) for ref in (sc_ref, sh_ref, shx_ref)]
        m0 = m[0] * sc
        em0 = ee * m0
        sa, ta = m[1] + m[2], m[1] - m[2]
        s1, t1 = (m[3] + m[4]) + sh, (m[3] - m[4]) + sh
        sb, tb = m[5] + m[6], m[5] - m[6]
        o6 = ((s1 - m0) + sa) + sb
        o2 = ((s1 - em0) + b2 * sa) + a2 * sb
        o4 = ((shx - m0) + kap * s1) - o2 - o6
        q5 = (a * ta + t1) + b * tb
        q1 = (b * ta + t1) + a * tb
        q3 = (kap * t1 + shx) - q1 - q5
        if isinstance(carry, str):
            for h, k in ((o2, 2), (o4, 4), (q3, 3), (q5, 5)):
                act(h, k)
            for k in range(2, M):
                out_copy(M * gi + k, rs)

            def finish(c0, c1):
                act(m0 + c0, 0)
                act(q1 + c1, 1)
                out_copy(M * gi, rs)
                out_copy(M * gi + 1, rs)
            return finish
        if carry is not None:
            q1 = q1 + carry[1]
        m7 = None
        if len(m) == NP:
            m7 = m[7] * sc
            em7 = ee * m7
            q1, q3, q5 = q1 - m7, q3 + em7, q5 - em7
        if carry is not None:
            act(m0 + carry[0], 0)
        act(o2, 2)
        act(o4, 4)
        act(q1, 1)
        act(q3, 3)
        act(q5, 5)
        if copy_out:
            for k in range(M):
                out_copy(M * gi + k, rs)
        return o6, m7

    def group(gi, rhs, carry, rows, copy_out, after_first=None):
        out = []
        for h, (r0, r1) in enumerate(rows):
            out.append(epilogue(gi, [prod(i, lambda lo, hi, v=rhs[i]: v, r0, r1) for i in range(NP)],
                                carry[h], r0, r1, copy_out))
            if h == 0 and after_first is not None:
                after_first(out[0])
        return out

    def short_half(gi, zs, off, rows, carry):
        rhs = transform(gi, zs, True)
        return [epilogue(gi, [prod(i, lambda lo, hi, v=rhs[i]: v, r0, r1, off=off) for i in range(NP - 1)],
                         carry(r0, r1), r0, r1, True, off) for r0, r1 in rows]

    def save_carry(carry, rows):
        for h, (r0, r1) in enumerate(rows):
            c_scr[0, r0:r1, :] = carry[h][0]
            c_scr[1, r0:r1, :] = carry[h][1]

    for cp in p_copies:
        cp.wait()
    row = lambda r: r[...].astype(f32).reshape(1, C)
    scale = row(pg) * jax.lax.rsqrt(row(pv) + 1e-5)
    shift = row(pb) - row(pm) * scale
    sc_ref[...] = jnp.broadcast_to(0.5 * scale, (NB, C)).T
    sh_t = jnp.broadcast_to(0.5 * shift, (NB, C)).T
    sh_ref[...] = sh_t
    shx_ref[...] = (3.0 - kap) * sh_t

    def rhs0(i):
        if i == 0:
            return lambda lo, hi: xall[1, lo:hi, :]
        if i == NP - 1:
            return lambda lo, hi: xall[M, lo:hi, :]
        return lambda lo, hi: upk(u_scr[i, lo // 2:hi // 2, :])

    done = [0] * NP

    def advance(steps):
        acc = {}
        for i, kt1 in steps:
            part = prod(i, rhs0(i), 0, C, done[i], kt1)
            if i in acc:
                acc[i] = acc[i] + part
            else:
                acc[i] = part if done[i] == 0 else m_scr[i] + part
            done[i] = kt1
        for i, v in acc.items():
            m_scr[i] = v

    w_copies[0].wait()
    weight_prep(0)
    xa_copies[0].wait()
    transform0(0)
    advance([(i, 1) for i in SET_F])
    w_copies[1].wait()
    xa_copies[1].wait()
    weight_prep(1)
    transform0(1)
    advance([(i, 1) for i in SET_G] + [(i, 2) for i in SET_G])
    w_copies[2].wait()
    xa_copies[2].wait()
    weight_prep(2)
    transform0(2)
    advance([(i, 2) for i in SET_F] + [(i, 3) for i in SET_F])
    for kt in (3, 4):
        w_copies[kt].wait()
        xa_copies[kt].wait()
    for kt in (3, 4):
        weight_prep(kt)
        transform0(kt)
    advance([(i, 3) for i in SET_G] + [(i, 4) for i in SET_F])
    xb_copy.wait()
    cs = []
    for r0, r1 in ROWS:
        m = [m_scr[i, r0:r1, :] + prod(i, rhs0(i), r0, r1, done[i]) if done[i] * 128 < k_rows[i]
             else m_scr[i, r0:r1, :] for i in range(NP)]
        cs.append(epilogue(0, m, None, r0, r1, False))
    carry = [jnp.concatenate([c[k] for c in cs], axis=0) for k in range(2)]
    carry = [(carry[0][r0:r1], carry[1][r0:r1]) for r0, r1 in PRO_ROWS]
    carry = group(1, transform(1), carry, PRO_ROWS, False)
    save_carry(carry, PRO_ROWS)
    xc_copy.wait()

    def ramp(gi, c):
        zs = (0, jax.lax.shift_right_logical(gi, 8), jax.lax.shift_right_logical(gi, 9))
        carry = [(c_scr[0, r0:r1, :], c_scr[1, r0:r1, :]) for r0, r1 in ROWS]
        save_carry(group(gi, transform(gi, zs), carry, ROWS, False), ROWS)
        return c

    jax.lax.fori_loop(2, K_PRO, ramp, 0)

    n_lo, n_hi = min(counts), max(counts)

    def body(it, c):
        blk = jax.lax.shift_right_logical(it + 1, 1)
        j = jnp.bitwise_and(it + 1, 1)
        g0 = GB * blk + N_PER * j
        pltpu.make_async_copy(xall.at[0:n_lo], xall.at[0:n_lo], in_sem.at[it]).wait()

        @pl.when(j == 1)
        def _():
            pltpu.make_async_copy(xall.at[0:n_hi - n_lo], xall.at[0:n_hi - n_lo], in_sem.at[it]).wait()

        @pl.when(it == 0)
        def _():
            for bt, s0, s1 in slot_ranges(0, M * K_PRO):
                pltpu.make_async_copy(oall.at[bt * TS + 1 + s0:bt * TS + 1 + s1],
                                      o_hbm.at[s0:s1, :, bt * NB:(bt + 1) * NB], out_sem.at[0]).start()

        zs = (0, jax.lax.shift_right_logical(it, 8), jax.lax.shift_right_logical(it, 9))
        second = j == 1
        fin = short_half(GB * (blk + j) - 1, zs, 1 - j, Z_ROWS, lambda r0, r1: "later")
        c_in = [c_scr[k, HZ:C, :] for k in range(2)]
        carry = [(c_scr[0, r0:r1, :], jnp.where(second, c_scr[1, r0:r1, :], 0.0)) for r0, r1 in ROWS]

        def finish_short(c_out):
            for f, (r0, r1) in zip(fin, Z_ROWS):
                f(*[jnp.where(second, c_out[k][r0:r1], c_in[k][r0:r1]) for k in range(2)])

        for r in range(N_PER):
            gi = g0 + r
            carry = group(gi, transform(gi, zs), carry, ROWS, True, finish_short if r == N_PER - 1 else None)
        save_carry(carry, ROWS)
        return c

    jax.lax.fori_loop(0, N_IT, body, 0)
    short_half(NGT - 1, (0, 0, 0), None, [(HZ + r0, HZ + r1) for r0, r1 in ZF_ROWS],
               lambda r0, r1: (c_scr[0, r0:r1, :], c_scr[1, r0:r1, :]))
    pltpu.make_async_copy(oall.at[0:NT * S], oall.at[0:NT * S], out_sem.at[0]).wait()


@jax.jit
def pallas_standalone__batchnorm__sampling_kernel(
    x: jax.Array,
    w: jax.Array,
    mean: jax.Array,
    var: jax.Array,
    g: jax.Array,
    b: jax.Array,
):
    B, S, C = x.shape
    assert (B, S, C) == (1024, 32, 576) and w.shape == (3, C, C)
    NT = B // NB
    KT = CM // 128 + 1
    n_it = NT - 1
    xt = jnp.transpose(x, (1, 2, 0))
    ot = pl.pallas_call(
        _kernel,
        in_specs=[pl.BlockSpec(memory_space=pl.ANY)] * 6,
        out_specs=pl.BlockSpec(memory_space=pl.ANY),
        out_shape=jax.ShapeDtypeStruct((S, C, B), x.dtype),
        scratch_shapes=[pltpu.VMEM((NT * (S + 1) + 1, C, NB), jnp.bfloat16),
                        pltpu.VMEM((NT * (S + 1), C, NB), jnp.bfloat16),
                        pltpu.VMEM((3, C, C), jnp.bfloat16),
                        pltpu.VMEM((C,), jnp.bfloat16),
                        pltpu.VMEM((C,), jnp.bfloat16),
                        pltpu.VMEM((C,), jnp.bfloat16),
                        pltpu.VMEM((C,), jnp.bfloat16),
                        pltpu.VMEM((NP, KT, C // 2, 128), jnp.uint32),
                        pltpu.VMEM((C, NB), jnp.float32),
                        pltpu.VMEM((C, NB), jnp.float32),
                        pltpu.VMEM((C, NB), jnp.float32),
                        pltpu.VMEM((NP - 1, KT * 64, NB), jnp.uint32),
                        pltpu.VMEM((NP, C, NB), jnp.float32),
                        pltpu.VMEM((2, C, NB), jnp.float32),
                        pltpu.SemaphoreType.DMA((n_it,)),
                        pltpu.SemaphoreType.DMA((1,)),
                        pltpu.SemaphoreType.DMA((KT,)),
                        pltpu.SemaphoreType.DMA((KT,)),
                        pltpu.SemaphoreType.DMA((6,))],
        compiler_params=pltpu.CompilerParams(vmem_limit_bytes=110 * 1024 * 1024,
                                             disable_bounds_checks=True,
                                             disable_semaphore_checks=True),
    )(xt, w, mean, var, g, b)
    return jnp.transpose(ot, (2, 0, 1))
```

```python
import jax
import jax.numpy as jnp
import jax.experimental.pallas as pl
import jax.experimental.pallas.tpu as pltpu

NB = 128
PA = 0.4375
PB = 1.0 / PA
CM = 512
M = 6
NP = M + 2
K_PRO = 5
N_PER = 5
TCH = 32
ROWS = ((0, 432), (432, 576))
PRO_ROWS = ((0, 464), (464, 576))
Z_ROWS = ((0, 240), (240, 288))
ZF_ROWS = ((0, 160), (160, 240), (240, 288))
SET_F, SET_G = (0, 7, 1, 2), (3, 4, 5, 6)

_PTS = (0.0, PA, -PA, 1.0, -1.0, PB, -PB)


def _den(i):
    d = 1.0
    for j, q in enumerate(_PTS):
        if j != i:
            d *= (_PTS[i] - q)
    return d


def _kernel(x_hbm, w_hbm, mean_hbm, var_hbm, g_hbm, b_hbm, o_hbm,
            xall, oall, wbuf, pm, pv, pg, pb, wt_ref, wt16, sc_ref, sh_ref, shx_ref, u_scr, m_scr, c_scr,
            in_sem, out_sem, w_sem, xa_sem, misc_sem):
    S, C, B = x_hbm.shape
    NT = B // NB
    TS = S + 1
    NGT = NT * TS // M
    GB = 2 * TS // M
    N_IT = NT - 1
    HZ = C // 2
    KT = CM // 128 + 1
    CR = C - CM
    f32 = jnp.float32
    bf16 = jnp.bfloat16
    pk = lambda v: pltpu.bitcast(v, jnp.uint32)
    upk = lambda v: pltpu.bitcast(v, bf16)
    k_rows = (C,) + (CM + 128,) * M + (CM,)

    a, b = PA, PB
    a2, b2 = a * a, b * b
    ee = a2 + 1.0 + b2
    kap = 2.0 - a2 - b2

    def krange(kt):
        return slice(kt * 128, min(C, (kt + 1) * 128))

    def slot_ranges(lo, hi):
        out = []
        for bt in range(NT):
            a0, a1 = max(lo, bt * TS + 1), min(hi, (bt + 1) * TS)
            if a0 < a1:
                out.append((bt, a0 - bt * TS - 1, a1 - bt * TS - 1))
        return out

    def in_copies(lo, hi, sem):
        return [pltpu.make_async_copy(x_hbm.at[s0:s1, :, bt * NB:(bt + 1) * NB],
                                      xall.at[bt * TS + 1 + s0:bt * TS + 1 + s1], sem)
                for bt, s0, s1 in slot_ranges(lo, hi)]

    need = lambda g: M * (g + 1) + 1
    p_copies = [pltpu.make_async_copy(src, dst, misc_sem.at[2 + i])
                for i, (src, dst) in enumerate(((mean_hbm, pm), (var_hbm, pv), (g_hbm, pg), (b_hbm, pb)))]
    w_copies = [pltpu.make_async_copy(w_hbm.at[:, krange(kt), :], wbuf.at[:, krange(kt), :], w_sem.at[kt])
                for kt in range(KT)]
    xa_copies = [pltpu.make_async_copy(x_hbm.at[0:M, krange(kt), 0:NB], xall.at[1:M + 1, krange(kt), :],
                                       xa_sem.at[kt]) for kt in range(KT)]
    (xb_copy,) = in_copies(need(0), need(1), misc_sem.at[0])
    (xc_copy,) = in_copies(need(1), need(K_PRO - 1), misc_sem.at[1])
    for cp in p_copies + [c for wx in zip(w_copies, xa_copies) for c in wx] + [xb_copy, xc_copy]:
        cp.start()
    counts = []
    lo = need(K_PRO - 1)
    for it in range(N_IT):
        blk, j = (it + 1) // 2, (it + 1) % 2
        hi = need(GB * blk + N_PER * j + N_PER - 1 + j)
        for cp in in_copies(lo, hi, in_sem.at[it]):
            cp.start()
        counts.append(sum(s1 - s0 for _, s0, s1 in slot_ranges(lo, hi)))
        lo = hi

    for bt in range(NT + 1):
        xall[bt * TS] = jnp.zeros((C, NB), bf16)

    def pair(d, i):
        p = _PTS[i]
        if p == 1.0:
            ev = d[0] + d[2] + d[4]
            od = d[1] + d[3]
            if len(d) == M:
                od = od + d[5]
        else:
            ev = d[0] + (p ** 2) * d[2] + (p ** 4) * d[4]
            od = p * d[1] + (p ** 3) * d[3]
            if len(d) == M:
                od = od + (p ** 5) * d[5]
        return ev + od, ev - od

    def ext_rows(i, u_i, d_prev, d_last):
        p = _PTS[i]
        if d_last is None:
            return d_prev + p * u_i
        if p == 1.0:
            return d_prev + u_i - d_last
        if p == -1.0:
            return d_prev - u_i - d_last
        return d_prev + p * u_i - (p ** M) * d_last

    def transform(gi, zs=(0, 0, 0), short=False):
        base = M * gi
        rhs = [xall[base + 1]]
        for i in range(1, M, 2):
            bz = base + zs[i // 2]
            d = [xall[bz + 1 + k].astype(f32) for k in range(M - short)]
            d_prev = xall[bz, CM:C, :].astype(f32)
            for k, u in enumerate(pair(d, i)):
                ext = ext_rows(i + k, u[CM:C], d_prev, None if short else d[M - 1][CM:C])
                rhs.append(jnp.concatenate([u, ext], axis=0).astype(bf16))
        if not short:
            rhs.append(xall[base + M, 0:CM, :])
        return rhs

    def transform0(kt):
        for c0 in range(krange(kt).start, krange(kt).stop, TCH):
            d = [xall[1 + i, c0:c0 + TCH, :].astype(f32) for i in range(M)]
            for i in range(1, M, 2):
                for k, u in enumerate(pair(d, i)):
                    u_scr[i + k, c0 // 2:(c0 + TCH) // 2, :] = pk(u.astype(bf16))
                    if c0 >= CM:
                        ext = ext_rows(i + k, u, xall[0, c0:c0 + TCH, :].astype(f32), d[M - 1])
                        u_scr[i + k, (c0 + CR) // 2:(c0 + CR + TCH) // 2, :] = pk(ext.astype(bf16))

    def weight_prep(kt):
        for d0 in range(0, C, 128):
            dn = min(128, C - d0)
            rows = slice(d0 // 2, (d0 + dn) // 2)
            if kt < KT - 1:
                g0, g1, g2 = [wbuf[2 - k, krange(kt), d0:d0 + dn].T for k in range(3)]
                wt_ref[NP - 1, kt, rows, :] = pk(g2)
                g2 = g2.astype(f32)
            else:
                g0r = wbuf[2, CM:C, d0:d0 + dn]
                g0 = jnp.concatenate([g0r, jnp.zeros_like(g0r)], axis=0).T
                g1 = jnp.concatenate([wbuf[1, CM:C, d0:d0 + dn], wbuf[0, CM:C, d0:d0 + dn]], axis=0).T
                g2 = None
            wt_ref[0, kt, rows, :] = pk(g0)
            scl = sc_ref[d0:d0 + dn, :]
            g0, g1 = g0.astype(f32) * scl, g1.astype(f32) * scl
            if g2 is not None:
                g2 = g2 * scl
            for i in range(1, M, 2):
                pt, den = _PTS[i], _den(i)
                ev = g0 * (1.0 / den)
                if g2 is not None:
                    ev = ev + g2 * (pt * pt / den)
                od = g1 * (pt / den)
                wt16[i - 1, kt, d0:d0 + dn, :] = (ev + od).astype(bf16)
                wt16[i, kt, d0:d0 + dn, :] = (ev - od).astype(bf16)

    def rows_of(r0, r1, off):
        if off is None:
            return pl.ds(r0, r1 - r0)
        return pl.ds(pl.multiple_of(off * HZ + r0, 16), r1 - r0)

    def pick(ref, r0, r1, off, div=1):
        if off is None:
            return ref[r0 // div:r1 // div, :]
        return jnp.where(off == 0, ref[r0 // div:r1 // div, :], ref[(HZ + r0) // div:(HZ + r1) // div, :])

    def prod(i, rhs, r0, r1, kt0=0, kt1=KT, off=None, src="packed"):
        hi = min(kt1 * 128, k_rows[i])
        tiles = []
        for kt in range(kt0, (hi + 127) // 128):
            if src == "packed" or i in (0, NP - 1):
                tiles.append(upk(pick(wt_ref.at[i, kt], r0, r1, off, 2)))
            else:
                tiles.append(wt16[i - 1, kt, r0:r1, :])
                if src == "convert":
                    wt_ref[i, kt, r0 // 2:r1 // 2, :] = pk(tiles[-1])
        lhs = jnp.concatenate(tiles, axis=1)[:, :hi - kt0 * 128]
        return jnp.dot(lhs, rhs(kt0 * 128, hi), preferred_element_type=f32)

    def out_copy(slot, rs):
        if isinstance(slot, int):
            bt, s1 = slot // TS, slot % TS
            pltpu.make_async_copy(oall.at[pl.ds(slot, 1), rs], o_hbm.at[pl.ds(s1 - 1, 1), rs, pl.ds(bt * NB, NB)],
                                  out_sem.at[0]).start()
            return
        bt = jax.lax.shift_right_logical(slot * 1986, 16)
        s1 = slot - bt * TS

        @pl.when(s1 > 0)
        def _():
            pltpu.make_async_copy(oall.at[pl.ds(slot, 1), rs],
                                  o_hbm.at[pl.ds(s1 - 1, 1), rs, pl.ds(pl.multiple_of(bt * NB, NB), NB)],
                                  out_sem.at[0]).start()

    def epilogue(gi, m, carry, r0, r1, copy_out, off=None):
        rs = rows_of(r0, r1, off)

        def act(h, k):
            oall[M * gi + k, rs, :] = (h * jnp.tanh(h) + h).astype(bf16)

        sc, sh, shx = [pick(ref, r0, r1, off) for ref in (sc_ref, sh_ref, shx_ref)]
        m0 = m[0] * sc
        em0 = ee * m0
        sa, ta = m[1] + m[2], m[1] - m[2]
        s1, t1 = (m[3] + m[4]) + sh, (m[3] - m[4]) + sh
        sb, tb = m[5] + m[6], m[5] - m[6]
        o6 = ((s1 - m0) + sa) + sb
        o2 = ((s1 - em0) + b2 * sa) + a2 * sb
        o4 = ((shx - m0) + kap * s1) - o2 - o6
        q5 = (a * ta + t1) + b * tb
        q1 = (b * ta + t1) + a * tb
        q3 = (kap * t1 + shx) - q1 - q5
        if isinstance(carry, str):
            for h, k in ((o2, 2), (o4, 4), (q3, 3), (q5, 5)):
                act(h, k)
            for k in range(2, M):
                out_copy(M * gi + k, rs)

            def finish(c0, c1):
                act(m0 + c0, 0)
                act(q1 + c1, 1)
                out_copy(M * gi, rs)
                out_copy(M * gi + 1, rs)
            return finish
        if carry is not None:
            q1 = q1 + carry[1]
        m7 = None
        if len(m) == NP:
            m7 = m[7] * sc
            em7 = ee * m7
            q1, q3, q5 = q1 - m7, q3 + em7, q5 - em7
        if carry is not None:
            act(m0 + carry[0], 0)
        act(o2, 2)
        act(o4, 4)
        act(q1, 1)
        act(q3, 3)
        act(q5, 5)
        if copy_out:
            for k in range(M):
                out_copy(M * gi + k, rs)
        return o6, m7

    def group(gi, rhs, carry, rows, copy_out, after_first=None, src="packed"):
        out = []
        for h, (r0, r1) in enumerate(rows):
            out.append(epilogue(gi, [prod(i, lambda lo, hi, v=rhs[i]: v, r0, r1, src=src) for i in range(NP)],
                                carry[h], r0, r1, copy_out))
            if h == 0 and after_first is not None:
                after_first(out[0])
        return out

    def short_half(gi, zs, off, rows, carry):
        rhs = transform(gi, zs, True)
        return [epilogue(gi, [prod(i, lambda lo, hi, v=rhs[i]: v, r0, r1, off=off) for i in range(NP - 1)],
                         carry(r0, r1), r0, r1, True, off) for r0, r1 in rows]

    def save_carry(carry, rows):
        for h, (r0, r1) in enumerate(rows):
            c_scr[0, r0:r1, :] = carry[h][0]
            c_scr[1, r0:r1, :] = carry[h][1]

    for cp in p_copies:
        cp.wait()
    row = lambda r: r[...].astype(f32).reshape(1, C)
    scale = row(pg) * jax.lax.rsqrt(row(pv) + 1e-5)
    shift = row(pb) - row(pm) * scale
    sc_ref[...] = jnp.broadcast_to(0.5 * scale, (NB, C)).T
    sh_t = jnp.broadcast_to(0.5 * shift, (NB, C)).T
    sh_ref[...] = sh_t
    shx_ref[...] = (3.0 - kap) * sh_t

    def rhs0(i):
        if i == 0:
            return lambda lo, hi: xall[1, lo:hi, :]
        if i == NP - 1:
            return lambda lo, hi: xall[M, lo:hi, :]
        return lambda lo, hi: upk(u_scr[i, lo // 2:hi // 2, :])

    done = [0] * NP

    def advance(steps):
        acc = {}
        for i, kt1 in steps:
            part = prod(i, rhs0(i), 0, C, done[i], kt1, src="bf16")
            if i in acc:
                acc[i] = acc[i] + part
            else:
                acc[i] = part if done[i] == 0 else m_scr[i] + part
            done[i] = kt1
        for i, v in acc.items():
            m_scr[i] = v

    w_copies[0].wait()
    weight_prep(0)
    xa_copies[0].wait()
    transform0(0)
    advance([(i, 1) for i in SET_F])
    w_copies[1].wait()
    xa_copies[1].wait()
    weight_prep(1)
    transform0(1)
    advance([(i, 1) for i in SET_G] + [(i, 2) for i in SET_G])
    w_copies[2].wait()
    xa_copies[2].wait()
    weight_prep(2)
    transform0(2)
    advance([(i, 2) for i in SET_F] + [(i, 3) for i in SET_F])
    for kt in (3, 4):
        w_copies[kt].wait()
        xa_copies[kt].wait()
    for kt in (3, 4):
        weight_prep(kt)
        transform0(kt)
    advance([(i, 3) for i in SET_G] + [(i, 4) for i in SET_F] + [(i, 5) for i in (0, 1, 2)] + [(3, 4)])
    xb_copy.wait()
    cs = []
    for r0, r1 in ROWS:
        m = [m_scr[i, r0:r1, :] + prod(i, rhs0(i), r0, r1, done[i], src="bf16") if done[i] * 128 < k_rows[i]
             else m_scr[i, r0:r1, :] for i in range(NP)]
        cs.append(epilogue(0, m, None, r0, r1, False))
    carry = [jnp.concatenate([c[k] for c in cs], axis=0) for k in range(2)]
    carry = [(carry[0][r0:r1], carry[1][r0:r1]) for r0, r1 in PRO_ROWS]
    carry = group(1, transform(1), carry, PRO_ROWS, False, src="convert")
    save_carry(carry, PRO_ROWS)
    xc_copy.wait()

    def ramp(gi, c):
        zs = (0, jax.lax.shift_right_logical(gi, 8), jax.lax.shift_right_logical(gi, 9))
        carry = [(c_scr[0, r0:r1, :], c_scr[1, r0:r1, :]) for r0, r1 in ROWS]
        save_carry(group(gi, transform(gi, zs), carry, ROWS, False), ROWS)
        return c

    jax.lax.fori_loop(2, K_PRO, ramp, 0)

    n_lo, n_hi = min(counts), max(counts)

    def body(it, c):
        blk = jax.lax.shift_right_logical(it + 1, 1)
        j = jnp.bitwise_and(it + 1, 1)
        g0 = GB * blk + N_PER * j
        pltpu.make_async_copy(xall.at[0:n_lo], xall.at[0:n_lo], in_sem.at[it]).wait()

        @pl.when(j == 1)
        def _():
            pltpu.make_async_copy(xall.at[0:n_hi - n_lo], xall.at[0:n_hi - n_lo], in_sem.at[it]).wait()

        @pl.when(it == 0)
        def _():
            for bt, s0, s1 in slot_ranges(0, M * K_PRO):
                pltpu.make_async_copy(oall.at[bt * TS + 1 + s0:bt * TS + 1 + s1],
                                      o_hbm.at[s0:s1, :, bt * NB:(bt + 1) * NB], out_sem.at[0]).start()

        zs = (0, jax.lax.shift_right_logical(it, 8), jax.lax.shift_right_logical(it, 9))
        second = j == 1
        fin = short_half(GB * (blk + j) - 1, zs, 1 - j, Z_ROWS, lambda r0, r1: "later")
        c_in = [c_scr[k, HZ:C, :] for k in range(2)]
        carry = [(c_scr[0, r0:r1, :], jnp.where(second, c_scr[1, r0:r1, :], 0.0)) for r0, r1 in ROWS]

        def finish_short(c_out):
            for f, (r0, r1) in zip(fin, Z_ROWS):
                f(*[jnp.where(second, c_out[k][r0:r1], c_in[k][r0:r1]) for k in range(2)])

        for r in range(N_PER):
            gi = g0 + r
            carry = group(gi, transform(gi, zs), carry, ROWS, True, finish_short if r == N_PER - 1 else None)
        save_carry(carry, ROWS)
        return c

    jax.lax.fori_loop(0, N_IT, body, 0)
    short_half(NGT - 1, (0, 0, 0), None, [(HZ + r0, HZ + r1) for r0, r1 in ZF_ROWS],
               lambda r0, r1: (c_scr[0, r0:r1, :], c_scr[1, r0:r1, :]))
    pltpu.make_async_copy(oall.at[0:NT * S], oall.at[0:NT * S], out_sem.at[0]).wait()


@jax.jit
def pallas_standalone__batchnorm__sampling_kernel(
    x: jax.Array,
    w: jax.Array,
    mean: jax.Array,
    var: jax.Array,
    g: jax.Array,
    b: jax.Array,
):
    B, S, C = x.shape
    assert (B, S, C) == (1024, 32, 576) and w.shape == (3, C, C)
    NT = B // NB
    KT = CM // 128 + 1
    n_it = NT - 1
    xt = jnp.transpose(x, (1, 2, 0))
    ot = pl.pallas_call(
        _kernel,
        in_specs=[pl.BlockSpec(memory_space=pl.ANY)] * 6,
        out_specs=pl.BlockSpec(memory_space=pl.ANY),
        out_shape=jax.ShapeDtypeStruct((S, C, B), x.dtype),
        scratch_shapes=[pltpu.VMEM((NT * (S + 1) + 1, C, NB), jnp.bfloat16),
                        pltpu.VMEM((NT * (S + 1), C, NB), jnp.bfloat16),
                        pltpu.VMEM((3, C, C), jnp.bfloat16),
                        pltpu.VMEM((C,), jnp.bfloat16),
                        pltpu.VMEM((C,), jnp.bfloat16),
                        pltpu.VMEM((C,), jnp.bfloat16),
                        pltpu.VMEM((C,), jnp.bfloat16),
                        pltpu.VMEM((NP, KT, C // 2, 128), jnp.uint32),
                        pltpu.VMEM((M, KT, C, 128), jnp.bfloat16),
                        pltpu.VMEM((C, NB), jnp.float32),
                        pltpu.VMEM((C, NB), jnp.float32),
                        pltpu.VMEM((C, NB), jnp.float32),
                        pltpu.VMEM((NP - 1, KT * 64, NB), jnp.uint32),
                        pltpu.VMEM((NP, C, NB), jnp.float32),
                        pltpu.VMEM((2, C, NB), jnp.float32),
                        pltpu.SemaphoreType.DMA((n_it,)),
                        pltpu.SemaphoreType.DMA((1,)),
                        pltpu.SemaphoreType.DMA((KT,)),
                        pltpu.SemaphoreType.DMA((KT,)),
                        pltpu.SemaphoreType.DMA((6,))],
        compiler_params=pltpu.CompilerParams(vmem_limit_bytes=110 * 1024 * 1024,
                                             disable_bounds_checks=True,
                                             disable_semaphore_checks=True),
    )(xt, w, mean, var, g, b)
    return jnp.transpose(ot, (2, 0, 1))
```

```python
import jax
import jax.numpy as jnp
import jax.experimental.pallas as pl
import jax.experimental.pallas.tpu as pltpu

NB = 128
PA = 0.4375
PB = 1.0 / PA
CM = 512
M = 6
NP = M + 2
K_PRO = 5
N_PER = 5
TCH = 32
ROWS = ((0, 432), (432, 576))
PRO_ROWS = ((0, 464), (464, 576))
Z_ROWS = ((0, 208), (208, 256), (256, 288))
ZF_ROWS = ((0, 160), (160, 240), (240, 288))
SET_F, SET_G = (0, 1, 2, 3), (4, 5, 6, 7)

_PTS = (0.0, PA, -PA, 1.0, -1.0, PB, -PB)


def _den(i):
    d = 1.0
    for j, q in enumerate(_PTS):
        if j != i:
            d *= (_PTS[i] - q)
    return d


def _kernel(x_hbm, w_hbm, mean_hbm, var_hbm, g_hbm, b_hbm, o_hbm,
            xall, oall, wbuf, pm, pv, pg, pb, wt_ref, wt16, sc_ref, sh_ref, shx_ref, u_scr, m_scr, c_scr,
            in_sem, out_sem, w_sem, xa_sem, misc_sem):
    S, C, B = x_hbm.shape
    NT = B // NB
    TS = S + 1
    NGT = NT * TS // M
    GB = 2 * TS // M
    N_IT = NT - 1
    HZ = C // 2
    KT = CM // 128 + 1
    CR = C - CM
    f32 = jnp.float32
    bf16 = jnp.bfloat16
    pk = lambda v: pltpu.bitcast(v, jnp.uint32)
    upk = lambda v: pltpu.bitcast(v, bf16)
    k_rows = (C,) + (CM + 128,) * M + (CM,)

    a, b = PA, PB
    a2, b2 = a * a, b * b
    ee = a2 + 1.0 + b2
    kap = 2.0 - a2 - b2

    def krange(kt):
        return slice(kt * 128, min(C, (kt + 1) * 128))

    def slot_ranges(lo, hi):
        out = []
        for bt in range(NT):
            a0, a1 = max(lo, bt * TS + 1), min(hi, (bt + 1) * TS)
            if a0 < a1:
                out.append((bt, a0 - bt * TS - 1, a1 - bt * TS - 1))
        return out

    def in_copies(lo, hi, sem):
        return [pltpu.make_async_copy(x_hbm.at[s0:s1, :, bt * NB:(bt + 1) * NB],
                                      xall.at[bt * TS + 1 + s0:bt * TS + 1 + s1], sem)
                for bt, s0, s1 in slot_ranges(lo, hi)]

    need = lambda g: M * (g + 1) + 1
    p_copies = [pltpu.make_async_copy(src, dst, misc_sem.at[2 + i])
                for i, (src, dst) in enumerate(((mean_hbm, pm), (var_hbm, pv), (g_hbm, pg), (b_hbm, pb)))]
    w_copies = [pltpu.make_async_copy(w_hbm.at[:, krange(kt), :], wbuf.at[:, krange(kt), :], w_sem.at[kt])
                for kt in range(KT)]
    xa_copies = [pltpu.make_async_copy(x_hbm.at[0:M, krange(kt), 0:NB], xall.at[1:M + 1, krange(kt), :],
                                       xa_sem.at[kt]) for kt in range(KT)]
    (xb_copy,) = in_copies(need(0), need(1), misc_sem.at[0])
    (xc_copy,) = in_copies(need(1), need(K_PRO - 1), misc_sem.at[1])
    for cp in p_copies + [c for wx in zip(w_copies, xa_copies) for c in wx] + [xb_copy, xc_copy]:
        cp.start()
    counts = []
    lo = need(K_PRO - 1)
    for it in range(N_IT):
        blk, j = (it + 1) // 2, (it + 1) % 2
        hi = need(GB * blk + N_PER * j + N_PER - 1 + j)
        for cp in in_copies(lo, hi, in_sem.at[it]):
            cp.start()
        counts.append(sum(s1 - s0 for _, s0, s1 in slot_ranges(lo, hi)))
        lo = hi

    for bt in range(NT + 1):
        xall[bt * TS] = jnp.zeros((C, NB), bf16)

    def pair(d, i):
        p = _PTS[i]
        if p == 1.0:
            ev = d[0] + d[2] + d[4]
            od = d[1] + d[3]
            if len(d) == M:
                od = od + d[5]
        else:
            ev = d[0] + (p ** 2) * d[2] + (p ** 4) * d[4]
            od = p * d[1] + (p ** 3) * d[3]
            if len(d) == M:
                od = od + (p ** 5) * d[5]
        return ev + od, ev - od

    def ext_rows(i, u_i, d_prev, d_last):
        p = _PTS[i]
        if d_last is None:
            return d_prev + p * u_i
        if p == 1.0:
            return d_prev + u_i - d_last
        if p == -1.0:
            return d_prev - u_i - d_last
        return d_prev + p * u_i - (p ** M) * d_last

    def transform(gi, zs=(0, 0, 0), short=False):
        base = M * gi
        rhs = [xall[base + 1]]
        for i in range(1, M, 2):
            bz = base + zs[i // 2]
            d = [xall[bz + 1 + k].astype(f32) for k in range(M - short)]
            d_prev = xall[bz, CM:C, :].astype(f32)
            for k, u in enumerate(pair(d, i)):
                ext = ext_rows(i + k, u[CM:C], d_prev, None if short else d[M - 1][CM:C])
                rhs.append(jnp.concatenate([u, ext], axis=0).astype(bf16))
        if not short:
            rhs.append(xall[base + M, 0:CM, :])
        return rhs

    def transform0(kt):
        for c0 in range(krange(kt).start, krange(kt).stop, TCH):
            d = [xall[1 + i, c0:c0 + TCH, :].astype(f32) for i in range(M)]
            for i in range(1, M, 2):
                for k, u in enumerate(pair(d, i)):
                    u_scr[i + k, c0 // 2:(c0 + TCH) // 2, :] = pk(u.astype(bf16))
                    if c0 >= CM:
                        ext = ext_rows(i + k, u, xall[0, c0:c0 + TCH, :].astype(f32), d[M - 1])
                        u_scr[i + k, (c0 + CR) // 2:(c0 + CR + TCH) // 2, :] = pk(ext.astype(bf16))

    def weight_prep(kt):
        for d0 in range(0, C, 128):
            dn = min(128, C - d0)
            rows = slice(d0 // 2, (d0 + dn) // 2)
            if kt < KT - 1:
                g0, g1, g2 = [wbuf[2 - k, krange(kt), d0:d0 + dn].T for k in range(3)]
                wt_ref[NP - 1, kt, rows, :] = pk(g2)
                g2 = g2.astype(f32)
            else:
                g0r = wbuf[2, CM:C, d0:d0 + dn]
                g0 = jnp.concatenate([g0r, jnp.zeros_like(g0r)], axis=0).T
                g1 = jnp.concatenate([wbuf[1, CM:C, d0:d0 + dn], wbuf[0, CM:C, d0:d0 + dn]], axis=0).T
                g2 = None
            wt_ref[0, kt, rows, :] = pk(g0)
            scl = sc_ref[d0:d0 + dn, :]
            g0, g1 = g0.astype(f32) * scl, g1.astype(f32) * scl
            if g2 is not None:
                g2 = g2 * scl
            for i in range(1, M, 2):
                pt, den = _PTS[i], _den(i)
                ev = g0 * (1.0 / den)
                if g2 is not None:
                    ev = ev + g2 * (pt * pt / den)
                od = g1 * (pt / den)
                wt16[i - 1, kt, d0:d0 + dn, :] = (ev + od).astype(bf16)
                wt16[i, kt, d0:d0 + dn, :] = (ev - od).astype(bf16)

    def rows_of(r0, r1, off):
        if off is None:
            return pl.ds(r0, r1 - r0)
        return pl.ds(pl.multiple_of(off * HZ + r0, 16), r1 - r0)

    def pick(ref, r0, r1, off, div=1):
        if off is None:
            return ref[r0 // div:r1 // div, :]
        return jnp.where(off == 0, ref[r0 // div:r1 // div, :], ref[(HZ + r0) // div:(HZ + r1) // div, :])

    def prod(i, rhs, r0, r1, kt0=0, kt1=KT, off=None, src="packed"):
        hi = min(kt1 * 128, k_rows[i])
        tiles = []
        for kt in range(kt0, (hi + 127) // 128):
            if src == "packed" or i in (0, NP - 1):
                tiles.append(upk(pick(wt_ref.at[i, kt], r0, r1, off, 2)))
            else:
                tiles.append(wt16[i - 1, kt, r0:r1, :])
                if src == "convert":
                    wt_ref[i, kt, r0 // 2:r1 // 2, :] = pk(tiles[-1])
        lhs = jnp.concatenate(tiles, axis=1)[:, :hi - kt0 * 128]
        return jnp.dot(lhs, rhs(kt0 * 128, hi), preferred_element_type=f32)

    def out_copy(slot, rs):
        if isinstance(slot, int):
            bt, s1 = slot // TS, slot % TS
            pltpu.make_async_copy(oall.at[pl.ds(slot, 1), rs], o_hbm.at[pl.ds(s1 - 1, 1), rs, pl.ds(bt * NB, NB)],
                                  out_sem.at[0]).start()
            return
        bt = jax.lax.shift_right_logical(slot * 1986, 16)
        s1 = slot - bt * TS

        @pl.when(s1 > 0)
        def _():
            pltpu.make_async_copy(oall.at[pl.ds(slot, 1), rs],
                                  o_hbm.at[pl.ds(s1 - 1, 1), rs, pl.ds(pl.multiple_of(bt * NB, NB), NB)],
                                  out_sem.at[0]).start()

    def epilogue(gi, m, carry, r0, r1, copy_out, off=None):
        rs = rows_of(r0, r1, off)

        def act(h, k):
            oall[M * gi + k, rs, :] = (h * jnp.tanh(h) + h).astype(bf16)

        sc, sh, shx = [pick(ref, r0, r1, off) for ref in (sc_ref, sh_ref, shx_ref)]
        m0 = m[0] * sc
        em0 = ee * m0
        sa, ta = m[1] + m[2], m[1] - m[2]
        s1, t1 = (m[3] + m[4]) + sh, (m[3] - m[4]) + sh
        sb, tb = m[5] + m[6], m[5] - m[6]
        o6 = ((s1 - m0) + sa) + sb
        o2 = ((s1 - em0) + b2 * sa) + a2 * sb
        o4 = ((shx - m0) + kap * s1) - o2 - o6
        q5 = (a * ta + t1) + b * tb
        q1 = (b * ta + t1) + a * tb
        q3 = (kap * t1 + shx) - q1 - q5
        if isinstance(carry, str):
            for h, k in ((o2, 2), (o4, 4), (q3, 3), (q5, 5)):
                act(h, k)
            for k in range(2, M):
                out_copy(M * gi + k, rs)

            def finish(c0, c1):
                act(m0 + c0, 0)
                act(q1 + c1, 1)
                out_copy(M * gi, rs)
                out_copy(M * gi + 1, rs)
            return finish
        if carry is not None:
            q1 = q1 + carry[1]
        m7 = None
        if len(m) == NP:
            m7 = m[7] * sc
            em7 = ee * m7
            q1, q3, q5 = q1 - m7, q3 + em7, q5 - em7
        if carry is not None:
            act(m0 + carry[0], 0)
        act(o2, 2)
        act(o4, 4)
        act(q1, 1)
        act(q3, 3)
        act(q5, 5)
        if copy_out:
            for k in range(M):
                out_copy(M * gi + k, rs)
        return o6, m7

    def group(gi, rhs, carry, rows, copy_out, after_first=None, src="packed"):
        out = []
        for h, (r0, r1) in enumerate(rows):
            out.append(epilogue(gi, [prod(i, lambda lo, hi, v=rhs[i]: v, r0, r1, src=src) for i in range(NP)],
                                carry[h], r0, r1, copy_out))
            if h == 0 and after_first is not None:
                after_first(out[0])
        return out

    def short_half(gi, zs, off, rows, carry):
        rhs = transform(gi, zs, True)
        return [epilogue(gi, [prod(i, lambda lo, hi, v=rhs[i]: v, r0, r1, off=off) for i in range(NP - 1)],
                         carry(r0, r1), r0, r1, True, off) for r0, r1 in rows]

    def save_carry(carry, rows):
        for h, (r0, r1) in enumerate(rows):
            c_scr[0, r0:r1, :] = carry[h][0]
            c_scr[1, r0:r1, :] = carry[h][1]

    for cp in p_copies:
        cp.wait()
    row = lambda r: r[...].astype(f32).reshape(1, C)
    scale = row(pg) * jax.lax.rsqrt(row(pv) + 1e-5)
    shift = row(pb) - row(pm) * scale
    sc_ref[...] = jnp.broadcast_to(0.5 * scale, (NB, C)).T
    sh_t = jnp.broadcast_to(0.5 * shift, (NB, C)).T
    sh_ref[...] = sh_t
    shx_ref[...] = (3.0 - kap) * sh_t

    def rhs0(i):
        if i == 0:
            return lambda lo, hi: xall[1, lo:hi, :]
        if i == NP - 1:
            return lambda lo, hi: xall[M, lo:hi, :]
        return lambda lo, hi: upk(u_scr[i, lo // 2:hi // 2, :])

    done = [0] * NP

    def advance(steps):
        acc = {}
        for i, kt1 in steps:
            part = prod(i, rhs0(i), 0, C, done[i], kt1, src="bf16")
            if i in acc:
                acc[i] = acc[i] + part
            else:
                acc[i] = part if done[i] == 0 else m_scr[i] + part
            done[i] = kt1
        for i, v in acc.items():
            m_scr[i] = v

    w_copies[0].wait()
    weight_prep(0)
    xa_copies[0].wait()
    transform0(0)
    advance([(i, 1) for i in SET_F])
    w_copies[1].wait()
    xa_copies[1].wait()
    weight_prep(1)
    transform0(1)
    advance([(i, 1) for i in SET_G] + [(i, 2) for i in SET_G])
    w_copies[2].wait()
    xa_copies[2].wait()
    weight_prep(2)
    transform0(2)
    advance([(i, 2) for i in SET_F] + [(i, 3) for i in SET_F])
    for kt in (3, 4):
        w_copies[kt].wait()
        xa_copies[kt].wait()
    for kt in (3, 4):
        weight_prep(kt)
        transform0(kt)
    advance([(i, 3) for i in SET_G] + [(i, 4) for i in SET_F] + [(i, 5) for i in SET_F])
    xb_copy.wait()
    cs = []
    for r0, r1 in ROWS:
        m = [m_scr[i, r0:r1, :] + prod(i, rhs0(i), r0, r1, done[i], src="bf16") if done[i] * 128 < k_rows[i]
             else m_scr[i, r0:r1, :] for i in range(NP)]
        cs.append(epilogue(0, m, None, r0, r1, False))
    carry = [jnp.concatenate([c[k] for c in cs], axis=0) for k in range(2)]
    carry = [(carry[0][r0:r1], carry[1][r0:r1]) for r0, r1 in PRO_ROWS]
    carry = group(1, transform(1), carry, PRO_ROWS, False, src="convert")
    save_carry(carry, PRO_ROWS)
    xc_copy.wait()

    def ramp(gi, c):
        zs = (0, jax.lax.shift_right_logical(gi, 8), jax.lax.shift_right_logical(gi, 9))
        carry = [(c_scr[0, r0:r1, :], c_scr[1, r0:r1, :]) for r0, r1 in ROWS]
        save_carry(group(gi, transform(gi, zs), carry, ROWS, False), ROWS)
        return c

    jax.lax.fori_loop(2, K_PRO, ramp, 0)

    n_hi, n_lo = counts[0], counts[1]
    assert counts == [n_hi, n_lo] * (N_IT // 2) + [n_hi]

    def body(it, c):
        blk = jax.lax.shift_right_logical(it + 1, 1)
        j = jnp.bitwise_and(it + 1, 1)
        g0 = GB * blk + N_PER * j
        for jj, n in ((0, n_lo), (1, n_hi)):
            @pl.when(j == jj)
            def _():
                pltpu.make_async_copy(xall.at[0:n], xall.at[0:n], in_sem.at[it]).wait()

        @pl.when(it == 0)
        def _():
            for bt, s0, s1 in slot_ranges(0, M * K_PRO):
                pltpu.make_async_copy(oall.at[bt * TS + 1 + s0:bt * TS + 1 + s1],
                                      o_hbm.at[s0:s1, :, bt * NB:(bt + 1) * NB], out_sem.at[0]).start()

        zs = (0, jax.lax.shift_right_logical(it, 8), jax.lax.shift_right_logical(it, 9))
        second = j == 1
        fin = short_half(GB * (blk + j) - 1, zs, 1 - j, Z_ROWS, lambda r0, r1: "later")
        c_in = [c_scr[k, HZ:C, :] for k in range(2)]
        carry = [(c_scr[0, r0:r1, :], jnp.where(second, c_scr[1, r0:r1, :], 0.0)) for r0, r1 in ROWS]

        def finish_short(c_out):
            for f, (r0, r1) in zip(fin, Z_ROWS):
                f(*[jnp.where(second, c_out[k][r0:r1], c_in[k][r0:r1]) for k in range(2)])

        for r in range(N_PER):
            gi = g0 + r
            carry = group(gi, transform(gi, zs), carry, ROWS, True, finish_short if r == N_PER - 1 else None)
        save_carry(carry, ROWS)
        return c

    jax.lax.fori_loop(0, N_IT, body, 0)
    short_half(NGT - 1, (0, 0, 0), None, [(HZ + r0, HZ + r1) for r0, r1 in ZF_ROWS],
               lambda r0, r1: (c_scr[0, r0:r1, :], c_scr[1, r0:r1, :]))
    pltpu.make_async_copy(oall.at[0:NT * S], oall.at[0:NT * S], out_sem.at[0]).wait()


@jax.jit
def pallas_standalone__batchnorm__sampling_kernel(
    x: jax.Array,
    w: jax.Array,
    mean: jax.Array,
    var: jax.Array,
    g: jax.Array,
    b: jax.Array,
):
    B, S, C = x.shape
    assert (B, S, C) == (1024, 32, 576) and w.shape == (3, C, C)
    NT = B // NB
    KT = CM // 128 + 1
    n_it = NT - 1
    xt = jnp.transpose(x, (1, 2, 0))
    ot = pl.pallas_call(
        _kernel,
        in_specs=[pl.BlockSpec(memory_space=pl.ANY)] * 6,
        out_specs=pl.BlockSpec(memory_space=pl.ANY),
        out_shape=jax.ShapeDtypeStruct((S, C, B), x.dtype),
        scratch_shapes=[pltpu.VMEM((NT * (S + 1) + 1, C, NB), jnp.bfloat16),
                        pltpu.VMEM((NT * (S + 1), C, NB), jnp.bfloat16),
                        pltpu.VMEM((3, C, C), jnp.bfloat16),
                        pltpu.VMEM((C,), jnp.bfloat16),
                        pltpu.VMEM((C,), jnp.bfloat16),
                        pltpu.VMEM((C,), jnp.bfloat16),
                        pltpu.VMEM((C,), jnp.bfloat16),
                        pltpu.VMEM((NP, KT, C // 2, 128), jnp.uint32),
                        pltpu.VMEM((M, KT, C, 128), jnp.bfloat16),
                        pltpu.VMEM((C, NB), jnp.float32),
                        pltpu.VMEM((C, NB), jnp.float32),
                        pltpu.VMEM((C, NB), jnp.float32),
                        pltpu.VMEM((NP - 1, KT * 64, NB), jnp.uint32),
                        pltpu.VMEM((NP, C, NB), jnp.float32),
                        pltpu.VMEM((2, C, NB), jnp.float32),
                        pltpu.SemaphoreType.DMA((n_it,)),
                        pltpu.SemaphoreType.DMA((1,)),
                        pltpu.SemaphoreType.DMA((KT,)),
                        pltpu.SemaphoreType.DMA((KT,)),
                        pltpu.SemaphoreType.DMA((6,))],
        compiler_params=pltpu.CompilerParams(vmem_limit_bytes=110 * 1024 * 1024,
                                             disable_bounds_checks=True,
                                             disable_semaphore_checks=True),
    )(xt, w, mean, var, g, b)
    return jnp.transpose(ot, (2, 0, 1))
```
